```python
import jax
import jax.numpy as jnp

def _softmax(x, axis=-1):
    return jax.nn.softmax(x, axis=axis)
def _gelu(x):
    return jax.nn.gelu(x, approximate=True)
def _silu(x):
    return jax.nn.silu(x)
def _sigmoid(x):
    return jax.nn.sigmoid(x)
def _layernorm(x, axis=-1, eps=1e-5):
    m = jnp.mean(x, axis=axis, keepdims=True)
    v = jnp.var(x, axis=axis, keepdims=True)
    return (x - m) / jnp.sqrt(v + eps)
def _scatter_add(tgt, idx, src, axis=0):
    return tgt.at[idx].add(src)
def _segment_sum(src, seg, n):
    return jax.ops.segment_sum(src, seg, n)
class _Rng:
    def __init__(self, key):
        self._k = key
    def _next(self):
        self._k, sub = jax.random.split(self._k)
        return sub
    def normal(self, shape):
        return jax.random.normal(self._next(), shape, dtype=jnp.bfloat16)
    def randint(self, lo, hi, shape):
        return jax.random.randint(self._next(), shape, lo, hi, dtype=jnp.int32)
    def uniform(self, shape, lo=0.0, hi=1.0):
        return jax.random.uniform(self._next(), shape, jnp.bfloat16, lo, hi)
    def permutation(self, n):
        return jax.random.permutation(self._next(), n)


kernel_name = 'recurrent_scan__linear_kernel_hedgehog__moe_arch_mod__prompt'

def setup_inputs():
    _rng = _Rng(jax.random.key(int.from_bytes(__import__("os").urandom(4), "little")))
    _w = (lambda a: (lambda t: t.astype(jnp.bfloat16) if jnp.issubdtype(t.dtype, jnp.floating) else t)(jnp.asarray(a)))
    def _A_setup():
        B, S, D, H = 1, 2048, 1024, 32
        Dh = D // H
        return {
            "x": _w((lambda *s: _rng.normal(s) * 0.05)(B, S, D)),
            "wqkv": _w((lambda *s: _rng.normal(s) * 0.05)(D, 3 * D)),
            "w_phi": _w((lambda *s: _rng.normal(s) * 0.05)(H, Dh, Dh) * (Dh ** -0.5)),
            "wo": _w((lambda *s: _rng.normal(s) * 0.05)(D, D)),
        }
    _A_in = _A_setup()

    def _B_setup():
        B, S, D, F, C = 1, 2048, 1024, 3584, 1
        return {
            "x": _w((lambda *s: _rng.normal(s) * 0.05)(B, S, D)),
            "w_r": _w((lambda *s: _rng.normal(s) * 0.05)(D)),
            "w_gate": _w((lambda *s: _rng.normal(s) * 0.05)(D, F)),
            "w_up": _w((lambda *s: _rng.normal(s) * 0.05)(D, F)),
            "w_down": _w((lambda *s: _rng.normal(s) * 0.05)(F, D)),
        }
    _B_in = _B_setup()

    return {
        "A_x": _A_in["x"],
        "A_wqkv": _A_in["wqkv"],
        "A_w_phi": _A_in["w_phi"],
        "A_wo": _A_in["wo"],
        "B_x": _B_in["x"],
        "B_w_r": _B_in["w_r"],
        "B_w_gate": _B_in["w_gate"],
        "B_w_up": _B_in["w_up"],
        "B_w_down": _B_in["w_down"],
    }

def reference(A_x, A_wqkv, A_w_phi, A_wo, B_x, B_w_r, B_w_gate, B_w_up, B_w_down):
    def _A_ref(x, wqkv, w_phi, wo):
        B, S, D = x.shape
        H = 32; Dh = D // H
        qkv = (lambda x, *d: x.transpose(*d))((x @ wqkv).reshape(B, S, 3, H, Dh), 2, 0, 3, 1, 4)
        q, k, v = qkv[0], qkv[1], qkv[2]
        pq = jnp.einsum("bhsd,hdf->bhsf", q, w_phi)
        pk = jnp.einsum("bhsd,hdf->bhsf", k, w_phi)
        phi_q = jnp.concatenate([_softmax(pq, axis=-1), _softmax(-pq, axis=-1)], axis=-1)
        phi_k = jnp.concatenate([_softmax(pk, axis=-1), _softmax(-pk, axis=-1)], axis=-1)
        kv = jnp.einsum("bhsf,bhsd->bhfd", phi_k, v)
        z  = jnp.einsum("bhsf->bhf", phi_k)
        num = jnp.einsum("bhqf,bhfd->bhqd", phi_q, kv)
        den = jnp.einsum("bhqf,bhf->bhq", phi_q, z)[..., None] + 1e-6
        o = num / den
        return (lambda x, *d: x.transpose(*d))(o, 0, 2, 1, 3).reshape(B, S, D) @ wo

    def _B_ref(x, w_r, w_gate, w_up, w_down):
        B, S, D = x.shape
        C = 1
        r = x @ w_r
        idx = jnp.argsort(-r, axis=-1)[:, :C]
        idx_e = jnp.repeat(idx.reshape(B, C, 1), D, axis=2)
        x_sel = jnp.take_along_axis(x, idx_e, axis=1)
        g = _silu(x_sel @ w_gate)
        u = x_sel @ w_up
        y = (g * u) @ w_down
        r_sel = _sigmoid(jnp.take_along_axis(r, idx, axis=1))
        y = y * r_sel.reshape(B, C, 1)
        b_off = (jnp.arange(B) * S).reshape(B, 1)
        flat_idx = (idx + b_off).reshape(B * C)
        zero = (x * 0.0).reshape(B * S, D)
        upd = _scatter_add(zero, flat_idx, y.reshape(B * C, D), axis=0)
        return x + upd.reshape(B, S, D)

    x = A_x
    xn = _layernorm(x, axis=-1)
    s = _A_ref(xn, A_wqkv, A_w_phi, A_wo)
    g = _silu(_B_ref(xn, B_w_r, B_w_gate, B_w_up, B_w_down))
    return x + s * g
```

```python
import functools

import jax
import jax.numpy as jnp
from jax import lax
import jax.experimental.pallas as pl
import jax.experimental.pallas.tpu as pltpu

S, D, H, DH, F = 2048, 1024, 32, 32, 3584
T = 256
NT = S // T
MC = 256
NC = D // MC
NP = H // 2
GR = 80
FC = F // (NT - 1)
NB = 256
LOG2E = 1.4426950408889634
EPS_LN = 1.0013580322265625e-05
F32 = jnp.float32
BF16 = jnp.bfloat16

_NT_DIMS = (((1,), (1,)), ((), ()))


def _dot_nt(a, b):
    return lax.dot_general(a, b, _NT_DIMS, preferred_element_type=F32)


def _dot(a, b):
    return jnp.dot(a, b, preferred_element_type=F32)


def _rb(x):
    return x.astype(BF16).astype(F32)


def _phi_pair(p):
    pos, neg = [], []
    for a in range(2):
        ph = p[32 * a:32 * a + 32, :]
        mx = jnp.max(ph, axis=0, keepdims=True)
        mn = jnp.min(ph, axis=0, keepdims=True)
        ep = jnp.exp2(ph - mx)
        en = jnp.exp2(mn - ph)
        pos.append(ep * pl.reciprocal(jnp.sum(ep, axis=0, keepdims=True), approx=True))
        neg.append(en * pl.reciprocal(jnp.sum(en, axis=0, keepdims=True), approx=True))
    return jnp.concatenate(pos + neg, axis=0).astype(BF16)


def _silu(x):
    h = 0.5 * x
    return h + h * jnp.tanh(h)


def _kernel(x_hbm, wqkv_hbm, wphi_hbm, wo_hbm, wr_hbm, wg_hbm, wu_hbm, wd_hbm, out_hbm,
            x_buf, xn_buf, w_buf, wt_buf, wphi_buf, wr_buf, wo_buf, wg_buf, wu_buf, wd_buf,
            bdt_buf, g_acc, g_buf, r_buf, o_buf, y_buf, out_buf,
            sem_x, sem_w, sem_s, sem_f, sem_o):
    def x_copy(i):
        return pltpu.make_async_copy(x_hbm.at[pl.ds(i * T, T), :], x_buf.at[pl.ds(i * T, T), :], sem_x.at[i])

    def w_copy(j):
        return pltpu.make_async_copy(wqkv_hbm.at[:, pl.ds(j * 256, 256)], w_buf.at[j], sem_w.at[j])

    phi_copy = pltpu.make_async_copy(wphi_hbm, wphi_buf, sem_s.at[0])
    wr_copy = pltpu.make_async_copy(wr_hbm, wr_buf, sem_s.at[1])
    wo_copy = pltpu.make_async_copy(wo_hbm, wo_buf, sem_s.at[2])

    def f_copies(c):
        return (pltpu.make_async_copy(wg_hbm.at[:, pl.ds(c * FC, FC)], wg_buf.at[c], sem_f.at[0, c]),
                pltpu.make_async_copy(wu_hbm.at[:, pl.ds(c * FC, FC)], wu_buf.at[c], sem_f.at[1, c]),
                pltpu.make_async_copy(wd_hbm.at[pl.ds(c * FC, FC), :], wd_buf.at[c], sem_f.at[2, c]))

    def out_copy(i):
        return pltpu.make_async_copy(out_buf.at[pl.ds(i * T, T), :], out_hbm.at[pl.ds(i * T, T), :], sem_o.at[i])

    phi_copy.start()
    wr_copy.start()
    x_copy(0).start()
    for j in range(4, 12):
        w_copy(j).start()
    x_copy(1).start()

    def layer_norm(i):
        rows = pl.ds(pl.multiple_of(i * T, T), T)
        x = x_buf[rows, :].astype(F32)
        m = jnp.mean(x, axis=-1, keepdims=True)
        xc = x - m
        v = jnp.mean(xc * xc, axis=-1, keepdims=True)
        den = _rb(jnp.sqrt(_rb(_rb(v) + EPS_LN)))
        xn_buf[rows, :] = (_rb(x - _rb(m)) * (1.0 / den)).astype(BF16)

    def fold(j):
        for u in range(2):
            g = (2 * j + u) % 8
            w = w_buf[j, :, u * 128:(u + 1) * 128]
            if j < 8:
                r = _dot_nt(bdt_buf[g], w) * LOG2E
            else:
                r = _dot_nt(bdt_buf[8], w)
            wt_buf[j * 256 + u * 128:j * 256 + (u + 1) * 128, :] = r.astype(BF16)

    phi_copy.wait()
    ri = lax.broadcasted_iota(jnp.int32, (128, 128), 0)
    ci = lax.broadcasted_iota(jnp.int32, (128, 128), 1)
    same_head = (ri // 32) == (ci // 32)
    e_r = lax.broadcasted_iota(jnp.int32, (128, 32), 0)
    e_c = lax.broadcasted_iota(jnp.int32, (128, 32), 1)
    tile_eye = jnp.where((e_r % 32) == e_c, 1.0, 0.0).astype(BF16)
    for g in range(8):
        wg4 = wphi_buf[4 * g:4 * g + 4].reshape(128, 32)
        bdt_buf[g] = jnp.where(same_head, _dot_nt(tile_eye, wg4), 0.0).astype(BF16)
    bdt_buf[8] = jnp.where(ri == ci, 1.0, 0.0).astype(BF16)

    wr_copy.wait()
    wt_buf[3 * D:3 * D + 16, :] = jnp.broadcast_to(wr_buf[...].astype(F32).reshape(1, D), (16, D)).astype(BF16)
    g_acc[...] = jnp.zeros_like(g_acc)
    y_buf[...] = jnp.zeros_like(y_buf)

    x_copy(0).wait()
    layer_norm(0)
    for j in range(4, 12):
        w_copy(j).wait()
        fold(j)
    for i in range(2, NT):
        x_copy(i).start()
    for j in range(4):
        w_copy(j).start()
    wo_copy.start()

    ones = jnp.ones((16, T), BF16)

    def kv_tile(i):
        rows = pl.ds(pl.multiple_of(i * T, T), T)
        xn = xn_buf[rows, :]
        for c in range(NC):
            pk = _dot_nt(wt_buf[D + c * MC:D + (c + 1) * MC, :], xn)
            if c == NC - 1:
                vr = _dot_nt(wt_buf[2 * D + c * MC:3 * D + 16, :], xn)
                r_buf[i] = vr[MC:MC + 8, :]
                vt = vr[:MC, :].astype(BF16)
            else:
                vt = _dot_nt(wt_buf[2 * D + c * MC:2 * D + (c + 1) * MC, :], xn).astype(BF16)
            for u in range(MC // 64):
                p = c * (MC // 64) + u
                phi = _phi_pair(pk[64 * u:64 * u + 64, :])
                lhs = jnp.concatenate([vt[64 * u:64 * u + 64, :], ones], axis=0)
                g_acc[p] += _dot_nt(lhs, phi)

    def pass1_body(i, carry):
        for cp in f_copies(i):
            cp.start()
        x_copy(i + 1).wait()
        layer_norm(i + 1)
        kv_tile(i)
        return carry

    lax.fori_loop(0, NT - 1, pass1_body, 0)
    for j in range(4):
        w_copy(j).wait()
    for j in range(4):
        fold(j)
    kv_tile(NT - 1)

    gr = lax.broadcasted_iota(jnp.int32, (GR, 128), 0)
    gc = lax.broadcasted_iota(jnp.int32, (GR, 128), 1)
    row_head = jnp.where(gr < 64, gr // 32, (gr - 64) // 8)
    keep = row_head == ((gc % 64) // 32)
    for p in range(NP):
        g_buf[p] = jnp.where(keep, g_acc[p], 0.0).astype(BF16)

    r_all = _rb(r_buf[...])
    tok = (lax.broadcasted_iota(jnp.int32, (NT, 8, T), 0) * T
           + lax.broadcasted_iota(jnp.int32, (NT, 8, T), 2))
    r_max = jnp.max(r_all)
    idx = jnp.min(jnp.where(r_all == r_max, tok, S - 1))
    sel_tile = idx // T
    blk = pl.multiple_of((idx // 16) * 16, 16)

    def tile_of(j):
        return (sel_tile + 1 + j) % NT

    def q_tile(j):
        rows = pl.ds(pl.multiple_of(tile_of(j) * T, T), T)
        xn = xn_buf[rows, :]
        slot = j % 2
        for c in range(NC):
            pq = _dot_nt(wt_buf[c * MC:(c + 1) * MC, :], xn)
            parts = []
            for u in range(MC // 64):
                p = c * (MC // 64) + u
                nd = _dot(g_buf[p], _phi_pair(pq[64 * u:64 * u + 64, :]))
                for a in range(2):
                    inv = pl.reciprocal(nd[64 + 8 * a:72 + 8 * a, :] + 1e-6, approx=True)
                    parts.append(nd[32 * a:32 * a + 32, :] * jnp.concatenate([inv] * 4, axis=0))
            ot = jnp.concatenate(parts, axis=0)
            o_buf[slot, :, c * MC:(c + 1) * MC] = ot.T.astype(BF16)

    def out_tile(j, upd=None):
        t = tile_of(j)
        rows = pl.ds(pl.multiple_of(t * T, T), T)
        o = o_buf[j % 2]
        for n in range(D // NB):
            cols = slice(n * NB, (n + 1) * NB)
            s = _dot(o, wo_buf[:, cols])
            xn = xn_buf[rows, cols].astype(F32)
            if upd is not None:
                xn = xn + upd[:, cols]
            out_buf[rows, cols] = (x_buf[rows, cols].astype(F32) + s * _silu(xn)).astype(BF16)
        out_copy(t).start()

    def ffn_chunk(c):
        xs = xn_buf[pl.ds(blk, 16), :]
        hg = _dot(xs, wg_buf[c])
        hu = _dot(xs, wu_buf[c])
        y_buf[...] += _dot((_silu(hg) * hu).astype(BF16), wd_buf[c])

    wo_copy.wait()
    q_tile(0)

    def pass2_body(j, carry):
        for cp in f_copies(j - 1):
            cp.wait()
        q_tile(j)
        out_tile(j - 1)
        ffn_chunk(j - 1)
        return carry

    lax.fori_loop(1, NT, pass2_body, 0)

    sub = lax.broadcasted_iota(jnp.int32, (16, D), 0)
    y_row = jnp.sum(jnp.where(sub == idx - blk, y_buf[...], 0.0), axis=0, keepdims=True)
    gate = 1.0 / (1.0 + jnp.exp(-jnp.full((1, D), r_max, F32)))
    trow = lax.broadcasted_iota(jnp.int32, (T, D), 0)
    upd = jnp.where(trow == idx - sel_tile * T, y_row * gate, 0.0)
    out_tile(NT - 1, upd)
    for i in range(NT):
        out_copy(i).wait()


@jax.jit
def pallas_recurrent_scan__linear_kernel_hedgehog__moe_arch_mod__prompt_kernel(
    A_x: jax.Array,
    A_wqkv: jax.Array,
    A_w_phi: jax.Array,
    A_wo: jax.Array,
    B_x: jax.Array,
    B_w_r: jax.Array,
    B_w_gate: jax.Array,
    B_w_up: jax.Array,
    B_w_down: jax.Array,
):
    del B_x
    any_spec = pl.BlockSpec(memory_space=pl.ANY)
    out = pl.pallas_call(
        _kernel,
        out_shape=jax.ShapeDtypeStruct((S, D), BF16),
        in_specs=[any_spec] * 8,
        out_specs=any_spec,
        scratch_shapes=[
            pltpu.VMEM((S, D), BF16),
            pltpu.VMEM((S, D), BF16),
            pltpu.VMEM((12, D, 256), BF16),
            pltpu.VMEM((3 * D + 16, D), BF16),
            pltpu.VMEM((H, DH, DH), BF16),
            pltpu.VMEM((D,), BF16),
            pltpu.VMEM((D, D), BF16),
            pltpu.VMEM((NT - 1, D, FC), BF16),
            pltpu.VMEM((NT - 1, D, FC), BF16),
            pltpu.VMEM((NT - 1, FC, D), BF16),
            pltpu.VMEM((9, 128, 128), BF16),
            pltpu.VMEM((NP, GR, 128), F32),
            pltpu.VMEM((NP, GR, 128), BF16),
            pltpu.VMEM((NT, 8, T), F32),
            pltpu.VMEM((2, T, D), BF16),
            pltpu.VMEM((16, D), F32),
            pltpu.VMEM((S, D), BF16),
            pltpu.SemaphoreType.DMA((NT,)),
            pltpu.SemaphoreType.DMA((12,)),
            pltpu.SemaphoreType.DMA((3,)),
            pltpu.SemaphoreType.DMA((3, NT - 1)),
            pltpu.SemaphoreType.DMA((NT,)),
        ],
        compiler_params=pltpu.CompilerParams(vmem_limit_bytes=100 * 1024 * 1024),
        name="hedgehog_mod",
    )(A_x.reshape(S, D), A_wqkv, A_w_phi, A_wo, B_w_r, B_w_gate, B_w_up, B_w_down)
    return out.reshape(1, S, D)
```

```python
import functools

import jax
import jax.numpy as jnp
from jax import lax
import jax.experimental.pallas as pl
import jax.experimental.pallas.tpu as pltpu

S, D, H, DH, F = 2048, 1024, 32, 32, 3584
T = 256
NT = S // T
MC = 256
NC = D // MC
NP = H // 2
GR = 80
FC = F // (NT - 1)
NB = 256
LOG2E = 1.4426950408889634
EPS_LN = 1.0013580322265625e-05
F32 = jnp.float32
BF16 = jnp.bfloat16
U32 = jnp.uint32

_NT_DIMS = (((1,), (1,)), ((), ()))


def _dot_nt(a, b):
    return lax.dot_general(a, b, _NT_DIMS, preferred_element_type=F32)


def _dot(a, b):
    return jnp.dot(a, b, preferred_element_type=F32)


def _rb(x):
    return x.astype(BF16).astype(F32)


def _pk(x):
    return pltpu.bitcast(x, jnp.uint32)


def _upk(x):
    return pltpu.bitcast(x, BF16)


def _phi_pair(p):
    pos, neg = [], []
    for a in range(2):
        ph = p[32 * a:32 * a + 32, :]
        mx = jnp.max(ph, axis=0, keepdims=True)
        mn = jnp.min(ph, axis=0, keepdims=True)
        ep = jnp.exp2(ph - mx)
        en = jnp.exp2(mn - ph)
        pos.append(ep * pl.reciprocal(jnp.sum(ep, axis=0, keepdims=True), approx=True))
        neg.append(en * pl.reciprocal(jnp.sum(en, axis=0, keepdims=True), approx=True))
    return jnp.concatenate(pos + neg, axis=0).astype(BF16)


def _silu(x):
    h = 0.5 * x
    return h + h * jnp.tanh(h)


def _kernel(x_hbm, wqkv_hbm, wphi_hbm, wo_hbm, wr_hbm, wg_hbm, wu_hbm, wd_hbm, out_hbm,
            x_buf, xn_buf, w_buf, wt_buf, wphi_buf, wr_buf, wo_buf, wg_buf, wu_buf, wd_buf,
            bdt_buf, g_acc, g_buf, r_buf, o_buf, y_buf, out_buf, zero_buf,
            sem_x, sem_w, sem_s, sem_f, sem_o):
    def x_copy(i):
        return pltpu.make_async_copy(x_hbm.at[pl.ds(i * T, T), :], x_buf.at[pl.ds(i * T, T), :], sem_x.at[i])

    def w_copy(j):
        return pltpu.make_async_copy(wqkv_hbm.at[:, pl.ds(j * 256, 256)], w_buf.at[j], sem_w.at[j])

    phi_copy = pltpu.make_async_copy(wphi_hbm, wphi_buf, sem_s.at[0])
    wr_copy = pltpu.make_async_copy(wr_hbm, wr_buf, sem_s.at[1])
    wo_copy = pltpu.make_async_copy(wo_hbm, wo_buf, sem_s.at[2])

    def f_copies(c):
        return (pltpu.make_async_copy(wg_hbm.at[:, pl.ds(c * FC, FC)], wg_buf.at[c], sem_f.at[0, c]),
                pltpu.make_async_copy(wu_hbm.at[:, pl.ds(c * FC, FC)], wu_buf.at[c], sem_f.at[1, c]),
                pltpu.make_async_copy(wd_hbm.at[pl.ds(c * FC, FC), :], wd_buf.at[c], sem_f.at[2, c]))

    def out_copy(i):
        return pltpu.make_async_copy(out_buf.at[pl.ds(i * T, T), :], out_hbm.at[pl.ds(i * T, T), :], sem_o.at[i])

    phi_copy.start()
    wr_copy.start()
    x_copy(0).start()
    for j in range(4, 12):
        w_copy(j).start()
    x_copy(1).start()

    def layer_norm(i, piece=0, npieces=1):
        n = T // npieces
        x = x_buf[pl.ds(pl.multiple_of(i * T + piece * n, n), n), :].astype(F32)
        m = jnp.mean(x, axis=-1, keepdims=True)
        xc = x - m
        v = jnp.mean(xc * xc, axis=-1, keepdims=True)
        den = _rb(jnp.sqrt(_rb(_rb(v) + EPS_LN)))
        rows = pl.ds(pl.multiple_of(i * (T // 2) + piece * (n // 2), n // 2), n // 2)
        xn = _pk((_rb(x - _rb(m)) * (1.0 / den)).astype(BF16))
        xn_buf[rows, :] = xn
        return xn

    def load_xn(i):
        return _upk(xn_buf[pl.ds(pl.multiple_of(i * (T // 2), T // 2), T // 2), :])

    def load_wt(r0, r1, dep=None):
        w = wt_buf[r0 // 2:r1 // 2, :]
        if dep is not None:
            w = tie(w, dep)
        return _upk(w)

    def tie(w, dep):
        acc = None
        for r in range(0, dep.shape[0], 8):
            for c in range(0, dep.shape[1], 128):
                piece = dep[r:r + 8, c:c + 128]
                acc = piece if acc is None else acc | piece
        first = w[:8, :128] | (acc & zero_buf[...])
        top = jnp.concatenate([first, w[:8, 128:]], axis=1)
        return jnp.concatenate([top, w[8:, :]], axis=0)

    def fold(j):
        for u in range(2):
            g = (2 * j + u) % 8
            w = w_buf[j, :, u * 128:(u + 1) * 128]
            if j < 8:
                r = _dot_nt(_upk(bdt_buf[g]), w) * LOG2E
            else:
                r = _dot_nt(_upk(bdt_buf[8]), w)
            wt_buf[j * 128 + u * 64:j * 128 + (u + 1) * 64, :] = _pk(r.astype(BF16))

    phi_copy.wait()
    ri = lax.broadcasted_iota(jnp.int32, (128, 128), 0)
    ci = lax.broadcasted_iota(jnp.int32, (128, 128), 1)
    same_head = (ri // 32) == (ci // 32)
    e_r = lax.broadcasted_iota(jnp.int32, (128, 32), 0)
    e_c = lax.broadcasted_iota(jnp.int32, (128, 32), 1)
    tile_eye = jnp.where((e_r % 32) == e_c, 1.0, 0.0).astype(BF16)
    for g in range(8):
        wg4 = wphi_buf[4 * g:4 * g + 4].reshape(128, 32)
        bdt_buf[g] = _pk(jnp.where(same_head, _dot_nt(tile_eye, wg4), 0.0).astype(BF16))
    bdt_buf[8] = _pk(jnp.where(ri == ci, 1.0, 0.0).astype(BF16))

    wr_copy.wait()
    wt_buf[3 * D // 2:3 * D // 2 + 8, :] = _pk(
        jnp.broadcast_to(wr_buf[...].astype(F32).reshape(1, D), (16, D)).astype(BF16))
    g_acc[...] = jnp.zeros_like(g_acc)
    zero_buf[...] = jnp.zeros_like(zero_buf)
    y_buf[...] = jnp.zeros_like(y_buf)

    x_copy(0).wait()
    layer_norm(0)
    for j in range(4, 12):
        w_copy(j).wait()
        fold(j)
    for i in range(2, NT):
        x_copy(i).start()
    for j in range(4):
        w_copy(j).start()
    wo_copy.start()

    ones = jnp.ones((16, T), BF16)

    def kv_tile(i, ln_tile=None):
        def ln(piece):
            if ln_tile is not None:
                return layer_norm(ln_tile, piece, 2 * NC)

        xn = load_xn(i)
        dep = None
        for c in range(NC):
            pk = _dot_nt(load_wt(D + c * MC, D + (c + 1) * MC, dep), xn)
            dep = ln(2 * c)
            if c == NC - 1:
                vr = _dot_nt(load_wt(2 * D + c * MC, 3 * D + 16, dep), xn)
                r_buf[i] = vr[MC:MC + 8, :]
                vt = vr[:MC, :].astype(BF16)
            else:
                vt = _dot_nt(load_wt(2 * D + c * MC, 2 * D + (c + 1) * MC, dep), xn).astype(BF16)
            dep = ln(2 * c + 1)
            for u in range(MC // 64):
                p = c * (MC // 64) + u
                phi = _phi_pair(pk[64 * u:64 * u + 64, :])
                lhs = jnp.concatenate([vt[64 * u:64 * u + 64, :], ones], axis=0)
                g_acc[p] += _dot_nt(lhs, phi)

    def pass1_body(i, carry):
        for cp in f_copies(i):
            cp.start()
        x_copy(i + 1).wait()
        kv_tile(i, i + 1)
        return carry

    lax.fori_loop(0, NT - 1, pass1_body, 0)
    for j in range(4):
        w_copy(j).wait()
    for j in range(4):
        fold(j)
    kv_tile(NT - 1)

    gr = lax.broadcasted_iota(jnp.int32, (GR, 128), 0)
    gc = lax.broadcasted_iota(jnp.int32, (GR, 128), 1)
    row_head = jnp.where(gr < 64, gr // 32, (gr - 64) // 8)
    keep = row_head == ((gc % 64) // 32)
    for p in range(NP):
        g_buf[p] = _pk(jnp.where(keep, g_acc[p], 0.0).astype(BF16))

    r_all = _rb(r_buf[...])
    tok = (lax.broadcasted_iota(jnp.int32, (NT, 8, T), 0) * T
           + lax.broadcasted_iota(jnp.int32, (NT, 8, T), 2))
    r_max = jnp.max(r_all)
    idx = jnp.min(jnp.where(r_all == r_max, tok, S - 1))
    sel_tile = idx // T
    blk = pl.multiple_of((idx // 16) * 16, 16)

    def tile_of(j):
        return (sel_tile + 1 + j) % NT

    KH = D // 2

    def q_rounds(j):
        t = tile_of(j)
        xn = load_xn(t)
        slot = j % 2
        st = {}

        def proj(c, n, h):
            def f():
                r = _dot_nt(load_wt(c * MC, (c + 1) * MC)[:, h * KH:(h + 1) * KH],
                            xn[n * 128:(n + 1) * 128, h * KH:(h + 1) * KH])
                st[c, n] = r if h == 0 else st[c, n] + r
            return f

        def num(c, n):
            def f():
                parts = []
                for u in range(MC // 64):
                    p = c * (MC // 64) + u
                    nd = _dot(_upk(g_buf[p]), _phi_pair(st[c, n][64 * u:64 * u + 64, :]))
                    for a in range(2):
                        inv = pl.reciprocal(nd[64 + 8 * a:72 + 8 * a, :] + 1e-6, approx=True)
                        parts.append(nd[32 * a:32 * a + 32, :] * jnp.concatenate([inv] * 4, axis=0))
                ot = jnp.concatenate(parts, axis=0)
                o_buf[slot, n * 64:(n + 1) * 64, c * MC:(c + 1) * MC] = _pk(ot.T.astype(BF16))
            return f

        big = [[proj(c, n, h) for n in range(T // 128) for h in range(2)] for c in range(NC)]
        small = [[num(c, n) for n in range(T // 128)] for c in range(NC)]
        return big, small

    def out_rounds(j, upd=None):
        t = tile_of(j)
        rows = pl.ds(pl.multiple_of(t * T, T), T)
        rows2 = pl.ds(pl.multiple_of(t * (T // 2), T // 2), T // 2)
        o = _upk(o_buf[j % 2])
        st = {}

        def proj(n, h):
            def f():
                cols = slice(n * 128, (n + 1) * 128)
                r = _dot(o[:, h * KH:(h + 1) * KH], wo_buf[h * KH:(h + 1) * KH, cols])
                if h == 0:
                    st[n] = r
                    return
                s = st[n] + r
                xn = _upk(xn_buf[rows2, cols]).astype(F32)
                if upd is not None:
                    xn = xn + upd[:, cols]
                out_buf[rows, cols] = (x_buf[rows, cols].astype(F32) + s * _silu(xn)).astype(BF16)
            return f

        return [proj(n, h) for n in range(D // 128) for h in range(2)]

    def ffn_rounds(c):
        xs = _upk(xn_buf[pl.ds(pl.multiple_of(blk // 2, 8), 8), :])
        st = {}

        def up(w_ref, key, n, h):
            def f():
                r = _dot(xs[:, h * KH:(h + 1) * KH], w_ref[c, h * KH:(h + 1) * KH, n * 128:(n + 1) * 128])
                st[key, n] = r if h == 0 else st[key, n] + r
            return f

        def down(n):
            def f():
                if 'h' not in st:
                    st['h'] = jnp.concatenate(
                        [_silu(st['g', m]) * st['u', m] for m in range(FC // 128)], axis=1).astype(BF16)
                y_buf[:, n * 128:(n + 1) * 128] += _dot(st['h'], wd_buf[c, :, n * 128:(n + 1) * 128])
            return f

        ups = [up(w, k, n, h) for n in range(FC // 128) for w, k in ((wg_buf, 'g'), (wu_buf, 'u')) for h in range(2)]
        return ups, [down(n) for n in range(D // 128)]

    wo_copy.wait()
    big, small = q_rounds(0)
    for c in range(NC):
        big[c][0]()
        big[c][1]()
        if c > 0:
            small[c - 1][1]()
        big[c][2]()
        big[c][3]()
        small[c][0]()
    small[NC - 1][1]()

    def pass2_body(j, carry):
        for cp in f_copies(j - 1):
            cp.wait()
        wo_r = out_rounds(j - 1)
        ups, downs = ffn_rounds(j - 1)
        big, small = q_rounds(j)
        ffn = ups + [None] * 0 + downs
        seq = []
        for c in range(NC):
            w = wo_r[4 * c:4 * c + 4]
            seq += [big[c][0], 'f', big[c][1], 'f', big[c][2], 'f', big[c][3], 'f',
                    w[0], 'f', w[1], small[c][0], w[2], small[c][1], w[3], 'f']
        for item in seq:
            if item == 'f':
                item = ffn.pop(0)
            item()
        assert not ffn
        out_copy(tile_of(j - 1)).start()
        return carry

    lax.fori_loop(1, NT, pass2_body, 0)

    sub = lax.broadcasted_iota(jnp.int32, (16, D), 0)
    y_row = jnp.sum(jnp.where(sub == idx - blk, y_buf[...], 0.0), axis=0, keepdims=True)
    gate = 1.0 / (1.0 + jnp.exp(-jnp.full((1, D), r_max, F32)))
    trow = lax.broadcasted_iota(jnp.int32, (T, D), 0)
    upd = jnp.where(trow == idx - sel_tile * T, y_row * gate, 0.0)
    for f in out_rounds(NT - 1, upd):
        f()
    out_copy(sel_tile).start()
    for i in range(NT):
        out_copy(i).wait()


@jax.jit
def pallas_recurrent_scan__linear_kernel_hedgehog__moe_arch_mod__prompt_kernel(
    A_x: jax.Array,
    A_wqkv: jax.Array,
    A_w_phi: jax.Array,
    A_wo: jax.Array,
    B_x: jax.Array,
    B_w_r: jax.Array,
    B_w_gate: jax.Array,
    B_w_up: jax.Array,
    B_w_down: jax.Array,
):
    del B_x
    any_spec = pl.BlockSpec(memory_space=pl.ANY)
    out = pl.pallas_call(
        _kernel,
        out_shape=jax.ShapeDtypeStruct((S, D), BF16),
        in_specs=[any_spec] * 8,
        out_specs=any_spec,
        scratch_shapes=[
            pltpu.VMEM((S, D), BF16),
            pltpu.VMEM((S // 2, D), U32),
            pltpu.VMEM((12, D, 256), BF16),
            pltpu.VMEM((3 * D // 2 + 8, D), U32),
            pltpu.VMEM((H, DH, DH), BF16),
            pltpu.VMEM((D,), BF16),
            pltpu.VMEM((D, D), BF16),
            pltpu.VMEM((NT - 1, D, FC), BF16),
            pltpu.VMEM((NT - 1, D, FC), BF16),
            pltpu.VMEM((NT - 1, FC, D), BF16),
            pltpu.VMEM((9, 64, 128), U32),
            pltpu.VMEM((NP, GR, 128), F32),
            pltpu.VMEM((NP, GR // 2, 128), U32),
            pltpu.VMEM((NT, 8, T), F32),
            pltpu.VMEM((2, T // 2, D), U32),
            pltpu.VMEM((16, D), F32),
            pltpu.VMEM((S, D), BF16),
            pltpu.VMEM((8, 128), U32),
            pltpu.SemaphoreType.DMA((NT,)),
            pltpu.SemaphoreType.DMA((12,)),
            pltpu.SemaphoreType.DMA((3,)),
            pltpu.SemaphoreType.DMA((3, NT - 1)),
            pltpu.SemaphoreType.DMA((NT,)),
        ],
        compiler_params=pltpu.CompilerParams(vmem_limit_bytes=100 * 1024 * 1024),
        name="hedgehog_mod",
    )(A_x.reshape(S, D), A_wqkv, A_w_phi, A_wo, B_w_r, B_w_gate, B_w_up, B_w_down)
    return out.reshape(1, S, D)
```

```python
import jax
import jax.numpy as jnp
from jax import lax
import jax.experimental.pallas as pl
import jax.experimental.pallas.tpu as pltpu

S, D, H, DH, F = 2048, 1024, 32, 32, 3584
T = 256
NT = S // T
MC = 256
NC = D // MC
PC = MC // 64
NP = H // 2
GR = 80
FC = 512
NF = F // FC
LOG2E = 1.4426950408889634
EPS_LN = 1.0013580322265625e-05
F32 = jnp.float32
BF16 = jnp.bfloat16
U32 = jnp.uint32

_NT_DIMS = (((1,), (1,)), ((), ()))


def _dot_nt(a, b):
    return lax.dot_general(a, b, _NT_DIMS, preferred_element_type=F32)


def _dot(a, b):
    return jnp.dot(a, b, preferred_element_type=F32)


def _rb(x):
    return x.astype(BF16).astype(F32)


def _pk(x):
    return pltpu.bitcast(x, U32)


def _upk(x):
    return pltpu.bitcast(x, BF16)


def _phi_pair(p):
    pos, neg = [], []
    for a in range(2):
        ph = p[32 * a:32 * a + 32, :]
        mx = jnp.max(ph, axis=0, keepdims=True)
        mn = jnp.min(ph, axis=0, keepdims=True)
        ep = jnp.exp2(ph - mx)
        en = jnp.exp2(mn - ph)
        pos.append(ep * pl.reciprocal(jnp.sum(ep, axis=0, keepdims=True), approx=True))
        neg.append(en * pl.reciprocal(jnp.sum(en, axis=0, keepdims=True), approx=True))
    return jnp.concatenate(pos + neg, axis=0).astype(BF16)


def _silu(x):
    h = 0.5 * x
    return h + h * jnp.tanh(h)


def _kernel(x_hbm, wqkv_hbm, wphi_hbm, wo_hbm, wr_hbm, wg_hbm, wu_hbm, wd_hbm, out_hbm,
            x_buf, xn_buf, w_buf, wt_buf, wphi_buf, wr_buf, wo_buf, wg_buf, wu_buf, wd_buf,
            bdt_buf, g_acc, g_buf, r_buf, o_buf, out_buf, zero_buf,
            sem_x, sem_w, sem_s, sem_o):
    x_cp = [pltpu.make_async_copy(x_hbm.at[pl.ds(i * T, T), :], x_buf.at[pl.ds(i * T, T), :], sem_x.at[i])
            for i in range(NT)]
    w_cp = [pltpu.make_async_copy(wqkv_hbm.at[:, pl.ds(j * MC, MC)], w_buf.at[j], sem_w.at[j])
            for j in range(3 * NC)]
    q_cp, k_cp, v_cp = w_cp[:NC], w_cp[NC:2 * NC], w_cp[2 * NC:]
    phi_cp = pltpu.make_async_copy(wphi_hbm, wphi_buf, sem_s.at[0])
    wr_cp = pltpu.make_async_copy(wr_hbm, wr_buf, sem_s.at[1])
    wo_cp = pltpu.make_async_copy(wo_hbm, wo_buf, sem_s.at[2])
    f_cp = [pltpu.make_async_copy(wg_hbm, wg_buf, sem_s.at[3]),
            pltpu.make_async_copy(wu_hbm, wu_buf, sem_s.at[4]),
            pltpu.make_async_copy(wd_hbm, wd_buf, sem_s.at[5])]

    def out_copy(t, j):
        rows = pl.ds(pl.multiple_of(t * T, T), T)
        return pltpu.make_async_copy(out_buf.at[rows, :], out_hbm.at[rows, :], sem_o.at[j])

    def start_in_order(copies):
        def body(j, carry):
            for k, cp in enumerate(copies):
                pl.when(j == k)(cp.start)
            zero_buf[...] = jnp.zeros_like(zero_buf)
            return carry
        lax.fori_loop(0, len(copies), body, 0)

    start_in_order([x_cp[0], v_cp[0], wr_cp, v_cp[1], phi_cp, k_cp[0], k_cp[1], v_cp[2], k_cp[2],
                    v_cp[3], k_cp[3]] + x_cp[1:] + q_cp + [wo_cp] + f_cp)

    def tie(w, dep):
        acc = None
        for r in range(0, dep.shape[0], 8):
            for c in range(0, dep.shape[1], 128):
                piece = dep[r:r + 8, c:c + 128]
                acc = piece if acc is None else acc | piece
        first = w[:8, :128] | (acc & zero_buf[...])
        top = jnp.concatenate([first, w[:8, 128:]], axis=1)
        return jnp.concatenate([top, w[8:, :]], axis=0)

    def layer_norm(i, piece=0, npieces=1):
        n = T // npieces
        r0 = i * T + piece * n
        x = x_buf[r0:r0 + n, :].astype(F32)
        m = jnp.mean(x, axis=-1, keepdims=True)
        xc = x - m
        v = jnp.mean(xc * xc, axis=-1, keepdims=True)
        den = _rb(jnp.sqrt(_rb(_rb(v) + EPS_LN)))
        xn = _pk((_rb(x - _rb(m)) * (1.0 / den)).astype(BF16))
        xn_buf[r0 // 2:(r0 + n) // 2, :] = xn
        return xn

    def load_wt(r0, r1, dep=None):
        w = wt_buf[r0 // 2:r1 // 2, :]
        if dep is not None:
            w = tie(w, dep)
        return _upk(w)

    def fold(j, u):
        w = w_buf[j, :, u * 128:(u + 1) * 128]
        if j < 2 * NC:
            r = _dot_nt(_upk(bdt_buf[(2 * j + u) % 8]), w) * LOG2E
        else:
            r = _dot_nt(_upk(bdt_buf[8]), w)
        wt_buf[j * 128 + u * 64:j * 128 + (u + 1) * 64, :] = _pk(r.astype(BF16))

    def fold2(j):
        fold(j, 0)
        fold(j, 1)

    ri = lax.broadcasted_iota(jnp.int32, (128, 128), 0)
    ci = lax.broadcasted_iota(jnp.int32, (128, 128), 1)

    def build_bdt():
        same_head = (ri // 32) == (ci // 32)
        e_r = lax.broadcasted_iota(jnp.int32, (128, 32), 0)
        e_c = lax.broadcasted_iota(jnp.int32, (128, 32), 1)
        tile_eye = jnp.where((e_r % 32) == e_c, 1.0, 0.0).astype(BF16)
        for g in range(8):
            wg4 = wphi_buf[4 * g:4 * g + 4].reshape(128, 32)
            bdt_buf[g] = _pk(jnp.where(same_head, _dot_nt(tile_eye, wg4), 0.0).astype(BF16))

    ones = jnp.ones((16, T), BF16)

    class KV:
        def __init__(self, i, ln_tile=None):
            self.i, self.ln_tile, self.piece, self.dep = i, ln_tile, 0, None
            self.pk, self.vt = {}, {}

        def xn(self):
            return _upk(xn_buf[self.i * T // 2:(self.i + 1) * T // 2, :])

        def ln(self, count=1):
            if self.ln_tile is None:
                return
            deps = [layer_norm(self.ln_tile, self.piece + e, 2 * NC) for e in range(count)]
            self.piece += count
            self.dep = jnp.concatenate(deps, axis=0)

        def take(self):
            dep, self.dep = self.dep, None
            return dep

        def k(self, c, dep=None):
            self.pk[c] = _dot_nt(load_wt(D + c * MC, D + (c + 1) * MC, dep), self.xn())

        def v(self, c, dep=None):
            if c == NC - 1:
                vr = _dot_nt(load_wt(2 * D + c * MC, 3 * D + 16, dep), self.xn())
                r_buf[self.i] = vr[MC:MC + 8, :]
                self.vt[c] = vr[:MC, :].astype(BF16)
            else:
                self.vt[c] = _dot_nt(load_wt(2 * D + c * MC, 2 * D + (c + 1) * MC, dep), self.xn()).astype(BF16)

        def g(self, c):
            pk, vt = self.pk.pop(c), self.vt.pop(c)
            for u in range(PC):
                phi = _phi_pair(pk[64 * u:64 * u + 64, :])
                lhs = jnp.concatenate([vt[64 * u:64 * u + 64, :], ones], axis=0)
                r = _dot_nt(lhs, phi)
                if self.i == 0:
                    g_acc[c * PC + u] = r
                else:
                    g_acc[c * PC + u] += r

    bdt_buf[8] = _pk(jnp.where(ri == ci, 1.0, 0.0).astype(BF16))
    x_cp[0].wait()
    layer_norm(0)
    t0 = KV(0, 1)
    v_cp[0].wait()
    fold2(2 * NC)
    t0.v(0)
    wr_cp.wait()
    v_cp[1].wait()
    phi_cp.wait()
    wt_buf[3 * D // 2:3 * D // 2 + 8, :] = _pk(
        jnp.broadcast_to(wr_buf[...].astype(F32).reshape(1, D), (16, D)).astype(BF16))
    fold2(2 * NC + 1)
    build_bdt()
    t0.v(1)
    k_cp[0].wait()
    k_cp[1].wait()
    fold2(NC)
    fold2(NC + 1)
    t0.k(0)
    t0.k(1)
    t0.g(0)
    v_cp[2].wait()
    k_cp[2].wait()
    fold2(NC + 2)
    fold2(2 * NC + 2)
    t0.g(1)
    t0.k(2)
    t0.v(2)
    v_cp[3].wait()
    k_cp[3].wait()
    x_cp[1].wait()
    x_cp[2].wait()
    fold2(NC + 3)
    fold2(2 * NC + 3)
    t0.g(2)
    t0.ln(3)
    t0.k(3, t0.take())
    t0.ln(3)
    t0.v(3, t0.take())
    t0.ln(2)
    prev = t0

    for i in range(1, NT):
        if i == 2:
            for cp in x_cp[3:] + q_cp:
                cp.wait()
        kv = KV(i, i + 1 if i + 1 < NT else None)
        for c in range(NC):
            kv.k(c, prev.take() if c == 0 else kv.take())
            kv.ln()
            if c == 0:
                prev.g(NC - 1)
            else:
                kv.g(c - 1)
            kv.v(c, kv.take())
            kv.ln()
        if 2 <= i < 2 + NC:
            fold2(i - 2)
        prev = kv
    prev.g(NC - 1)

    gr = lax.broadcasted_iota(jnp.int32, (GR, 128), 0)
    gc = lax.broadcasted_iota(jnp.int32, (GR, 128), 1)
    row_head = jnp.where(gr < 64, gr // 32, (gr - 64) // 8)
    keep = row_head == ((gc % 64) // 32)
    for p in range(NP):
        g_buf[p] = _pk(jnp.where(keep, g_acc[p], 0.0).astype(BF16))

    r_all = _rb(r_buf[...])
    tok = (lax.broadcasted_iota(jnp.int32, (NT, 8, T), 0) * T
           + lax.broadcasted_iota(jnp.int32, (NT, 8, T), 2))
    r_max = jnp.max(r_all)
    idx = jnp.min(jnp.where(r_all == r_max, tok, S - 1))
    sel_tile = idx // T
    blk = pl.multiple_of((idx // 16) * 16, 16)

    def tile_of(j):
        return (sel_tile + 1 + j) % NT

    class Q:
        def __init__(self, j):
            self.j = j
            self.row0 = tile_of(j) * (T // 2)
            self.pq = {}

        def proj(self, c, n):
            xn = _upk(xn_buf[pl.ds(pl.multiple_of(self.row0 + n * 64, 64), 64), :])
            self.pq[c, n] = _dot_nt(load_wt(c * MC, (c + 1) * MC), xn)

        def num(self, c, n):
            pq = self.pq.pop((c, n))
            parts = []
            for u in range(PC):
                nd = _dot(_upk(g_buf[c * PC + u]), _phi_pair(pq[64 * u:64 * u + 64, :]))
                for a in range(2):
                    inv = pl.reciprocal(nd[64 + 8 * a:72 + 8 * a, :] + 1e-6, approx=True)
                    parts.append(nd[32 * a:32 * a + 32, :] * jnp.concatenate([inv] * 4, axis=0))
            ot = jnp.concatenate(parts, axis=0)
            o_buf[self.j % 2, n * 64:(n + 1) * 64, c * MC:(c + 1) * MC] = _pk(ot.T.astype(BF16))

    def out_cols(j, n, upd=None):
        t = tile_of(j)
        rows = pl.ds(pl.multiple_of(t * T, T), T)
        rows2 = pl.ds(pl.multiple_of(t * (T // 2), T // 2), T // 2)
        cols = slice(n * 128, (n + 1) * 128)
        s = _dot(_upk(o_buf[j % 2]), wo_buf[:, cols])
        xn = _upk(xn_buf[rows2, cols]).astype(F32)
        if upd is not None:
            xn = xn + upd[:, cols]
        out_buf[rows, cols] = (x_buf[rows, cols].astype(F32) + s * _silu(xn)).astype(BF16)

    def ffn_steps():
        st = {}

        def up(w_ref, key, n):
            def f():
                xs = _upk(xn_buf[pl.ds(pl.multiple_of(blk // 2, 8), 8), :])
                st[key, n] = _dot(xs, w_ref[:, n * 128:(n + 1) * 128])
            return f

        def down(c, n):
            def f():
                if ('h', c) not in st:
                    ms = range(c * FC // 128, (c + 1) * FC // 128)
                    st['h', c] = jnp.concatenate(
                        [_silu(st.pop(('g', m))) * st.pop(('u', m)) for m in ms], axis=1).astype(BF16)
                r = _dot(st['h', c], wd_buf[c * FC:(c + 1) * FC, n * 256:(n + 1) * 256])
                st['y', n] = r if c == 0 else st['y', n] + r
            return f

        steps = []
        for c in range(NF):
            for m in range(c * FC // 128, (c + 1) * FC // 128):
                steps += [up(wg_buf, 'g', m), up(wu_buf, 'u', m)]
            steps += [down(c, n) for n in range(D // 256)]
        return steps, st

    q = Q(0)
    for c in range(NC):
        q.proj(c, 0)
        if c > 0:
            q.num(c - 1, 1)
        q.proj(c, 1)
        q.num(c, 0)
    wo_cp.wait()
    for cp in f_cp:
        cp.wait()
    ffn, ffn_st = ffn_steps()
    for j in range(1, NT):
        qn = Q(j)
        for c in range(NC):
            qn.proj(c, 0)
            if c == 0:
                q.num(NC - 1, 1)
            qn.proj(c, 1)
            ffn.pop(0)()
            out_cols(j - 1, 2 * c)
            ffn.pop(0)()
            qn.num(c, 0)
            out_cols(j - 1, 2 * c + 1)
            ffn.pop(0)()
            if c < NC - 1:
                qn.num(c, 1)
        out_copy(tile_of(j - 1), j - 1).start()
        q = qn
    assert not ffn
    q.num(NC - 1, 1)

    y = jnp.concatenate([ffn_st['y', n] for n in range(D // 256)], axis=1)
    sub = lax.broadcasted_iota(jnp.int32, (16, D), 0)
    y_row = jnp.sum(jnp.where(sub == idx - blk, y, 0.0), axis=0, keepdims=True)
    gate = 1.0 / (1.0 + jnp.exp(-jnp.full((1, D), r_max, F32)))
    trow = lax.broadcasted_iota(jnp.int32, (T, D), 0)
    upd = jnp.where(trow == idx - sel_tile * T, y_row * gate, 0.0)
    for n in range(D // 128):
        out_cols(NT - 1, n, upd)
    out_copy(sel_tile, NT - 1).start()
    for j in range(NT):
        out_copy(tile_of(j), j).wait()


@jax.jit
def pallas_recurrent_scan__linear_kernel_hedgehog__moe_arch_mod__prompt_kernel(
    A_x: jax.Array,
    A_wqkv: jax.Array,
    A_w_phi: jax.Array,
    A_wo: jax.Array,
    B_x: jax.Array,
    B_w_r: jax.Array,
    B_w_gate: jax.Array,
    B_w_up: jax.Array,
    B_w_down: jax.Array,
):
    del B_x
    any_spec = pl.BlockSpec(memory_space=pl.ANY)
    out = pl.pallas_call(
        _kernel,
        out_shape=jax.ShapeDtypeStruct((S, D), BF16),
        in_specs=[any_spec] * 8,
        out_specs=any_spec,
        scratch_shapes=[
            pltpu.VMEM((S, D), BF16),
            pltpu.VMEM((S // 2, D), U32),
            pltpu.VMEM((3 * NC, D, MC), BF16),
            pltpu.VMEM((3 * D // 2 + 8, D), U32),
            pltpu.VMEM((H, DH, DH), BF16),
            pltpu.VMEM((D,), BF16),
            pltpu.VMEM((D, D), BF16),
            pltpu.VMEM((D, F), BF16),
            pltpu.VMEM((D, F), BF16),
            pltpu.VMEM((F, D), BF16),
            pltpu.VMEM((9, 64, 128), U32),
            pltpu.VMEM((NP, GR, 128), F32),
            pltpu.VMEM((NP, GR // 2, 128), U32),
            pltpu.VMEM((NT, 8, T), F32),
            pltpu.VMEM((2, T // 2, D), U32),
            pltpu.VMEM((S, D), BF16),
            pltpu.VMEM((8, 128), U32),
            pltpu.SemaphoreType.DMA((NT,)),
            pltpu.SemaphoreType.DMA((3 * NC,)),
            pltpu.SemaphoreType.DMA((6,)),
            pltpu.SemaphoreType.DMA((NT,)),
        ],
        compiler_params=pltpu.CompilerParams(
            vmem_limit_bytes=100 * 1024 * 1024,
            disable_bounds_checks=True,
            disable_semaphore_checks=True,
        ),
        name="hedgehog_mod",
    )(A_x.reshape(S, D), A_wqkv, A_w_phi, A_wo, B_w_r, B_w_gate, B_w_up, B_w_down)
    return out.reshape(1, S, D)
```

```python
import jax
import jax.numpy as jnp
from jax import lax
import jax.experimental.pallas as pl
import jax.experimental.pallas.tpu as pltpu

S, D, H, DH, F = 2048, 1024, 32, 32, 3584
T = 256
NT = S // T
MC = 256
NC = D // MC
PC = MC // 64
NP = H // 2
GR = 80
FC = 512
LNP = 16
KROW = D + 16
VROW = KROW + D
LOG2E = 1.4426950408889634
EPS_LN = 1.0013580322265625e-05
F32 = jnp.float32
BF16 = jnp.bfloat16
U32 = jnp.uint32

_NT_DIMS = (((1,), (1,)), ((), ()))


def _dot_nt(a, b):
    return lax.dot_general(a, b, _NT_DIMS, preferred_element_type=F32)


def _dot(a, b):
    return jnp.dot(a, b, preferred_element_type=F32)


def _rb(x):
    return x.astype(BF16).astype(F32)


def _pk(x):
    return pltpu.bitcast(x, U32)


def _upk(x):
    return pltpu.bitcast(x, BF16)


def _phi_pair(p, link=None):
    pos, neg = [], []
    for a in range(2):
        ph = p[32 * a:32 * a + 32, :]
        mx = jnp.max(ph, axis=0, keepdims=True)
        mn = jnp.min(ph, axis=0, keepdims=True)
        if link is not None:
            mx, mn = link.start(mx, mn)
        ep = jnp.exp2(ph - mx)
        en = jnp.exp2(mn - ph)
        pos.append(ep * pl.reciprocal(jnp.sum(ep, axis=0, keepdims=True), approx=True))
        neg.append(en * pl.reciprocal(jnp.sum(en, axis=0, keepdims=True), approx=True))
        if link is not None:
            link.done(pos[-1], neg[-1])
    return jnp.concatenate(pos + neg, axis=0).astype(BF16)


def _silu(x):
    h = 0.5 * x
    return h + h * jnp.tanh(h)


def _kernel(x_hbm, wqkv_hbm, wphi_hbm, wo_hbm, wr_hbm, wg_hbm, wu_hbm, wd_hbm, out_hbm,
            x_buf, xn_buf, w_buf, wt_buf, wphi_buf, wr_buf, wo_buf, wg_buf, wu_buf, wd_buf,
            bdt_buf, g_acc, g_buf, r_buf, o_buf, out_buf, zero_buf, wop_buf,
            sem_x, sem_w, sem_s, sem_o):
    x_cp = [pltpu.make_async_copy(x_hbm.at[pl.ds(i * T, T), :], x_buf.at[pl.ds(i * T, T), :], sem_x.at[i])
            for i in range(NT)]
    w_cp = [pltpu.make_async_copy(wqkv_hbm.at[:, pl.ds(j * MC, MC)], w_buf.at[j], sem_w.at[j])
            for j in range(3 * NC)]
    q_cp, k_cp, v_cp = w_cp[:NC], w_cp[NC:2 * NC], w_cp[2 * NC:]
    phi_cp = pltpu.make_async_copy(wphi_hbm, wphi_buf, sem_s.at[0])
    wr_cp = pltpu.make_async_copy(wr_hbm, wr_buf, sem_s.at[1])
    wo_cp = pltpu.make_async_copy(wo_hbm, wo_buf, sem_s.at[2])
    f_cp = [pltpu.make_async_copy(wg_hbm, wg_buf, sem_s.at[3]),
            pltpu.make_async_copy(wu_hbm, wu_buf, sem_s.at[4]),
            pltpu.make_async_copy(wd_hbm, wd_buf, sem_s.at[5])]

    def out_copy(t, j):
        rows = pl.ds(pl.multiple_of(t * T, T), T)
        return pltpu.make_async_copy(out_buf.at[rows, :], out_hbm.at[rows, :], sem_o.at[j])

    def start_in_order(copies):
        def body(j, carry):
            for k, cp in enumerate(copies):
                pl.when(j == k)(cp.start)
            zero_buf[...] = jnp.zeros_like(zero_buf)
            return carry
        lax.fori_loop(0, len(copies), body, 0)

    start_in_order([x_cp[0], v_cp[0], wr_cp, v_cp[1], phi_cp, k_cp[0], k_cp[1], v_cp[2], k_cp[2],
                    v_cp[3], k_cp[3]])
    start_in_order(x_cp[1:] + q_cp)
    start_in_order([wo_cp] + f_cp)

    def tie(w, dep):
        acc = None
        for r in range(0, dep.shape[0], 8):
            for c in range(0, dep.shape[1], 128):
                piece = dep[r:r + 8, c:c + 128]
                acc = piece if acc is None else acc | piece
        first = w[:8, :128] | (acc & zero_buf[...])
        top = jnp.concatenate([first, w[:8, 128:]], axis=1)
        return jnp.concatenate([top, w[8:, :]], axis=0)

    def after(x, dep):
        z = pltpu.bitcast(dep, U32)[:x.shape[0], :] & zero_buf[:x.shape[0], :]
        return pltpu.bitcast(pltpu.bitcast(x, U32) | z, F32)

    class Link:
        def __init__(self):
            self.prev = None

        def start(self, mx, mn):
            if self.prev is None:
                return mx, mn
            return after(mx, self.prev[0]), after(mn, self.prev[1])

        def done(self, pos, neg):
            self.prev = (pos[24:32, :], neg[24:32, :])

    def layer_norm(i, piece=0, npieces=1):
        n = T // npieces
        r0 = i * T + piece * n
        x = x_buf[r0:r0 + n, :].astype(F32)
        m = jnp.mean(x, axis=-1, keepdims=True)
        xc = x - m
        v = jnp.mean(xc * xc, axis=-1, keepdims=True)
        den = _rb(jnp.sqrt(_rb(_rb(v) + EPS_LN)))
        xn = _pk((_rb(x - _rb(m)) * (1.0 / den)).astype(BF16))
        xn_buf[r0 // 2:(r0 + n) // 2, :] = xn
        return xn

    def load_wt(r0, r1, dep=None):
        w = wt_buf[r0 // 2:r1 // 2, :]
        if dep is not None:
            w = tie(w, dep)
        return _upk(w)

    def fold(j, u):
        w = w_buf[j, :, u * 128:(u + 1) * 128]
        if j < 2 * NC:
            r = _dot_nt(_upk(bdt_buf[(2 * j + u) % 8]), w) * LOG2E
        else:
            r = _dot_nt(_upk(bdt_buf[8]), w)
        row = (j * MC + u * 128 + (16 if j >= NC else 0)) // 2
        wt_buf[row:row + 64, :] = _pk(r.astype(BF16))

    def fold2(j):
        fold(j, 0)
        fold(j, 1)

    ri = lax.broadcasted_iota(jnp.int32, (128, 128), 0)
    ci = lax.broadcasted_iota(jnp.int32, (128, 128), 1)

    def build_bdt():
        same_head = (ri // 32) == (ci // 32)
        e_r = lax.broadcasted_iota(jnp.int32, (128, 32), 0)
        e_c = lax.broadcasted_iota(jnp.int32, (128, 32), 1)
        tile_eye = jnp.where((e_r % 32) == e_c, 1.0, 0.0).astype(BF16)
        for g in range(8):
            wg4 = wphi_buf[4 * g:4 * g + 4].reshape(128, 32)
            bdt_buf[g] = _pk(jnp.where(same_head, _dot_nt(tile_eye, wg4), 0.0).astype(BF16))

    ones = jnp.ones((16, T), BF16)

    class KV:
        def __init__(self, i, ln_tile=None):
            self.i, self.ln_tile, self.piece, self.dep = i, ln_tile, 0, None
            self.pk, self.vt = {}, {}

        def ln(self, count=1):
            if self.ln_tile is None or count == 0:
                return
            deps = [layer_norm(self.ln_tile, self.piece + e, LNP) for e in range(count)]
            self.piece += count
            self.dep = jnp.concatenate(deps, axis=0)

        def take(self):
            dep, self.dep = self.dep, None
            return dep

        def proj(self, r0, r1, dep, count):
            halves = []
            for n in range(2):
                row = (self.i * T + n * 128) // 2
                halves.append(_dot_nt(load_wt(r0, r1, dep), _upk(xn_buf[row:row + 64, :])))
                self.ln(count)
                if n == 0:
                    dep = self.take()
            return jnp.concatenate(halves, axis=1)

        def k(self, c, dep=None, count=0):
            if c == 0:
                kr = self.proj(KROW - 16, KROW + MC, dep, count)
                r_buf[self.i] = kr[:8, :]
                self.pk[c] = kr[16:, :]
            else:
                self.pk[c] = self.proj(KROW + c * MC, KROW + (c + 1) * MC, dep, count)

        def v(self, c, dep=None, count=0):
            self.vt[c] = self.proj(VROW + c * MC, VROW + (c + 1) * MC, dep, count).astype(BF16)

        def g(self, c):
            pk, vt = self.pk.pop(c), self.vt.pop(c)
            for u in range(PC):
                phi = _phi_pair(pk[64 * u:64 * u + 64, :])
                lhs = jnp.concatenate([vt[64 * u:64 * u + 64, :], ones], axis=0)
                r = _dot_nt(lhs, phi)
                if self.i == 0:
                    g_acc[c * PC + u] = r
                else:
                    g_acc[c * PC + u] += r

    bdt_buf[8] = _pk(jnp.where(ri == ci, 1.0, 0.0).astype(BF16))
    x_cp[0].wait()
    layer_norm(0)
    t0 = KV(0, 1)
    v_cp[0].wait()
    fold2(2 * NC)
    t0.v(0)
    wr_cp.wait()
    v_cp[1].wait()
    phi_cp.wait()
    wt_buf[D // 2:D // 2 + 8, :] = _pk(
        jnp.broadcast_to(wr_buf[...].astype(F32).reshape(1, D), (16, D)).astype(BF16))
    fold2(2 * NC + 1)
    build_bdt()
    t0.v(1)
    k_cp[0].wait()
    k_cp[1].wait()
    fold2(NC)
    fold2(NC + 1)
    t0.k(0)
    t0.k(1)
    t0.g(0)
    v_cp[2].wait()
    k_cp[2].wait()
    fold2(NC + 2)
    fold2(2 * NC + 2)
    t0.g(1)
    t0.k(2)
    t0.v(2)
    v_cp[3].wait()
    k_cp[3].wait()
    x_cp[1].wait()
    x_cp[2].wait()
    fold2(NC + 3)
    fold2(2 * NC + 3)
    t0.g(2)
    t0.ln(4)
    t0.k(3, t0.take(), 3)
    t0.v(3, t0.take(), 3)
    prev = t0

    for i in range(1, NT):
        if i == 2:
            for cp in x_cp[3:] + q_cp:
                cp.wait()
        kv = KV(i, i + 1 if i + 1 < NT else None)
        for c in range(NC):
            kv.k(c, prev.take() if c == 0 else kv.take(), 1)
            if c == 0:
                prev.g(NC - 1)
            else:
                kv.g(c - 1)
            kv.v(c, kv.take(), 1)
        if 2 <= i < 2 + NC:
            fold2(i - 2)
        prev = kv
    prev.g(NC - 1)

    gr = lax.broadcasted_iota(jnp.int32, (GR, 128), 0)
    gc = lax.broadcasted_iota(jnp.int32, (GR, 128), 1)
    row_head = jnp.where(gr < 64, gr // 32, (gr - 64) // 8)
    keep = row_head == ((gc % 64) // 32)
    for p in range(NP):
        g_buf[p] = _pk(jnp.where(keep, g_acc[p], 0.0).astype(BF16))

    r_all = _rb(r_buf[...])
    tok = (lax.broadcasted_iota(jnp.int32, (NT, 8, T), 0) * T
           + lax.broadcasted_iota(jnp.int32, (NT, 8, T), 2))
    r_max = jnp.max(r_all)
    idx = jnp.min(jnp.where(r_all == r_max, tok, S - 1))
    sel_tile = idx // T
    blk = pl.multiple_of((idx // 16) * 16, 16)

    def tile_of(j):
        return (sel_tile + 1 + j) % NT

    def last_copy(n):
        rows = pl.ds(pl.multiple_of(sel_tile * T, T), T)
        cols = pl.ds(n * 256, 256)
        return pltpu.make_async_copy(out_buf.at[rows, cols], out_hbm.at[rows, cols], sem_o.at[NT - 1 + n])

    class Q:
        def __init__(self, j):
            self.j = j
            self.row0 = tile_of(j) * (T // 2)
            self.pq = {}

        def proj(self, c, n, dep=None):
            xn = _upk(xn_buf[pl.ds(pl.multiple_of(self.row0 + n * 64, 64), 64), :])
            self.pq[c, n] = _dot_nt(load_wt(c * MC, (c + 1) * MC, dep), xn)

        def num(self, c, n):
            pq = self.pq.pop((c, n))
            parts = []
            link = Link()
            for u in range(PC):
                nd = _dot(_upk(g_buf[c * PC + u]), _phi_pair(pq[64 * u:64 * u + 64, :], link))
                for a in range(2):
                    inv = pl.reciprocal(nd[64 + 8 * a:72 + 8 * a, :] + 1e-6, approx=True)
                    parts.append(nd[32 * a:32 * a + 32, :] * jnp.concatenate([inv] * 4, axis=0))
            ot = jnp.concatenate(parts, axis=0)
            o_buf[self.j % 2, n * 64:(n + 1) * 64, c * MC:(c + 1) * MC] = _pk(ot.T.astype(BF16))

    def out_cols(j, n, dep=None, upd=None):
        t = tile_of(j)
        rows = pl.ds(pl.multiple_of(t * T, T), T)
        rows2 = pl.ds(pl.multiple_of(t * (T // 2), T // 2), T // 2)
        cols = slice(n * 128, (n + 1) * 128)
        o = o_buf[j % 2]
        if dep is not None:
            o = tie(o, dep)
        s = _dot(_upk(o), _upk(wop_buf[:, cols]))
        xn = _upk(xn_buf[rows2, cols]).astype(F32)
        if upd is not None:
            xn = xn + upd[:, cols]
        out_buf[rows, cols] = (x_buf[rows, cols].astype(F32) + s * _silu(xn)).astype(BF16)

    def ffn_steps():
        st = {}

        def up(w_ref, key, n):
            def f():
                xs = _upk(xn_buf[pl.ds(pl.multiple_of(blk // 2, 8), 8), :])
                st[key, n] = _dot(xs, w_ref[:, n * 128:(n + 1) * 128])
            return f

        def down(c, n):
            def f():
                if ('h', c) not in st:
                    ms = range(c * FC // 128, (c + 1) * FC // 128)
                    st['h', c] = jnp.concatenate(
                        [_silu(st.pop(('g', m))) * st.pop(('u', m)) for m in ms], axis=1).astype(BF16)
                r = _dot(st['h', c], wd_buf[c * FC:(c + 1) * FC, n * 256:(n + 1) * 256])
                st['y', n] = r if c == 0 else st['y', n] + r
            return f

        steps = []
        for c in range(F // FC):
            for m in range(c * FC // 128, (c + 1) * FC // 128):
                steps += [up(wg_buf, 'g', m), up(wu_buf, 'u', m)]
            steps += [down(c, n) for n in range(D // 256)]
        return steps, st

    wo_cp.wait()
    for cp in f_cp:
        cp.wait()
    wop_buf[...] = _pk(wo_buf[...])
    ffn, ffn_st = ffn_steps()

    q = Q(0)
    for c in range(NC):
        q.proj(c, 0)
        if c > 0:
            q.num(c - 1, 1)
        q.proj(c, 1)
        q.num(c, 0)
    for j in range(1, NT):
        qn = Q(j)
        for c in range(NC):
            qn.proj(c, 0)
            if c == 0:
                q.num(NC - 1, 1)
            qn.proj(c, 1)
            ffn.pop(0)()
            out_cols(j - 1, 2 * c)
            ffn.pop(0)()
            qn.num(c, 0)
            out_cols(j - 1, 2 * c + 1)
            ffn.pop(0)()
            if c < NC - 1:
                qn.num(c, 1)
        out_copy(tile_of(j - 1), j - 1).start()
        q = qn
    q.num(NC - 1, 1)

    y = jnp.concatenate([ffn_st['y', n] for n in range(D // 256)], axis=1)
    sub = lax.broadcasted_iota(jnp.int32, (16, D), 0)
    y_row = jnp.sum(jnp.where(sub == idx - blk, y, 0.0), axis=0, keepdims=True)
    gate = 1.0 / (1.0 + jnp.exp(-jnp.full((1, D), r_max, F32)))
    trow = lax.broadcasted_iota(jnp.int32, (T, D), 0)
    upd = jnp.where(trow == idx - sel_tile * T, y_row * gate, 0.0)
    for n in range(D // 128):
        out_cols(NT - 1, n, None, upd)
        if n % 2 == 1:
            last_copy(n // 2).start()
    for j in range(NT - 1):
        out_copy(tile_of(j), j).wait()
    for n in range(D // 256):
        last_copy(n).wait()


@jax.jit
def pallas_recurrent_scan__linear_kernel_hedgehog__moe_arch_mod__prompt_kernel(
    A_x: jax.Array,
    A_wqkv: jax.Array,
    A_w_phi: jax.Array,
    A_wo: jax.Array,
    B_x: jax.Array,
    B_w_r: jax.Array,
    B_w_gate: jax.Array,
    B_w_up: jax.Array,
    B_w_down: jax.Array,
):
    del B_x
    any_spec = pl.BlockSpec(memory_space=pl.ANY)
    out = pl.pallas_call(
        _kernel,
        out_shape=jax.ShapeDtypeStruct((S, D), BF16),
        in_specs=[any_spec] * 8,
        out_specs=any_spec,
        scratch_shapes=[
            pltpu.VMEM((S, D), BF16),
            pltpu.VMEM((S // 2, D), U32),
            pltpu.VMEM((3 * NC, D, MC), BF16),
            pltpu.VMEM((3 * D // 2 + 8, D), U32),
            pltpu.VMEM((H, DH, DH), BF16),
            pltpu.VMEM((D,), BF16),
            pltpu.VMEM((D, D), BF16),
            pltpu.VMEM((D, F), BF16),
            pltpu.VMEM((D, F), BF16),
            pltpu.VMEM((F, D), BF16),
            pltpu.VMEM((9, 64, 128), U32),
            pltpu.VMEM((NP, GR, 128), F32),
            pltpu.VMEM((NP, GR // 2, 128), U32),
            pltpu.VMEM((NT, 8, T), F32),
            pltpu.VMEM((2, T // 2, D), U32),
            pltpu.VMEM((S, D), BF16),
            pltpu.VMEM((8, 128), U32),
            pltpu.VMEM((D // 2, D), U32),
            pltpu.SemaphoreType.DMA((NT,)),
            pltpu.SemaphoreType.DMA((3 * NC,)),
            pltpu.SemaphoreType.DMA((6,)),
            pltpu.SemaphoreType.DMA((NT + 3,)),
        ],
        compiler_params=pltpu.CompilerParams(
            vmem_limit_bytes=100 * 1024 * 1024,
            disable_bounds_checks=True,
            disable_semaphore_checks=True,
        ),
        name="hedgehog_mod",
    )(A_x.reshape(S, D), A_wqkv, A_w_phi, A_wo, B_w_r, B_w_gate, B_w_up, B_w_down)
    return out.reshape(1, S, D)
```

```python
import jax
import jax.numpy as jnp
from jax import lax
import jax.experimental.pallas as pl
import jax.experimental.pallas.tpu as pltpu

S, D, H, DH, F = 2048, 1024, 32, 32, 3584
T = 256
NT = S // T
MC = 256
NC = D // MC
PC = MC // 64
NP = H // 2
GR = 80
FC = 512
LNP = 16
KROW = D + 16
VROW = KROW + D
LOG2E = 1.4426950408889634
EPS_LN = 1.0013580322265625e-05
F32 = jnp.float32
BF16 = jnp.bfloat16
U32 = jnp.uint32

_NT_DIMS = (((1,), (1,)), ((), ()))


def _dot_nt(a, b):
    return lax.dot_general(a, b, _NT_DIMS, preferred_element_type=F32)


def _dot(a, b):
    return jnp.dot(a, b, preferred_element_type=F32)


def _rb(x):
    return x.astype(BF16).astype(F32)


def _pk(x):
    return pltpu.bitcast(x, U32)


def _upk(x):
    return pltpu.bitcast(x, BF16)


def _phi_pair(p, link=None):
    pos, neg = [], []
    for a in range(2):
        ph = p[32 * a:32 * a + 32, :]
        mx = jnp.max(ph, axis=0, keepdims=True)
        mn = jnp.min(ph, axis=0, keepdims=True)
        if link is not None:
            mx, mn = link.start(mx, mn)
        ep = jnp.exp2(ph - mx)
        en = jnp.exp2(mn - ph)
        pos.append(ep * pl.reciprocal(jnp.sum(ep, axis=0, keepdims=True), approx=True))
        neg.append(en * pl.reciprocal(jnp.sum(en, axis=0, keepdims=True), approx=True))
        if link is not None:
            link.done(pos[-1], neg[-1])
    return jnp.concatenate(pos + neg, axis=0).astype(BF16)


def _silu(x):
    h = 0.5 * x
    return h + h * jnp.tanh(h)


def _kernel(x_hbm, wqkv_hbm, wphi_hbm, wo_hbm, wr_hbm, wg_hbm, wu_hbm, wd_hbm, out_hbm,
            x_buf, xn_buf, w_buf, wt_buf, wphi_buf, wr_buf, wo_buf, wg_buf, wu_buf, wd_buf,
            bdt_buf, g_acc, g_buf, r_buf, o_buf, out_buf, zero_buf, wop_buf,
            sem_x, sem_w, sem_s, sem_o):
    x_cp = [pltpu.make_async_copy(x_hbm.at[pl.ds(i * T, T), :], x_buf.at[pl.ds(i * T, T), :], sem_x.at[i])
            for i in range(NT)]
    w_cp = [pltpu.make_async_copy(wqkv_hbm.at[:, pl.ds(j * MC, MC)], w_buf.at[j], sem_w.at[j])
            for j in range(3 * NC)]
    q_cp, k_cp, v_cp = w_cp[:NC], w_cp[NC:2 * NC], w_cp[2 * NC:]
    phi_cp = pltpu.make_async_copy(wphi_hbm, wphi_buf, sem_s.at[0])
    wr_cp = pltpu.make_async_copy(wr_hbm, wr_buf, sem_s.at[1])
    wo_cp = pltpu.make_async_copy(wo_hbm, wo_buf, sem_s.at[2])
    f_cp = [pltpu.make_async_copy(wg_hbm, wg_buf, sem_s.at[3]),
            pltpu.make_async_copy(wu_hbm, wu_buf, sem_s.at[4]),
            pltpu.make_async_copy(wd_hbm, wd_buf, sem_s.at[5])]

    def out_copy(t, j):
        rows = pl.ds(pl.multiple_of(t * T, T), T)
        return pltpu.make_async_copy(out_buf.at[rows, :], out_hbm.at[rows, :], sem_o.at[j])

    def start_in_order(copies):
        def body(j, carry):
            for k, cp in enumerate(copies):
                pl.when(j == k)(cp.start)
            zero_buf[...] = jnp.zeros_like(zero_buf)
            return carry
        lax.fori_loop(0, len(copies), body, 0)

    start_in_order([x_cp[0], v_cp[0], wr_cp, v_cp[1], phi_cp, k_cp[0], k_cp[1], v_cp[2], k_cp[2],
                    v_cp[3], k_cp[3]])
    start_in_order(x_cp[1:] + q_cp)
    start_in_order([wo_cp] + f_cp)

    def tie(w, dep):
        acc = None
        for r in range(0, dep.shape[0], 8):
            for c in range(0, dep.shape[1], 128):
                piece = dep[r:r + 8, c:c + 128]
                acc = piece if acc is None else acc | piece
        first = w[:8, :128] | (acc & zero_buf[...])
        top = jnp.concatenate([first, w[:8, 128:]], axis=1)
        return jnp.concatenate([top, w[8:, :]], axis=0)

    def after(x, dep):
        z = pltpu.bitcast(dep, U32)[:x.shape[0], :] & zero_buf[:x.shape[0], :]
        return pltpu.bitcast(pltpu.bitcast(x, U32) | z, F32)

    class Link:
        def __init__(self):
            self.prev = None

        def start(self, mx, mn):
            if self.prev is None:
                return mx, mn
            return after(mx, self.prev[0]), after(mn, self.prev[1])

        def done(self, pos, neg):
            self.prev = (pos[24:32, :], neg[24:32, :])

    def layer_norm(i, piece=0, npieces=1):
        n = T // npieces
        r0 = i * T + piece * n
        x = x_buf[r0:r0 + n, :].astype(F32)
        m = jnp.mean(x, axis=-1, keepdims=True)
        xc = x - m
        v = jnp.mean(xc * xc, axis=-1, keepdims=True)
        den = _rb(jnp.sqrt(_rb(_rb(v) + EPS_LN)))
        xn = _pk((_rb(x - _rb(m)) * (1.0 / den)).astype(BF16))
        xn_buf[r0 // 2:(r0 + n) // 2, :] = xn
        return xn

    def load_wt(r0, r1, dep=None):
        w = wt_buf[r0 // 2:r1 // 2, :]
        if dep is not None:
            w = tie(w, dep)
        return _upk(w)

    def fold(j, u):
        w = w_buf[j, :, u * 128:(u + 1) * 128]
        if j < 2 * NC:
            r = _dot_nt(_upk(bdt_buf[(2 * j + u) % 8]), w) * LOG2E
        else:
            r = _dot_nt(_upk(bdt_buf[8]), w)
        row = (j * MC + u * 128 + (16 if j >= NC else 0)) // 2
        wt_buf[row:row + 64, :] = _pk(r.astype(BF16))

    def fold2(j):
        fold(j, 0)
        fold(j, 1)

    ri = lax.broadcasted_iota(jnp.int32, (128, 128), 0)
    ci = lax.broadcasted_iota(jnp.int32, (128, 128), 1)

    def build_bdt():
        same_head = (ri // 32) == (ci // 32)
        e_r = lax.broadcasted_iota(jnp.int32, (128, 32), 0)
        e_c = lax.broadcasted_iota(jnp.int32, (128, 32), 1)
        tile_eye = jnp.where((e_r % 32) == e_c, 1.0, 0.0).astype(BF16)
        for g in range(8):
            wg4 = wphi_buf[4 * g:4 * g + 4].reshape(128, 32)
            bdt_buf[g] = _pk(jnp.where(same_head, _dot_nt(tile_eye, wg4), 0.0).astype(BF16))

    ones = jnp.ones((16, T), BF16)

    class KV:
        def __init__(self, i, ln_tile=None):
            self.i, self.ln_tile, self.piece, self.dep = i, ln_tile, 0, None
            self.pk, self.vt = {}, {}

        def ln(self, count=1):
            if self.ln_tile is None or count == 0:
                return
            deps = [layer_norm(self.ln_tile, self.piece + e, LNP) for e in range(count)]
            self.piece += count
            self.dep = jnp.concatenate(deps, axis=0)

        def take(self):
            dep, self.dep = self.dep, None
            return dep

        def proj(self, r0, r1, dep, count):
            halves = []
            for n in range(2):
                row = (self.i * T + n * 128) // 2
                halves.append(_dot_nt(load_wt(r0, r1, dep), _upk(xn_buf[row:row + 64, :])))
                self.ln(count)
                if n == 0:
                    dep = self.take()
            return jnp.concatenate(halves, axis=1)

        def k(self, c, dep=None, count=0):
            if c == 0:
                kr = self.proj(KROW - 16, KROW + MC, dep, count)
                r_buf[self.i] = kr[:8, :]
                self.pk[c] = kr[16:, :]
            else:
                self.pk[c] = self.proj(KROW + c * MC, KROW + (c + 1) * MC, dep, count)

        def v(self, c, dep=None, count=0):
            self.vt[c] = self.proj(VROW + c * MC, VROW + (c + 1) * MC, dep, count).astype(BF16)

        def g(self, c):
            pk, vt = self.pk.pop(c), self.vt.pop(c)
            for u in range(PC):
                phi = _phi_pair(pk[64 * u:64 * u + 64, :])
                lhs = jnp.concatenate([vt[64 * u:64 * u + 64, :], ones], axis=0)
                r = _dot_nt(lhs, phi)
                if self.i == 0:
                    g_acc[c * PC + u] = r
                else:
                    g_acc[c * PC + u] += r

    bdt_buf[8] = _pk(jnp.where(ri == ci, 1.0, 0.0).astype(BF16))
    x_cp[0].wait()
    layer_norm(0)
    t0 = KV(0, 1)
    v_cp[0].wait()
    fold2(2 * NC)
    t0.v(0)
    wr_cp.wait()
    v_cp[1].wait()
    phi_cp.wait()
    wt_buf[D // 2:D // 2 + 8, :] = _pk(
        jnp.broadcast_to(wr_buf[...].astype(F32).reshape(1, D), (16, D)).astype(BF16))
    fold2(2 * NC + 1)
    build_bdt()
    t0.v(1)
    k_cp[0].wait()
    k_cp[1].wait()
    fold2(NC)
    fold2(NC + 1)
    t0.k(0)
    t0.k(1)
    t0.g(0)
    v_cp[2].wait()
    k_cp[2].wait()
    fold2(NC + 2)
    fold2(2 * NC + 2)
    t0.g(1)
    t0.k(2)
    t0.v(2)
    v_cp[3].wait()
    k_cp[3].wait()
    x_cp[1].wait()
    x_cp[2].wait()
    fold2(NC + 3)
    fold2(2 * NC + 3)
    t0.g(2)
    t0.ln(4)
    t0.k(3, t0.take(), 3)
    t0.v(3, t0.take(), 3)
    prev = t0

    for i in range(1, NT):
        if i == 2:
            for cp in x_cp[3:] + q_cp:
                cp.wait()
        kv = KV(i, i + 1 if i + 1 < NT else None)
        for c in range(NC):
            kv.k(c, prev.take() if c == 0 else kv.take(), 1)
            if c == 0:
                prev.g(NC - 1)
            else:
                kv.g(c - 1)
            kv.v(c, kv.take(), 1)
        if 2 <= i < 2 + NC:
            fold2(i - 2)
        prev = kv
    prev.g(NC - 1)

    gr = lax.broadcasted_iota(jnp.int32, (GR, 128), 0)
    gc = lax.broadcasted_iota(jnp.int32, (GR, 128), 1)
    row_head = jnp.where(gr < 64, gr // 32, (gr - 64) // 8)
    keep = row_head == ((gc % 64) // 32)
    for p in range(NP):
        g_buf[p] = _pk(jnp.where(keep, g_acc[p], 0.0).astype(BF16))

    r_all = _rb(r_buf[...])
    tok = (lax.broadcasted_iota(jnp.int32, (NT, 8, T), 0) * T
           + lax.broadcasted_iota(jnp.int32, (NT, 8, T), 2))
    r_max = jnp.max(r_all)
    idx = jnp.min(jnp.where(r_all == r_max, tok, S - 1))
    sel_tile = idx // T
    blk = pl.multiple_of((idx // 16) * 16, 16)

    def tile_of(j):
        return (sel_tile + 1 + j) % NT

    def last_copy(n):
        rows = pl.ds(pl.multiple_of(sel_tile * T, T), T)
        cols = pl.ds(n * 256, 256)
        return pltpu.make_async_copy(out_buf.at[rows, cols], out_hbm.at[rows, cols], sem_o.at[NT - 1 + n])

    class Q:
        def __init__(self, j):
            self.j = j
            self.row0 = tile_of(j) * (T // 2)
            self.pq = {}

        def proj(self, c, n, dep=None):
            xn = _upk(xn_buf[pl.ds(pl.multiple_of(self.row0 + n * 64, 64), 64), :])
            self.pq[c, n] = _dot_nt(load_wt(c * MC, (c + 1) * MC, dep), xn)

        def num(self, c, n):
            pq = self.pq.pop((c, n))
            parts = []
            link = Link()
            for u in range(PC):
                nd = _dot(_upk(g_buf[c * PC + u]), _phi_pair(pq[64 * u:64 * u + 64, :], link))
                for a in range(2):
                    inv = pl.reciprocal(nd[64 + 8 * a:72 + 8 * a, :] + 1e-6, approx=True)
                    parts.append(nd[32 * a:32 * a + 32, :] * jnp.concatenate([inv] * 4, axis=0))
            ot = jnp.concatenate(parts, axis=0)
            o_buf[self.j % 2, n * 64:(n + 1) * 64, c * MC:(c + 1) * MC] = _pk(ot.T.astype(BF16))

    def out_cols(j, n, dep=None, upd=None):
        t = tile_of(j)
        rows = pl.ds(pl.multiple_of(t * T, T), T)
        rows2 = pl.ds(pl.multiple_of(t * (T // 2), T // 2), T // 2)
        cols = slice(n * 128, (n + 1) * 128)
        o = o_buf[j % 2]
        if dep is not None:
            o = tie(o, dep)
        s = _dot(_upk(o), _upk(wop_buf[:, cols]))
        xn = _upk(xn_buf[rows2, cols]).astype(F32)
        if upd is not None:
            xn = xn + upd[:, cols]
        out_buf[rows, cols] = (x_buf[rows, cols].astype(F32) + s * _silu(xn)).astype(BF16)

    def ffn_steps():
        st = {}
        KH = D // 2

        def up(w_ref, key, n, h):
            def f():
                xs = _upk(xn_buf[pl.ds(pl.multiple_of(blk // 2, 8), 8), h * KH:(h + 1) * KH])
                r = _dot(xs, w_ref[h * KH:(h + 1) * KH, n * 128:(n + 1) * 128])
                if h == 0:
                    z = zero_buf[...]
                    st[key, n] = pltpu.bitcast(pltpu.bitcast(r, U32) | jnp.concatenate([z, z], axis=0), F32)
                else:
                    st[key, n] = st[key, n] + r
            return f

        def down(c, n):
            def f():
                if ('h', c) not in st:
                    ms = range(c * FC // 128, (c + 1) * FC // 128)
                    st['h', c] = jnp.concatenate(
                        [_silu(st.pop(('g', m))) * st.pop(('u', m)) for m in ms], axis=1).astype(BF16)
                r = _dot(st['h', c], wd_buf[c * FC:(c + 1) * FC, n * 128:(n + 1) * 128])
                st['y', n] = r if c == 0 else st['y', n] + r
            return f

        steps = []
        for c in range(F // FC + 1):
            ups = [up(w, k, m, h) for m in range(c * FC // 128, (c + 1) * FC // 128)
                   for h in range(2) for w, k in ((wg_buf, 'g'), (wu_buf, 'u'))] if c < F // FC else []
            downs = [down(c - 1, n) for n in range(D // 128)] if c > 0 else []
            while ups or downs:
                steps += ups[:2] + downs[:1]
                ups, downs = ups[2:], downs[1:]
        return steps, st

    wo_cp.wait()
    for cp in f_cp:
        cp.wait()
    wop_buf[...] = _pk(wo_buf[...])
    ffn, ffn_st = ffn_steps()

    q = Q(0)
    for c in range(NC):
        q.proj(c, 0)
        if c > 0:
            q.num(c - 1, 1)
        q.proj(c, 1)
        q.num(c, 0)
    def small():
        if ffn:
            ffn.pop(0)()

    pending = []

    def out_step():
        j, n = pending.pop(0)
        out_cols(j, n)
        if n == D // 128 - 1:
            out_copy(tile_of(j), j).start()

    for j in range(1, NT):
        qn = Q(j)
        pending += [(j - 1, n) for n in range(D // 128)]
        for c in range(NC):
            qn.proj(c, 0)
            small()
            qn.proj(c, 1)
            small()
            if c == 0:
                q.num(NC - 1, 1)
            else:
                qn.num(c - 1, 1)
            small()
            if (j, c) != (1, 0):
                out_step()
            small()
            qn.num(c, 0)
            small()
            out_step()
            small()
        q = qn
    assert not ffn
    q.num(NC - 1, 1)
    out_step()

    y = jnp.concatenate([ffn_st['y', n] for n in range(D // 128)], axis=1)
    sub = lax.broadcasted_iota(jnp.int32, (16, D), 0)
    y_row = jnp.sum(jnp.where(sub == idx - blk, y, 0.0), axis=0, keepdims=True)
    gate = 1.0 / (1.0 + jnp.exp(-jnp.full((1, D), r_max, F32)))
    trow = lax.broadcasted_iota(jnp.int32, (T, D), 0)
    upd = jnp.where(trow == idx - sel_tile * T, y_row * gate, 0.0)
    for n in range(D // 128):
        out_cols(NT - 1, n, None, upd)
        if n % 2 == 1:
            last_copy(n // 2).start()
    for j in range(NT - 1):
        out_copy(tile_of(j), j).wait()
    for n in range(D // 256):
        last_copy(n).wait()


@jax.jit
def pallas_recurrent_scan__linear_kernel_hedgehog__moe_arch_mod__prompt_kernel(
    A_x: jax.Array,
    A_wqkv: jax.Array,
    A_w_phi: jax.Array,
    A_wo: jax.Array,
    B_x: jax.Array,
    B_w_r: jax.Array,
    B_w_gate: jax.Array,
    B_w_up: jax.Array,
    B_w_down: jax.Array,
):
    del B_x
    any_spec = pl.BlockSpec(memory_space=pl.ANY)
    out = pl.pallas_call(
        _kernel,
        out_shape=jax.ShapeDtypeStruct((S, D), BF16),
        in_specs=[any_spec] * 8,
        out_specs=any_spec,
        scratch_shapes=[
            pltpu.VMEM((S, D), BF16),
            pltpu.VMEM((S // 2, D), U32),
            pltpu.VMEM((3 * NC, D, MC), BF16),
            pltpu.VMEM((3 * D // 2 + 8, D), U32),
            pltpu.VMEM((H, DH, DH), BF16),
            pltpu.VMEM((D,), BF16),
            pltpu.VMEM((D, D), BF16),
            pltpu.VMEM((D, F), BF16),
            pltpu.VMEM((D, F), BF16),
            pltpu.VMEM((F, D), BF16),
            pltpu.VMEM((9, 64, 128), U32),
            pltpu.VMEM((NP, GR, 128), F32),
            pltpu.VMEM((NP, GR // 2, 128), U32),
            pltpu.VMEM((NT, 8, T), F32),
            pltpu.VMEM((2, T // 2, D), U32),
            pltpu.VMEM((S, D), BF16),
            pltpu.VMEM((8, 128), U32),
            pltpu.VMEM((D // 2, D), U32),
            pltpu.SemaphoreType.DMA((NT,)),
            pltpu.SemaphoreType.DMA((3 * NC,)),
            pltpu.SemaphoreType.DMA((6,)),
            pltpu.SemaphoreType.DMA((NT + 3,)),
        ],
        compiler_params=pltpu.CompilerParams(
            vmem_limit_bytes=100 * 1024 * 1024,
            disable_bounds_checks=True,
            disable_semaphore_checks=True,
        ),
        name="hedgehog_mod",
    )(A_x.reshape(S, D), A_wqkv, A_w_phi, A_wo, B_w_r, B_w_gate, B_w_up, B_w_down)
    return out.reshape(1, S, D)
```

```python
import jax
import jax.numpy as jnp
from jax import lax
import jax.experimental.pallas as pl
import jax.experimental.pallas.tpu as pltpu

S, D, H, DH, F = 2048, 1024, 32, 32, 3584
T = 256
NT = S // T
MC = 256
NC = D // MC
PC = MC // 64
NP = H // 2
GR = 80
FC = 512
LNP = 16
KROW = D + 16
VROW = KROW + D
WTR = (VROW + D) // 2
QFOLD_EARLY = False
PACK_EARLY = True
BREAK_CSE = False
PATTERN = "PfQfnfWfmfWf"
LOG2E = 1.4426950408889634
EPS_LN = 1.0013580322265625e-05
F32 = jnp.float32
BF16 = jnp.bfloat16
U32 = jnp.uint32

_NT_DIMS = (((1,), (1,)), ((), ()))


def _dot_nt(a, b):
    return lax.dot_general(a, b, _NT_DIMS, preferred_element_type=F32)


def _dot(a, b):
    return jnp.dot(a, b, preferred_element_type=F32)


def _rb(x):
    return x.astype(BF16).astype(F32)


def _pk(x):
    return pltpu.bitcast(x, U32)


def _upk(x):
    return pltpu.bitcast(x, BF16)


def _phi_pair(p, link=None):
    pos, neg = [], []
    for a in range(2):
        ph = p[32 * a:32 * a + 32, :]
        mx = jnp.max(ph, axis=0, keepdims=True)
        mn = jnp.min(ph, axis=0, keepdims=True)
        if link is not None:
            mx, mn = link.start(mx, mn)
        ep = jnp.exp2(ph - mx)
        en = jnp.exp2(mn - ph)
        pos.append(ep * pl.reciprocal(jnp.sum(ep, axis=0, keepdims=True), approx=True))
        neg.append(en * pl.reciprocal(jnp.sum(en, axis=0, keepdims=True), approx=True))
        if link is not None:
            link.done(pos[-1], neg[-1])
    return jnp.concatenate(pos + neg, axis=0).astype(BF16)


def _silu(x):
    h = 0.5 * x
    return h + h * jnp.tanh(h)


def _kernel(x_hbm, wqkv_hbm, wphi_hbm, wo_hbm, wr_hbm, wg_hbm, wu_hbm, wd_hbm, out_hbm,
            x_buf, xn_buf, w_buf, wt_buf, wphi_buf, wr_buf, wo_buf, wg_buf, wu_buf, wd_buf,
            bdt_buf, g_acc, g_buf, r_buf, o_buf, out_buf, zero_buf, wop_buf,
            sem_x, sem_w, sem_s, sem_o):
    x_cp = [pltpu.make_async_copy(x_hbm.at[pl.ds(i * T, T), :], x_buf.at[pl.ds(i * T, T), :], sem_x.at[i])
            for i in range(NT)]
    w_cp = [pltpu.make_async_copy(wqkv_hbm.at[:, pl.ds(j * MC, MC)], w_buf.at[j], sem_w.at[j])
            for j in range(3 * NC)]
    q_cp, k_cp, v_cp = w_cp[:NC], w_cp[NC:2 * NC], w_cp[2 * NC:]
    phi_cp = pltpu.make_async_copy(wphi_hbm, wphi_buf, sem_s.at[0])
    wr_cp = pltpu.make_async_copy(wr_hbm, wr_buf, sem_s.at[1])
    wo_cp = pltpu.make_async_copy(wo_hbm, wo_buf, sem_s.at[2])
    f_cp = [pltpu.make_async_copy(wg_hbm, wg_buf, sem_s.at[3]),
            pltpu.make_async_copy(wu_hbm, wu_buf, sem_s.at[4]),
            pltpu.make_async_copy(wd_hbm, wd_buf, sem_s.at[5])]

    def out_copy(t, j):
        rows = pl.ds(pl.multiple_of(t * T, T), T)
        return pltpu.make_async_copy(out_buf.at[rows, :], out_hbm.at[rows, :], sem_o.at[j])

    def start_in_order(copies):
        def body(j, carry):
            for k, cp in enumerate(copies):
                pl.when(j == k)(cp.start)
            zero_buf[...] = jnp.zeros_like(zero_buf)
            return carry
        lax.fori_loop(0, len(copies), body, 0)

    start_in_order([x_cp[0], v_cp[0], x_cp[1], v_cp[1], wr_cp, phi_cp, k_cp[0], k_cp[1], v_cp[2], k_cp[2],
                    v_cp[3], k_cp[3]])
    if QFOLD_EARLY:
        start_in_order(x_cp[2:] + q_cp)
        start_in_order([wo_cp] + f_cp)
    else:
        start_in_order(x_cp[2:] + [wo_cp])
        start_in_order(q_cp + f_cp)

    def tie(w, dep):
        acc = None
        for r in range(0, dep.shape[0], 8):
            for c in range(0, dep.shape[1], 128):
                piece = dep[r:r + 8, c:c + 128]
                acc = piece if acc is None else acc | piece
        first = w[:8, :128] | (acc & zero_buf[...])
        top = jnp.concatenate([first, w[:8, 128:]], axis=1)
        return jnp.concatenate([top, w[8:, :]], axis=0)

    def after(x, dep):
        z = pltpu.bitcast(dep, U32)[:x.shape[0], :] & zero_buf[:x.shape[0], :]
        return pltpu.bitcast(pltpu.bitcast(x, U32) | z, F32)

    class Link:
        def __init__(self):
            self.prev = None

        def start(self, mx, mn):
            if self.prev is None:
                return mx, mn
            return after(mx, self.prev[0]), after(mn, self.prev[1])

        def done(self, pos, neg):
            self.prev = (pos[24:32, :], neg[24:32, :])

    def layer_norm(i, piece=0, npieces=1):
        n = T // npieces
        r0 = i * T + piece * n
        x = x_buf[r0:r0 + n, :].astype(F32)
        m = jnp.mean(x, axis=-1, keepdims=True)
        xc = x - m
        v = jnp.mean(xc * xc, axis=-1, keepdims=True)
        den = _rb(jnp.sqrt(_rb(_rb(v) + EPS_LN)))
        xn = _pk((_rb(x - _rb(m)) * (1.0 / den)).astype(BF16))
        xn_buf[r0 // 2:(r0 + n) // 2, :] = xn
        return xn

    def load_wt(r0, r1, dep=None):
        w = wt_buf[r0 // 2:r1 // 2, :]
        if dep is not None:
            w = tie(w, dep)
        return _upk(w)

    def fold(j, u):
        w = w_buf[j, :, u * 128:(u + 1) * 128]
        if j < 2 * NC:
            r = _dot_nt(_upk(bdt_buf[(2 * j + u) % 8]), w) * LOG2E
        else:
            r = _dot_nt(_upk(bdt_buf[8]), w)
        row = (j * MC + u * 128 + (16 if j >= NC else 0)) // 2
        wt_buf[row:row + 64, :] = _pk(r.astype(BF16))

    def fold2(j):
        fold(j, 0)
        fold(j, 1)

    ri = lax.broadcasted_iota(jnp.int32, (128, 128), 0)
    ci = lax.broadcasted_iota(jnp.int32, (128, 128), 1)

    def build_bdt():
        same_head = (ri // 32) == (ci // 32)
        e_r = lax.broadcasted_iota(jnp.int32, (128, 32), 0)
        e_c = lax.broadcasted_iota(jnp.int32, (128, 32), 1)
        tile_eye = jnp.where((e_r % 32) == e_c, 1.0, 0.0).astype(BF16)
        for g in range(8):
            wg4 = wphi_buf[4 * g:4 * g + 4].reshape(128, 32)
            bdt_buf[g] = _pk(jnp.where(same_head, _dot_nt(tile_eye, wg4), 0.0).astype(BF16))

    ones = jnp.ones((16, T), BF16)

    side = []

    def take_side(count=1):
        deps = [side.pop(0) for _ in range(min(count, len(side)))]
        deps = [f() for f in deps if f is not None]
        return (jnp.concatenate(deps, axis=0) if len(deps) > 1 else deps[0]) if deps else None

    def ln_pieces(i):
        return [lambda p=p: layer_norm(i, p, LNP) for p in range(LNP)]

    def pack_wo(p):
        rows = D // LNP
        w = _pk(wo_buf[p * rows:(p + 1) * rows, :])
        wop_buf[p * rows // 2:(p + 1) * rows // 2, :] = w
        return w

    class KV:
        def __init__(self, i):
            self.i = i
            self.pk, self.vt, self.ph = {}, {}, {}

        def proj(self, r0, r1):
            halves = []
            for n in range(2):
                row = (self.i * T + n * 128) // 2
                halves.append(_dot_nt(load_wt(r0, r1, take_side()), _upk(xn_buf[row:row + 64, :])))
            return jnp.concatenate(halves, axis=1)

        def k(self, c):
            if c == 0:
                kr = self.proj(KROW - 16, KROW + MC)
                r_buf[self.i] = kr[:8, :]
                self.pk[c] = kr[16:, :]
            else:
                self.pk[c] = self.proj(KROW + c * MC, KROW + (c + 1) * MC)

        def v(self, c):
            self.vt[c] = self.proj(VROW + c * MC, VROW + (c + 1) * MC).astype(BF16)

        def phi(self, c):
            if c not in self.ph:
                pk = self.pk.pop(c)
                self.ph[c] = [_phi_pair(pk[64 * u:64 * u + 64, :]) for u in range(PC)]
            return self.ph[c]

        def g(self, c):
            vt = self.vt.pop(c)
            for u, phi in enumerate(self.phi(c)):
                lhs = jnp.concatenate([vt[64 * u:64 * u + 64, :], ones], axis=0)
                r = _dot_nt(lhs, phi)
                if self.i == 0:
                    g_acc[c * PC + u] = r
                else:
                    g_acc[c * PC + u] += r

    bdt_buf[8] = _pk(jnp.where(ri == ci, 1.0, 0.0).astype(BF16))
    x_cp[0].wait()
    layer_norm(0)
    t0, t1 = KV(0), KV(1)
    v_cp[0].wait()
    fold2(2 * NC)
    t0.v(0)
    x_cp[1].wait()
    layer_norm(1)
    v_cp[1].wait()
    fold2(2 * NC + 1)
    t1.v(0)
    t0.v(1)
    t1.v(1)
    wr_cp.wait()
    phi_cp.wait()
    k_cp[0].wait()
    k_cp[1].wait()
    wt_buf[D // 2:D // 2 + 8, :] = _pk(
        jnp.broadcast_to(wr_buf[...].astype(F32).reshape(1, D), (16, D)).astype(BF16))
    build_bdt()
    fold2(NC)
    fold2(NC + 1)
    t0.k(0)
    t1.k(0)
    t0.k(1)
    t0.g(0)
    t1.k(1)
    t1.g(0)
    t0.g(1)
    t1.phi(1)
    for cp in [v_cp[2], k_cp[2], v_cp[3], k_cp[3], x_cp[2]]:
        cp.wait()
    side += ln_pieces(2)
    fold2(NC + 2)
    fold2(2 * NC + 2)
    t1.g(1)
    t0.k(2)
    t0.v(2)
    fold2(NC + 3)
    t1.k(2)
    t0.g(2)
    t1.v(2)
    fold2(2 * NC + 3)
    t0.k(3)
    t1.g(2)
    t0.v(3)
    t1.k(3)
    t0.g(3)
    t1.v(3)
    t1.phi(3)
    prev = t1

    def break_cse():
        if BREAK_CSE:
            wt_buf[WTR:WTR + 8, :128] = zero_buf[...]
            wop_buf[D // 2:D // 2 + 8, :128] = zero_buf[...]

    for i in range(2, NT):
        if i == 2:
            for cp in x_cp[3:] + (q_cp if QFOLD_EARLY else []) + ([wo_cp] if PACK_EARLY else []):
                cp.wait()
        if i == 2:
            side += [None]
        if i + 1 < NT:
            side += ln_pieces(i + 1)
        elif PACK_EARLY:
            side += [lambda p=p: pack_wo(p) for p in range(LNP)]
        break_cse()
        kv = KV(i)
        for c in range(NC):
            kv.k(c)
            if c == 0:
                prev.g(NC - 1)
            else:
                kv.g(c - 1)
            kv.v(c)
        if QFOLD_EARLY and i - 2 < NC:
            fold2(i - 2)
        prev = kv
    prev.g(NC - 1)
    take_side(len(side))

    gr = lax.broadcasted_iota(jnp.int32, (GR, 128), 0)
    gc = lax.broadcasted_iota(jnp.int32, (GR, 128), 1)
    row_head = jnp.where(gr < 64, gr // 32, (gr - 64) // 8)
    keep = row_head == ((gc % 64) // 32)
    for p in range(NP):
        g_buf[p] = _pk(jnp.where(keep, g_acc[p], 0.0).astype(BF16))

    r_all = _rb(r_buf[...])
    tok = (lax.broadcasted_iota(jnp.int32, (NT, 8, T), 0) * T
           + lax.broadcasted_iota(jnp.int32, (NT, 8, T), 2))
    r_max = jnp.max(r_all)
    idx = jnp.min(jnp.where(r_all == r_max, tok, S - 1))
    sel_tile = idx // T
    blk = pl.multiple_of((idx // 16) * 16, 16)

    def tile_of(j):
        return (sel_tile + 1 + j) % NT

    def last_copy(n):
        rows = pl.ds(pl.multiple_of(sel_tile * T, T), T)
        cols = pl.ds(n * 256, 256)
        return pltpu.make_async_copy(out_buf.at[rows, cols], out_hbm.at[rows, cols], sem_o.at[NT - 1 + n])

    class Q:
        def __init__(self, j):
            self.j = j
            self.row0 = tile_of(j) * (T // 2)
            self.pq = {}

        def proj(self, c, n, dep=None):
            xn = _upk(xn_buf[pl.ds(pl.multiple_of(self.row0 + n * 64, 64), 64), :])
            self.pq[c, n] = _dot_nt(load_wt(c * MC, (c + 1) * MC, dep), xn)

        def num(self, c, n):
            pq = self.pq.pop((c, n))
            parts = []
            link = Link()
            for u in range(PC):
                nd = _dot(_upk(g_buf[c * PC + u]), _phi_pair(pq[64 * u:64 * u + 64, :], link))
                for a in range(2):
                    inv = pl.reciprocal(nd[64 + 8 * a:72 + 8 * a, :] + 1e-6, approx=True)
                    parts.append(nd[32 * a:32 * a + 32, :] * jnp.concatenate([inv] * 4, axis=0))
            ot = jnp.concatenate(parts, axis=0)
            o_buf[self.j % 2, n * 64:(n + 1) * 64, c * MC:(c + 1) * MC] = _pk(ot.T.astype(BF16))

    def out_cols(j, n, dep=None, upd=None):
        t = tile_of(j)
        rows = pl.ds(pl.multiple_of(t * T, T), T)
        rows2 = pl.ds(pl.multiple_of(t * (T // 2), T // 2), T // 2)
        cols = slice(n * 128, (n + 1) * 128)
        o = o_buf[j % 2]
        if dep is not None:
            o = tie(o, dep)
        s = _dot(_upk(o), _upk(wop_buf[:D // 2, cols]))
        xn = _upk(xn_buf[rows2, cols]).astype(F32)
        if upd is not None:
            xn = xn + upd[:, cols]
        out_buf[rows, cols] = (x_buf[rows, cols].astype(F32) + s * _silu(xn)).astype(BF16)

    def ffn_steps():
        st = {}
        KH = D // 2

        def up(w_ref, key, n, h):
            def f():
                xs = _upk(xn_buf[pl.ds(pl.multiple_of(blk // 2, 8), 8), h * KH:(h + 1) * KH])
                r = _dot(xs, w_ref[h * KH:(h + 1) * KH, n * 128:(n + 1) * 128])
                if h == 0:
                    z = zero_buf[...]
                    st[key, n] = pltpu.bitcast(pltpu.bitcast(r, U32) | jnp.concatenate([z, z], axis=0), F32)
                else:
                    st[key, n] = st[key, n] + r
            return f

        def down(c, n):
            def f():
                if ('h', c) not in st:
                    ms = range(c * FC // 128, (c + 1) * FC // 128)
                    st['h', c] = jnp.concatenate(
                        [_silu(st.pop(('g', m))) * st.pop(('u', m)) for m in ms], axis=1).astype(BF16)
                r = _dot(st['h', c], wd_buf[c * FC:(c + 1) * FC, n * 128:(n + 1) * 128])
                st['y', n] = r if c == 0 else st['y', n] + r
            return f

        steps = []
        for c in range(F // FC + 1):
            ups = [up(w, k, m, h) for m in range(c * FC // 128, (c + 1) * FC // 128)
                   for h in range(2) for w, k in ((wg_buf, 'g'), (wu_buf, 'u'))] if c < F // FC else []
            downs = [down(c - 1, n) for n in range(D // 128)] if c > 0 else []
            while ups or downs:
                steps += ups[:2] + downs[:1]
                ups, downs = ups[2:], downs[1:]
        return steps, st

    for cp in ([] if QFOLD_EARLY else q_cp) + ([] if PACK_EARLY else [wo_cp]) + f_cp:
        cp.wait()
    if not QFOLD_EARLY:
        for j in range(NC):
            fold2(j)
    if not PACK_EARLY:
        wop_buf[:D // 2, :] = _pk(wo_buf[...])
    ffn, ffn_st = ffn_steps()

    q = Q(0)
    for c in range(NC):
        q.proj(c, 0)
        if c > 0:
            q.num(c - 1, 1)
        q.proj(c, 1)
        q.num(c, 0)
    def small():
        if ffn:
            ffn.pop(0)()

    pending = []

    def out_step():
        j, n = pending.pop(0)
        out_cols(j, n)
        if n == D // 128 - 1:
            out_copy(tile_of(j), j).start()

    for j in range(1, NT):
        qn = Q(j)
        pending += [(j - 1, n) for n in range(D // 128)]
        break_cse()
        for c in range(NC):
            first_w = True
            for tok in PATTERN:
                if tok == 'P':
                    qn.proj(c, 0)
                elif tok == 'Q':
                    qn.proj(c, 1)
                elif tok == 'f':
                    small()
                elif tok == 'n':
                    (q if c == 0 else qn).num((c - 1) % NC, 1)
                elif tok == 'm':
                    qn.num(c, 0)
                elif tok == 'W':
                    if (j, c) != (1, 0) or not first_w:
                        out_step()
                    first_w = False
        q = qn
    assert not ffn
    q.num(NC - 1, 1)
    out_step()

    y = jnp.concatenate([ffn_st['y', n] for n in range(D // 128)], axis=1)
    sub = lax.broadcasted_iota(jnp.int32, (16, D), 0)
    y_row = jnp.sum(jnp.where(sub == idx - blk, y, 0.0), axis=0, keepdims=True)
    gate = 1.0 / (1.0 + jnp.exp(-jnp.full((1, D), r_max, F32)))
    trow = lax.broadcasted_iota(jnp.int32, (T, D), 0)
    upd = jnp.where(trow == idx - sel_tile * T, y_row * gate, 0.0)
    for n in range(D // 128):
        out_cols(NT - 1, n, None, upd)
        if n % 2 == 1:
            last_copy(n // 2).start()
    for j in range(NT - 1):
        out_copy(tile_of(j), j).wait()
    for n in range(D // 256):
        last_copy(n).wait()


@jax.jit
def pallas_recurrent_scan__linear_kernel_hedgehog__moe_arch_mod__prompt_kernel(
    A_x: jax.Array,
    A_wqkv: jax.Array,
    A_w_phi: jax.Array,
    A_wo: jax.Array,
    B_x: jax.Array,
    B_w_r: jax.Array,
    B_w_gate: jax.Array,
    B_w_up: jax.Array,
    B_w_down: jax.Array,
):
    del B_x
    any_spec = pl.BlockSpec(memory_space=pl.ANY)
    out = pl.pallas_call(
        _kernel,
        out_shape=jax.ShapeDtypeStruct((S, D), BF16),
        in_specs=[any_spec] * 8,
        out_specs=any_spec,
        scratch_shapes=[
            pltpu.VMEM((S, D), BF16),
            pltpu.VMEM((S // 2, D), U32),
            pltpu.VMEM((3 * NC, D, MC), BF16),
            pltpu.VMEM((WTR + 8, D), U32),
            pltpu.VMEM((H, DH, DH), BF16),
            pltpu.VMEM((D,), BF16),
            pltpu.VMEM((D, D), BF16),
            pltpu.VMEM((D, F), BF16),
            pltpu.VMEM((D, F), BF16),
            pltpu.VMEM((F, D), BF16),
            pltpu.VMEM((9, 64, 128), U32),
            pltpu.VMEM((NP, GR, 128), F32),
            pltpu.VMEM((NP, GR // 2, 128), U32),
            pltpu.VMEM((NT, 8, T), F32),
            pltpu.VMEM((2, T // 2, D), U32),
            pltpu.VMEM((S, D), BF16),
            pltpu.VMEM((8, 128), U32),
            pltpu.VMEM((D // 2 + 8, D), U32),
            pltpu.SemaphoreType.DMA((NT,)),
            pltpu.SemaphoreType.DMA((3 * NC,)),
            pltpu.SemaphoreType.DMA((6,)),
            pltpu.SemaphoreType.DMA((NT + 3,)),
        ],
        compiler_params=pltpu.CompilerParams(
            vmem_limit_bytes=100 * 1024 * 1024,
            disable_bounds_checks=True,
            disable_semaphore_checks=True,
        ),
        name="hedgehog_mod",
    )(A_x.reshape(S, D), A_wqkv, A_w_phi, A_wo, B_w_r, B_w_gate, B_w_up, B_w_down)
    return out.reshape(1, S, D)
```

```python
import jax
import jax.numpy as jnp
from jax import lax
import jax.experimental.pallas as pl
import jax.experimental.pallas.tpu as pltpu

S, D, H, DH, F = 2048, 1024, 32, 32, 3584
T = 256
NT = S // T
MC = 256
NC = D // MC
PC = MC // 64
NP = H // 2
FC = 512
LNP = 16
KROW = D + 16
VROW = KROW + D
WTR = (VROW + D) // 2
QFOLD_EARLY = False
PACK_EARLY = True
BREAK_CSE = False
PATTERN = "PQffWfnfWffm"
DENVPU = True
ZVPU = True
VXLU = (1, 2, 3)
VX32 = True
GA = 64 if ZVPU else 80
GR = 64 if DENVPU else 80
LOG2E = 1.4426950408889634
EPS_LN = 1.0013580322265625e-05
F32 = jnp.float32
BF16 = jnp.bfloat16
U32 = jnp.uint32

_NT_DIMS = (((1,), (1,)), ((), ()))


def _dot_nt(a, b):
    return lax.dot_general(a, b, _NT_DIMS, preferred_element_type=F32)


def _dot(a, b):
    return jnp.dot(a, b, preferred_element_type=F32)


def _rb(x):
    return x.astype(BF16).astype(F32)


def _pk(x):
    return pltpu.bitcast(x, U32)


def _upk(x):
    return pltpu.bitcast(x, BF16)


def _phi_pair(p, link=None):
    pos, neg = [], []
    for a in range(2):
        ph = p[32 * a:32 * a + 32, :]
        mx = jnp.max(ph, axis=0, keepdims=True)
        mn = jnp.min(ph, axis=0, keepdims=True)
        if link is not None:
            mx, mn = link.start(mx, mn)
        ep = jnp.exp2(ph - mx)
        en = jnp.exp2(mn - ph)
        pos.append(ep * pl.reciprocal(jnp.sum(ep, axis=0, keepdims=True), approx=True))
        neg.append(en * pl.reciprocal(jnp.sum(en, axis=0, keepdims=True), approx=True))
        if link is not None:
            link.done(pos[-1], neg[-1])
    return jnp.concatenate(pos + neg, axis=0)


def _silu(x):
    h = 0.5 * x
    return h + h * jnp.tanh(h)


def _kernel(x_hbm, wqkv_hbm, wphi_hbm, wo_hbm, wr_hbm, wg_hbm, wu_hbm, wd_hbm, out_hbm,
            x_buf, xn_buf, w_buf, wt_buf, wphi_buf, wr_buf, wo_buf, wg_buf, wu_buf, wd_buf,
            bdt_buf, g_acc, g_buf, r_buf, o_buf, out_buf, zero_buf, wop_buf, z_acc, zb_buf,
            sem_x, sem_w, sem_s, sem_o):
    x_cp = [pltpu.make_async_copy(x_hbm.at[pl.ds(i * T, T), :], x_buf.at[pl.ds(i * T, T), :], sem_x.at[i])
            for i in range(NT)]
    w_cp = [pltpu.make_async_copy(wqkv_hbm.at[:, pl.ds(j * MC, MC)], w_buf.at[j], sem_w.at[j])
            for j in range(3 * NC)]
    q_cp, k_cp, v_cp = w_cp[:NC], w_cp[NC:2 * NC], w_cp[2 * NC:]
    phi_cp = pltpu.make_async_copy(wphi_hbm, wphi_buf, sem_s.at[0])
    wr_cp = pltpu.make_async_copy(wr_hbm, wr_buf, sem_s.at[1])
    wo_cp = pltpu.make_async_copy(wo_hbm, wo_buf, sem_s.at[2])
    f_cp = [pltpu.make_async_copy(wg_hbm, wg_buf, sem_s.at[3]),
            pltpu.make_async_copy(wu_hbm, wu_buf, sem_s.at[4]),
            pltpu.make_async_copy(wd_hbm, wd_buf, sem_s.at[5])]

    def out_copy(t, j):
        rows = pl.ds(pl.multiple_of(t * T, T), T)
        return pltpu.make_async_copy(out_buf.at[rows, :], out_hbm.at[rows, :], sem_o.at[j])

    def start_in_order(copies):
        def body(j, carry):
            for k, cp in enumerate(copies):
                pl.when(j == k)(cp.start)
            zero_buf[...] = jnp.zeros_like(zero_buf)
            return carry
        lax.fori_loop(0, len(copies), body, 0)

    start_in_order([x_cp[0], v_cp[0], x_cp[1], v_cp[1], wr_cp, phi_cp, k_cp[0], k_cp[1], v_cp[2], k_cp[2],
                    v_cp[3], k_cp[3]])
    if QFOLD_EARLY:
        start_in_order(x_cp[2:] + q_cp)
        start_in_order([wo_cp] + f_cp)
    else:
        start_in_order(x_cp[2:] + [wo_cp])
        start_in_order(q_cp + f_cp)

    def tie(w, dep):
        acc = None
        for r in range(0, dep.shape[0], 8):
            for c in range(0, dep.shape[1], 128):
                piece = dep[r:r + 8, c:c + 128]
                acc = piece if acc is None else acc | piece
        first = w[:8, :128] | (acc & zero_buf[...])
        top = jnp.concatenate([first, w[:8, 128:]], axis=1)
        return jnp.concatenate([top, w[8:, :]], axis=0)

    def after(x, dep):
        z = pltpu.bitcast(dep, U32)[:x.shape[0], :] & zero_buf[:x.shape[0], :]
        return pltpu.bitcast(pltpu.bitcast(x, U32) | z, F32)

    class Link:
        def __init__(self):
            self.prev = None

        def start(self, mx, mn):
            if self.prev is None:
                return mx, mn
            return after(mx, self.prev[0]), after(mn, self.prev[1])

        def done(self, pos, neg):
            self.prev = (pos[24:32, :], neg[24:32, :])

    def layer_norm(i, piece=0, npieces=1):
        n = T // npieces
        r0 = i * T + piece * n
        x = x_buf[r0:r0 + n, :].astype(F32)
        m = jnp.mean(x, axis=-1, keepdims=True)
        xc = x - m
        v = jnp.mean(xc * xc, axis=-1, keepdims=True)
        den = _rb(jnp.sqrt(_rb(_rb(v) + EPS_LN)))
        xn = _pk((_rb(x - _rb(m)) * (1.0 / den)).astype(BF16))
        xn_buf[r0 // 2:(r0 + n) // 2, :] = xn
        return xn

    def load_wt(r0, r1, dep=None):
        w = wt_buf[r0 // 2:r1 // 2, :]
        if dep is not None:
            w = tie(w, dep)
        return _upk(w)

    def fold(j, u):
        w = w_buf[j, :, u * 128:(u + 1) * 128]
        if j < 2 * NC:
            r = _dot_nt(_upk(bdt_buf[(2 * j + u) % 8]), w) * LOG2E
        elif j - 2 * NC in VXLU:
            r = w.astype(F32).T if VX32 else w.T
        else:
            r = _dot_nt(_upk(bdt_buf[8]), w)
        row = (j * MC + u * 128 + (16 if j >= NC else 0)) // 2
        wt_buf[row:row + 64, :] = _pk(r.astype(BF16))

    def fold2(j):
        fold(j, 0)
        fold(j, 1)

    ri = lax.broadcasted_iota(jnp.int32, (128, 128), 0)
    ci = lax.broadcasted_iota(jnp.int32, (128, 128), 1)

    def build_bdt():
        same_head = (ri // 32) == (ci // 32)
        e_r = lax.broadcasted_iota(jnp.int32, (128, 32), 0)
        e_c = lax.broadcasted_iota(jnp.int32, (128, 32), 1)
        tile_eye = jnp.where((e_r % 32) == e_c, 1.0, 0.0).astype(BF16)
        for g in range(8):
            wg4 = wphi_buf[4 * g:4 * g + 4].reshape(128, 32)
            bdt_buf[g] = _pk(jnp.where(same_head, _dot_nt(tile_eye, wg4), 0.0).astype(BF16))

    ones = jnp.ones((16, T), BF16)

    side = []

    def take_side(count=1):
        deps = [side.pop(0) for _ in range(min(count, len(side)))]
        deps = [f() for f in deps if f is not None]
        return (jnp.concatenate(deps, axis=0) if len(deps) > 1 else deps[0]) if deps else None

    def ln_pieces(i):
        return [lambda p=p: layer_norm(i, p, LNP) for p in range(LNP)]

    def pack_wo(p):
        rows = D // LNP
        w = _pk(wo_buf[p * rows:(p + 1) * rows, :])
        wop_buf[p * rows // 2:(p + 1) * rows // 2, :] = w
        return w

    class KV:
        def __init__(self, i):
            self.i = i
            self.pk, self.vt, self.ph = {}, {}, {}

        def proj(self, r0, r1):
            halves = []
            for n in range(2):
                row = (self.i * T + n * 128) // 2
                halves.append(_dot_nt(load_wt(r0, r1, take_side()), _upk(xn_buf[row:row + 64, :])))
            return jnp.concatenate(halves, axis=1)

        def k(self, c):
            if c == 0:
                kr = self.proj(KROW - 16, KROW + MC)
                r_buf[self.i] = kr[:8, :]
                self.pk[c] = kr[16:, :]
            else:
                self.pk[c] = self.proj(KROW + c * MC, KROW + (c + 1) * MC)

        def v(self, c):
            self.vt[c] = self.proj(VROW + c * MC, VROW + (c + 1) * MC).astype(BF16)

        def phi(self, c):
            if c not in self.ph:
                pk = self.pk.pop(c)
                self.ph[c] = []
                for u in range(PC):
                    phi = _phi_pair(pk[64 * u:64 * u + 64, :])
                    z = None
                    if ZVPU:
                        z = phi[:, :128] + phi[:, 128:]
                        if self.i > 0:
                            z = z + z_acc[c * PC + u]
                        z_acc[c * PC + u] = z
                    self.ph[c].append((phi.astype(BF16), z))
            return self.ph[c]

        def g(self, c):
            vt = self.vt.pop(c)
            for u, (phi, z) in enumerate(self.phi(c)):
                lhs = vt[64 * u:64 * u + 64, :]
                if ZVPU:
                    lhs = _upk(tie(_pk(lhs), pltpu.bitcast(z, U32)))
                else:
                    lhs = jnp.concatenate([lhs, ones], axis=0)
                r = _dot_nt(lhs, phi)
                if self.i == 0:
                    g_acc[c * PC + u] = r
                else:
                    g_acc[c * PC + u] += r

    bdt_buf[8] = _pk(jnp.where(ri == ci, 1.0, 0.0).astype(BF16))
    x_cp[0].wait()
    layer_norm(0)
    t0, t1 = KV(0), KV(1)
    v_cp[0].wait()
    fold2(2 * NC)
    t0.v(0)
    x_cp[1].wait()
    layer_norm(1)
    v_cp[1].wait()
    fold2(2 * NC + 1)
    t1.v(0)
    t0.v(1)
    t1.v(1)
    wr_cp.wait()
    phi_cp.wait()
    k_cp[0].wait()
    k_cp[1].wait()
    wt_buf[D // 2:D // 2 + 8, :] = _pk(
        jnp.broadcast_to(wr_buf[...].astype(F32).reshape(1, D), (16, D)).astype(BF16))
    build_bdt()
    fold2(NC)
    fold2(NC + 1)
    t0.k(0)
    t1.k(0)
    t0.k(1)
    t0.g(0)
    t1.k(1)
    t1.g(0)
    t0.g(1)
    t1.phi(1)
    for cp in [v_cp[2], k_cp[2], v_cp[3], k_cp[3], x_cp[2]]:
        cp.wait()
    side += ln_pieces(2)
    fold2(NC + 2)
    fold2(2 * NC + 2)
    fold2(NC + 3)
    t1.g(1)
    t0.k(2)
    t1.k(2)
    t0.v(2)
    fold2(2 * NC + 3)
    t0.g(2)
    t1.v(2)
    t0.k(3)
    t1.g(2)
    t0.v(3)
    t1.k(3)
    t0.g(3)
    t1.v(3)
    t1.phi(3)
    prev = t1

    def break_cse():
        if BREAK_CSE:
            wt_buf[WTR:WTR + 8, :128] = zero_buf[...]
            wop_buf[D // 2:D // 2 + 8, :128] = zero_buf[...]

    for i in range(2, NT):
        if i == 2:
            for cp in x_cp[3:] + (q_cp if QFOLD_EARLY else []) + ([wo_cp] if PACK_EARLY else []):
                cp.wait()
        if i == 2:
            side += [None]
        if i + 1 < NT:
            side += ln_pieces(i + 1)
        elif PACK_EARLY:
            side += [lambda p=p: pack_wo(p) for p in range(LNP)]
        break_cse()
        kv = KV(i)
        for c in range(NC):
            kv.k(c)
            if c == 0:
                prev.g(NC - 1)
            else:
                kv.g(c - 1)
            kv.v(c)
        if QFOLD_EARLY and i - 2 < NC:
            fold2(i - 2)
        prev = kv
    prev.g(NC - 1)
    take_side(len(side))

    gr = lax.broadcasted_iota(jnp.int32, (GR, 128), 0)
    gc = lax.broadcasted_iota(jnp.int32, (GR, 128), 1)
    row_head = jnp.where(gr < 64, gr // 32, (gr - 64) // 8)
    keep = row_head == ((gc % 64) // 32)
    for p in range(NP):
        g_buf[p] = _pk(jnp.where(keep, g_acc[p, :GR, :], 0.0).astype(BF16))
        if ZVPU:
            zb_buf[p] = jnp.broadcast_to(jnp.sum(z_acc[p], axis=1, keepdims=True), (128, 128))
        elif DENVPU:
            zb_buf[p] = jnp.broadcast_to(g_acc[p, 64:65, :], (128, 128)).T

    r_all = _rb(r_buf[...])
    tok = (lax.broadcasted_iota(jnp.int32, (NT, 8, T), 0) * T
           + lax.broadcasted_iota(jnp.int32, (NT, 8, T), 2))
    r_max = jnp.max(r_all)
    idx = jnp.min(jnp.where(r_all == r_max, tok, S - 1))
    sel_tile = idx // T
    blk = pl.multiple_of((idx // 16) * 16, 16)

    def tile_of(j):
        return (sel_tile + 1 + j) % NT

    def last_copy(n):
        rows = pl.ds(pl.multiple_of(sel_tile * T, T), T)
        cols = pl.ds(n * 256, 256)
        return pltpu.make_async_copy(out_buf.at[rows, cols], out_hbm.at[rows, cols], sem_o.at[NT - 1 + n])

    class Q:
        def __init__(self, j):
            self.j = j
            self.row0 = tile_of(j) * (T // 2)
            self.pq = {}

        def proj(self, c, n, dep=None):
            xn = _upk(xn_buf[pl.ds(pl.multiple_of(self.row0 + n * 64, 64), 64), :])
            self.pq[c, n] = _dot_nt(load_wt(c * MC, (c + 1) * MC, dep), xn)

        def num(self, c, n):
            pq = self.pq.pop((c, n))
            parts = []
            link = Link()
            for u in range(PC):
                phi = _phi_pair(pq[64 * u:64 * u + 64, :], link)
                nd = _dot(_upk(g_buf[c * PC + u]), phi.astype(BF16))
                if DENVPU:
                    zp = phi * zb_buf[c * PC + u]
                    zp = zp[:64, :] + zp[64:, :]
                for a in range(2):
                    if DENVPU:
                        den = jnp.sum(zp[32 * a:32 * a + 32, :], axis=0, keepdims=True)
                        parts.append(nd[32 * a:32 * a + 32, :] * pl.reciprocal(den + 1e-6, approx=True))
                    else:
                        inv = pl.reciprocal(nd[64 + 8 * a:72 + 8 * a, :] + 1e-6, approx=True)
                        parts.append(nd[32 * a:32 * a + 32, :] * jnp.concatenate([inv] * 4, axis=0))
            ot = jnp.concatenate(parts, axis=0)
            o_buf[self.j % 2, n * 64:(n + 1) * 64, c * MC:(c + 1) * MC] = _pk(ot.T.astype(BF16))

    def out_cols(j, n, dep=None, upd=None):
        t = tile_of(j)
        rows = pl.ds(pl.multiple_of(t * T, T), T)
        rows2 = pl.ds(pl.multiple_of(t * (T // 2), T // 2), T // 2)
        cols = slice(n * 128, (n + 1) * 128)
        o = o_buf[j % 2]
        if dep is not None:
            o = tie(o, dep)
        s = _dot(_upk(o), _upk(wop_buf[:D // 2, cols]))
        xn = _upk(xn_buf[rows2, cols]).astype(F32)
        if upd is not None:
            xn = xn + upd[:, cols]
        out_buf[rows, cols] = (x_buf[rows, cols].astype(F32) + s * _silu(xn)).astype(BF16)

    def ffn_steps():
        st = {}
        KH = D // 2

        def apart(r):
            z = zero_buf[...]
            return pltpu.bitcast(pltpu.bitcast(r, U32) | jnp.concatenate([z, z], axis=0), F32)

        def up(w_ref, key, n, h):
            def f():
                xs = _upk(xn_buf[pl.ds(pl.multiple_of(blk // 2, 8), 8), h * KH:(h + 1) * KH])
                r = _dot(xs, w_ref[h * KH:(h + 1) * KH, n * 128:(n + 1) * 128])
                st[key, n] = apart(r) if h == 0 else st[key, n] + r
            return f

        def down(c, n):
            def f():
                if ('h', c) not in st:
                    ms = range(c * FC // 128, (c + 1) * FC // 128)
                    st['h', c] = jnp.concatenate(
                        [_silu(st.pop(('g', m))) * st.pop(('u', m)) for m in ms], axis=1).astype(BF16)
                r = _dot(st['h', c], wd_buf[c * FC:(c + 1) * FC, n * 128:(n + 1) * 128])
                st['y', n] = apart(r) if c == 0 else st['y', n] + r
            return f

        steps = []
        for c in range(F // FC + 1):
            ups = [up(w, k, m, h) for m in range(c * FC // 128, (c + 1) * FC // 128)
                   for h in range(2) for w, k in ((wg_buf, 'g'), (wu_buf, 'u'))] if c < F // FC else []
            downs = [down(c - 1, n) for n in range(D // 128)] if c > 0 else []
            while ups or downs:
                steps += ups[:2] + downs[:1]
                ups, downs = ups[2:], downs[1:]
        return steps, st

    for cp in ([] if QFOLD_EARLY else q_cp) + ([] if PACK_EARLY else [wo_cp]) + f_cp:
        cp.wait()
    if not QFOLD_EARLY:
        for j in range(NC):
            fold2(j)
    if not PACK_EARLY:
        wop_buf[:D // 2, :] = _pk(wo_buf[...])
    ffn, ffn_st = ffn_steps()

    q = Q(0)
    for c in range(NC):
        q.proj(c, 0)
        if c > 0:
            q.num(c - 1, 1)
        q.proj(c, 1)
        q.num(c, 0)
    def small():
        if ffn:
            ffn.pop(0)()

    pending = []

    def out_step():
        j, n = pending.pop(0)
        out_cols(j, n)
        if n == D // 128 - 1:
            out_copy(tile_of(j), j).start()

    for j in range(1, NT):
        qn = Q(j)
        pending += [(j - 1, n) for n in range(D // 128)]
        break_cse()
        for c in range(NC):
            first_w = True
            for tok in PATTERN:
                if tok == 'P':
                    qn.proj(c, 0)
                elif tok == 'Q':
                    qn.proj(c, 1)
                elif tok == 'f':
                    small()
                elif tok == 'n':
                    (q if c == 0 else qn).num((c - 1) % NC, 1)
                elif tok == 'm':
                    qn.num(c, 0)
                elif tok == 'W':
                    if (j, c) != (1, 0) or not first_w:
                        out_step()
                    first_w = False
        q = qn
    assert not ffn
    q.num(NC - 1, 1)
    out_step()

    y = jnp.concatenate([ffn_st['y', n] for n in range(D // 128)], axis=1)
    sub = lax.broadcasted_iota(jnp.int32, (16, D), 0)
    y_row = jnp.sum(jnp.where(sub == idx - blk, y, 0.0), axis=0, keepdims=True)
    gate = 1.0 / (1.0 + jnp.exp(-jnp.full((1, D), r_max, F32)))
    trow = lax.broadcasted_iota(jnp.int32, (T, D), 0)
    upd = jnp.where(trow == idx - sel_tile * T, y_row * gate, 0.0)
    for n in range(D // 128):
        out_cols(NT - 1, n, None, upd)
        if n % 2 == 1:
            last_copy(n // 2).start()
    for j in range(NT - 1):
        out_copy(tile_of(j), j).wait()
    for n in range(D // 256):
        last_copy(n).wait()


@jax.jit
def pallas_recurrent_scan__linear_kernel_hedgehog__moe_arch_mod__prompt_kernel(
    A_x: jax.Array,
    A_wqkv: jax.Array,
    A_w_phi: jax.Array,
    A_wo: jax.Array,
    B_x: jax.Array,
    B_w_r: jax.Array,
    B_w_gate: jax.Array,
    B_w_up: jax.Array,
    B_w_down: jax.Array,
):
    del B_x
    any_spec = pl.BlockSpec(memory_space=pl.ANY)
    out = pl.pallas_call(
        _kernel,
        out_shape=jax.ShapeDtypeStruct((S, D), BF16),
        in_specs=[any_spec] * 8,
        out_specs=any_spec,
        scratch_shapes=[
            pltpu.VMEM((S, D), BF16),
            pltpu.VMEM((S // 2, D), U32),
            pltpu.VMEM((3 * NC, D, MC), BF16),
            pltpu.VMEM((WTR + 8, D), U32),
            pltpu.VMEM((H, DH, DH), BF16),
            pltpu.VMEM((D,), BF16),
            pltpu.VMEM((D, D), BF16),
            pltpu.VMEM((D, F), BF16),
            pltpu.VMEM((D, F), BF16),
            pltpu.VMEM((F, D), BF16),
            pltpu.VMEM((9, 64, 128), U32),
            pltpu.VMEM((NP, GA, 128), F32),
            pltpu.VMEM((NP, GR // 2, 128), U32),
            pltpu.VMEM((NT, 8, T), F32),
            pltpu.VMEM((2, T // 2, D), U32),
            pltpu.VMEM((S, D), BF16),
            pltpu.VMEM((8, 128), U32),
            pltpu.VMEM((D // 2 + 8, D), U32),
            pltpu.VMEM((NP, 128, 128), F32),
            pltpu.VMEM((NP, 128, 128), F32),
            pltpu.SemaphoreType.DMA((NT,)),
            pltpu.SemaphoreType.DMA((3 * NC,)),
            pltpu.SemaphoreType.DMA((6,)),
            pltpu.SemaphoreType.DMA((NT + 3,)),
        ],
        compiler_params=pltpu.CompilerParams(
            vmem_limit_bytes=100 * 1024 * 1024,
            disable_bounds_checks=True,
            disable_semaphore_checks=True,
        ),
        name="hedgehog_mod",
    )(A_x.reshape(S, D), A_wqkv, A_w_phi, A_wo, B_w_r, B_w_gate, B_w_up, B_w_down)
    return out.reshape(1, S, D)
```

```python
import jax
import jax.numpy as jnp
from jax import lax
import jax.experimental.pallas as pl
import jax.experimental.pallas.tpu as pltpu

S, D, H, DH, F = 2048, 1024, 32, 32, 3584
T = 256
NT = S // T
MC = 256
NC = D // MC
PC = MC // 64
NP = H // 2
FC = 512
LNP = 16
KROW = D + 16
VROW = KROW + D
WTR = (VROW + D) // 2
QFOLD_EARLY = False
PATTERN = "PfQfnfWfmfWf"
DENVPU = True
ZVPU = True
VXLU = (1, 2, 3)
VX32 = True
GA = 64 if ZVPU else 80
GR = 64 if DENVPU else 80
LOG2E = 1.4426950408889634
EPS_LN = 1.0013580322265625e-05
F32 = jnp.float32
BF16 = jnp.bfloat16
U32 = jnp.uint32

_NT_DIMS = (((1,), (1,)), ((), ()))


def _dot_nt(a, b):
    return lax.dot_general(a, b, _NT_DIMS, preferred_element_type=F32)


def _dot(a, b):
    return jnp.dot(a, b, preferred_element_type=F32)


def _rb(x):
    return x.astype(BF16).astype(F32)


def _pk(x):
    return pltpu.bitcast(x, U32)


def _upk(x):
    return pltpu.bitcast(x, BF16)


def _phi_pair(p, link=None):
    pos, neg = [], []
    for a in range(2):
        ph = p[32 * a:32 * a + 32, :]
        mx = jnp.max(ph, axis=0, keepdims=True)
        mn = jnp.min(ph, axis=0, keepdims=True)
        if link is not None:
            mx, mn = link.start(mx, mn)
        ep = jnp.exp2(ph - mx)
        en = jnp.exp2(mn - ph)
        pos.append(ep * pl.reciprocal(jnp.sum(ep, axis=0, keepdims=True), approx=True))
        neg.append(en * pl.reciprocal(jnp.sum(en, axis=0, keepdims=True), approx=True))
        if link is not None:
            link.done(pos[-1], neg[-1])
    return jnp.concatenate(pos + neg, axis=0)


def _silu(x):
    h = 0.5 * x
    return h + h * jnp.tanh(h)


def _kernel(x_hbm, wqkv_hbm, wphi_hbm, wo_hbm, wr_hbm, wg_hbm, wu_hbm, wd_hbm, out_hbm,
            x_buf, xn_buf, w_buf, wt_buf, wphi_buf, wr_buf, wo_buf, wg_buf, wu_buf, wd_buf,
            bdt_buf, g_acc, g_buf, r_buf, o_buf, out_buf, zero_buf, z_acc, zb_buf,
            sem_x, sem_w, sem_s, sem_o):
    x_cp = [pltpu.make_async_copy(x_hbm.at[pl.ds(i * T, T), :], x_buf.at[pl.ds(i * T, T), :], sem_x.at[i])
            for i in range(NT)]
    w_cp = [pltpu.make_async_copy(wqkv_hbm.at[:, pl.ds(j * MC, MC)], w_buf.at[j].bitcast(BF16), sem_w.at[j])
            for j in range(3 * NC)]
    q_cp, k_cp, v_cp = w_cp[:NC], w_cp[NC:2 * NC], w_cp[2 * NC:]
    phi_cp = pltpu.make_async_copy(wphi_hbm, wphi_buf, sem_s.at[0])
    wr_cp = pltpu.make_async_copy(wr_hbm, wr_buf, sem_s.at[1])
    wo_cp = pltpu.make_async_copy(wo_hbm, wo_buf.bitcast(BF16), sem_s.at[2])
    f_cp = [pltpu.make_async_copy(wg_hbm, wg_buf.bitcast(BF16), sem_s.at[3]),
            pltpu.make_async_copy(wu_hbm, wu_buf.bitcast(BF16), sem_s.at[4]),
            pltpu.make_async_copy(wd_hbm, wd_buf.bitcast(BF16), sem_s.at[5])]

    def out_copy(t, j):
        rows = pl.ds(pl.multiple_of(t * T, T), T)
        return pltpu.make_async_copy(out_buf.at[rows, :], out_hbm.at[rows, :], sem_o.at[j])

    copies = [x_cp[0], v_cp[0], x_cp[1], v_cp[1], wr_cp, phi_cp, k_cp[0], k_cp[1], v_cp[2], k_cp[2],
              v_cp[3], k_cp[3]] + x_cp[2:] + q_cp + [wo_cp] + f_cp

    def start_all(j, carry):
        for k, cp in enumerate(copies):
            pl.when((k + 2) * j == j)(cp.start)
        zero_buf[...] = jnp.zeros_like(zero_buf)
        return carry

    lax.fori_loop(0, 2, start_all, 0)

    def tie(w, dep):
        acc = None
        for r in range(0, dep.shape[0], 8):
            for c in range(0, dep.shape[1], 128):
                piece = dep[r:r + 8, c:c + 128]
                acc = piece if acc is None else acc | piece
        first = w[:8, :128] | (acc & zero_buf[...])
        top = jnp.concatenate([first, w[:8, 128:]], axis=1)
        return jnp.concatenate([top, w[8:, :]], axis=0)

    def after(x, dep):
        z = pltpu.bitcast(dep, U32)[:x.shape[0], :] & zero_buf[:x.shape[0], :]
        return pltpu.bitcast(pltpu.bitcast(x, U32) | z, F32)

    class Link:
        def __init__(self):
            self.prev = None

        def start(self, mx, mn):
            if self.prev is None:
                return mx, mn
            return after(mx, self.prev[0]), after(mn, self.prev[1])

        def done(self, pos, neg):
            self.prev = (pos[24:32, :], neg[24:32, :])

    def layer_norm(i, piece=0, npieces=1):
        n = T // npieces
        r0 = i * T + piece * n
        x = x_buf[r0:r0 + n, :].astype(F32)
        m = jnp.mean(x, axis=-1, keepdims=True)
        mb = _rb(m)
        d = x - mb
        v = jnp.mean(d * d, axis=-1, keepdims=True) - (m - mb) * (m - mb)
        den = _rb(jnp.sqrt(_rb(_rb(v) + EPS_LN)))
        xn = _pk((_rb(d) * (1.0 / den)).astype(BF16))
        xn_buf[r0 // 2:(r0 + n) // 2, :] = xn
        return xn

    def load_wt(r0, r1, dep=None):
        w = wt_buf[r0 // 2:r1 // 2, :]
        if dep is not None:
            w = tie(w, dep)
        return _upk(w)

    def fold(j, u):
        w = _upk(w_buf[j, :, u * 128:(u + 1) * 128])
        if j < 2 * NC:
            r = _dot_nt(_upk(bdt_buf[(2 * j + u) % 8]), w) * LOG2E
        elif j - 2 * NC in VXLU:
            r = w.astype(F32).T if VX32 else w.T
        else:
            r = _dot_nt(_upk(bdt_buf[8]), w)
        row = (j * MC + u * 128 + (16 if j >= NC else 0)) // 2
        wt_buf[row:row + 64, :] = _pk(r.astype(BF16))

    def fold2(j):
        fold(j, 0)
        fold(j, 1)

    ri = lax.broadcasted_iota(jnp.int32, (128, 128), 0)
    ci = lax.broadcasted_iota(jnp.int32, (128, 128), 1)

    def build_bdt():
        same_head = (ri // 32) == (ci // 32)
        e_r = lax.broadcasted_iota(jnp.int32, (128, 32), 0)
        e_c = lax.broadcasted_iota(jnp.int32, (128, 32), 1)
        tile_eye = jnp.where((e_r % 32) == e_c, 1.0, 0.0).astype(BF16)
        for g in range(8):
            wg4 = wphi_buf[4 * g:4 * g + 4].reshape(128, 32)
            bdt_buf[g] = _pk(jnp.where(same_head, _dot_nt(tile_eye, wg4), 0.0).astype(BF16))

    ones = jnp.ones((16, T), BF16)

    side = []

    def take_side(count=1):
        deps = [side.pop(0) for _ in range(min(count, len(side)))]
        deps = [f() for f in deps if f is not None]
        return (jnp.concatenate(deps, axis=0) if len(deps) > 1 else deps[0]) if deps else None

    def ln_pieces(i):
        return [lambda p=p: layer_norm(i, p, LNP) for p in range(LNP)]

    class KV:
        def __init__(self, i):
            self.i = i
            self.pk, self.vt, self.ph = {}, {}, {}

        def proj(self, r0, r1):
            halves = []
            for n in range(2):
                row = (self.i * T + n * 128) // 2
                halves.append(_dot_nt(load_wt(r0, r1, take_side()), _upk(xn_buf[row:row + 64, :])))
            return jnp.concatenate(halves, axis=1)

        def k(self, c):
            if c == 0:
                kr = self.proj(KROW - 16, KROW + MC)
                r_buf[self.i] = kr[:8, :]
                self.pk[c] = kr[16:, :]
            else:
                self.pk[c] = self.proj(KROW + c * MC, KROW + (c + 1) * MC)

        def v(self, c):
            self.vt[c] = self.proj(VROW + c * MC, VROW + (c + 1) * MC).astype(BF16)

        def phi(self, c):
            if c not in self.ph:
                pk = self.pk.pop(c)
                self.ph[c] = []
                for u in range(PC):
                    phi = _phi_pair(pk[64 * u:64 * u + 64, :])
                    z = None
                    if ZVPU:
                        z = phi[:, :128] + phi[:, 128:]
                        if self.i > 0:
                            z = z + z_acc[c * PC + u]
                        z_acc[c * PC + u] = z
                    self.ph[c].append((phi.astype(BF16), z))
            return self.ph[c]

        def g(self, c):
            vt = self.vt.pop(c)
            for u, (phi, z) in enumerate(self.phi(c)):
                lhs = vt[64 * u:64 * u + 64, :]
                if ZVPU:
                    lhs = _upk(tie(_pk(lhs), pltpu.bitcast(z, U32)))
                else:
                    lhs = jnp.concatenate([lhs, ones], axis=0)
                r = _dot_nt(lhs, phi)
                if self.i == 0:
                    g_acc[c * PC + u] = r
                else:
                    g_acc[c * PC + u] += r

    bdt_buf[8] = _pk(jnp.where(ri == ci, 1.0, 0.0).astype(BF16))
    x_cp[0].wait()
    layer_norm(0)
    t0, t1 = KV(0), KV(1)
    v_cp[0].wait()
    fold2(2 * NC)
    t0.v(0)
    x_cp[1].wait()
    layer_norm(1)
    v_cp[1].wait()
    fold2(2 * NC + 1)
    t1.v(0)
    t0.v(1)
    t1.v(1)
    wr_cp.wait()
    phi_cp.wait()
    k_cp[0].wait()
    k_cp[1].wait()
    wt_buf[D // 2:D // 2 + 8, :] = _pk(
        jnp.broadcast_to(wr_buf[...].astype(F32).reshape(1, D), (16, D)).astype(BF16))
    build_bdt()
    fold2(NC)
    fold2(NC + 1)
    t0.k(0)
    t1.k(0)
    t0.k(1)
    t0.g(0)
    t1.k(1)
    t1.g(0)
    t0.g(1)
    t1.phi(1)
    for cp in [v_cp[2], k_cp[2], v_cp[3], k_cp[3], x_cp[2]]:
        cp.wait()
    side += ln_pieces(2)
    fold2(NC + 2)
    fold2(2 * NC + 2)
    fold2(NC + 3)
    t1.g(1)
    t0.k(2)
    t1.k(2)
    t0.v(2)
    fold2(2 * NC + 3)
    t0.g(2)
    t1.v(2)
    t0.k(3)
    t1.g(2)
    t0.v(3)
    t1.k(3)
    t0.g(3)
    t1.v(3)
    t1.phi(3)
    prev = t1

    for i in range(2, NT):
        if i == 2:
            for cp in x_cp[3:] + (q_cp if QFOLD_EARLY else []):
                cp.wait()
        if i == 2:
            side += [None]
        if i + 1 < NT:
            side += ln_pieces(i + 1)
        kv = KV(i)
        for c in range(NC):
            kv.k(c)
            if c == 0:
                prev.g(NC - 1)
            else:
                kv.g(c - 1)
            kv.v(c)
        if QFOLD_EARLY and i - 2 < NC:
            fold2(i - 2)
        prev = kv
    prev.g(NC - 1)
    take_side(len(side))

    gr = lax.broadcasted_iota(jnp.int32, (GR, 128), 0)
    gc = lax.broadcasted_iota(jnp.int32, (GR, 128), 1)
    row_head = jnp.where(gr < 64, gr // 32, (gr - 64) // 8)
    keep = row_head == ((gc % 64) // 32)
    for p in range(NP):
        g_buf[p] = _pk(jnp.where(keep, g_acc[p, :GR, :], 0.0).astype(BF16))
        if ZVPU:
            zb_buf[p] = jnp.broadcast_to(jnp.sum(z_acc[p], axis=1, keepdims=True), (128, 128))
        elif DENVPU:
            zb_buf[p] = jnp.broadcast_to(g_acc[p, 64:65, :], (128, 128)).T

    r_all = _rb(r_buf[...])
    tok = (lax.broadcasted_iota(jnp.int32, (NT, 8, T), 0) * T
           + lax.broadcasted_iota(jnp.int32, (NT, 8, T), 2))
    r_max = jnp.max(r_all)
    idx = jnp.min(jnp.where(r_all == r_max, tok, S - 1))
    sel_tile = idx // T
    blk = pl.multiple_of((idx // 16) * 16, 16)

    def tile_of(j):
        return (sel_tile + 1 + j) % NT

    def last_copy(n):
        rows = pl.ds(pl.multiple_of(sel_tile * T, T), T)
        cols = pl.ds(n * 256, 256)
        return pltpu.make_async_copy(out_buf.at[rows, cols], out_hbm.at[rows, cols], sem_o.at[NT - 1 + n])

    class Q:
        def __init__(self, j):
            self.j = j
            self.row0 = tile_of(j) * (T // 2)
            self.pq = {}

        def proj(self, c, n, dep=None):
            xn = _upk(xn_buf[pl.ds(pl.multiple_of(self.row0 + n * 64, 64), 64), :])
            self.pq[c, n] = _dot_nt(load_wt(c * MC, (c + 1) * MC, dep), xn)

        def num(self, c, n):
            pq = self.pq.pop((c, n))
            parts = []
            link = Link()
            for u in range(PC):
                phi = _phi_pair(pq[64 * u:64 * u + 64, :], link)
                nd = _dot(_upk(g_buf[c * PC + u]), phi.astype(BF16))
                if DENVPU:
                    zp = phi * zb_buf[c * PC + u]
                    zp = zp[:64, :] + zp[64:, :]
                for a in range(2):
                    if DENVPU:
                        den = jnp.sum(zp[32 * a:32 * a + 32, :], axis=0, keepdims=True)
                        parts.append(nd[32 * a:32 * a + 32, :] * pl.reciprocal(den + 1e-6, approx=True))
                    else:
                        inv = pl.reciprocal(nd[64 + 8 * a:72 + 8 * a, :] + 1e-6, approx=True)
                        parts.append(nd[32 * a:32 * a + 32, :] * jnp.concatenate([inv] * 4, axis=0))
            ot = jnp.concatenate(parts, axis=0)
            o_buf[self.j % 2, n * 64:(n + 1) * 64, c * MC:(c + 1) * MC] = _pk(ot.T.astype(BF16))

    def out_cols(j, n, dep=None, upd=None):
        t = tile_of(j)
        rows = pl.ds(pl.multiple_of(t * T, T), T)
        rows2 = pl.ds(pl.multiple_of(t * (T // 2), T // 2), T // 2)
        cols = slice(n * 128, (n + 1) * 128)
        o = o_buf[j % 2]
        if dep is not None:
            o = tie(o, dep)
        s = _dot(_upk(o), _upk(wo_buf[:, cols]))
        xn = _upk(xn_buf[rows2, cols]).astype(F32)
        if upd is not None:
            xn = xn + upd[:, cols]
        out_buf[rows, cols] = (x_buf[rows, cols].astype(F32) + s * _silu(xn)).astype(BF16)

    def ffn_steps():
        st = {}
        KH = D // 2

        def apart(r):
            z = zero_buf[...]
            return pltpu.bitcast(pltpu.bitcast(r, U32) | jnp.concatenate([z, z], axis=0), F32)

        def up(w_ref, key, n, h):
            def f():
                xs = _upk(xn_buf[pl.ds(pl.multiple_of(blk // 2, 8), 8), h * KH:(h + 1) * KH])
                r = _dot(xs, _upk(w_ref[h * KH // 2:(h + 1) * KH // 2, n * 128:(n + 1) * 128]))
                st[key, n] = apart(r) if h == 0 else st[key, n] + r
            return f

        def down(c, n):
            def f():
                if ('h', c) not in st:
                    ms = range(c * FC // 128, (c + 1) * FC // 128)
                    st['h', c] = jnp.concatenate(
                        [_silu(st.pop(('g', m))) * st.pop(('u', m)) for m in ms], axis=1).astype(BF16)
                r = _dot(st['h', c], _upk(wd_buf[c * FC // 2:(c + 1) * FC // 2, n * 128:(n + 1) * 128]))
                st['y', n] = apart(r) if c == 0 else st['y', n] + r
            return f

        steps = []
        for c in range(F // FC + 1):
            ups = [up(w, k, m, h) for m in range(c * FC // 128, (c + 1) * FC // 128)
                   for h in range(2) for w, k in ((wg_buf, 'g'), (wu_buf, 'u'))] if c < F // FC else []
            downs = [down(c - 1, n) for n in range(D // 128)] if c > 0 else []
            while ups or downs:
                steps += ups[:2] + downs[:1]
                ups, downs = ups[2:], downs[1:]
        return steps, st

    for cp in ([] if QFOLD_EARLY else q_cp) + [wo_cp] + f_cp:
        cp.wait()
    if not QFOLD_EARLY:
        for j in range(NC):
            fold2(j)
    ffn, ffn_st = ffn_steps()

    q = Q(0)
    for c in range(NC):
        q.proj(c, 0)
        if c > 0:
            q.num(c - 1, 1)
        q.proj(c, 1)
        q.num(c, 0)
    def small():
        if ffn:
            ffn.pop(0)()

    pending = []

    def out_step():
        j, n = pending.pop(0)
        out_cols(j, n)
        if n == D // 128 - 1:
            out_copy(tile_of(j), j).start()

    for j in range(1, NT):
        qn = Q(j)
        pending += [(j - 1, n) for n in range(D // 128)]
        for c in range(NC):
            first_w = True
            for tok in PATTERN:
                if tok == 'P':
                    qn.proj(c, 0)
                elif tok == 'Q':
                    qn.proj(c, 1)
                elif tok == 'f':
                    small()
                elif tok == 'n':
                    (q if c == 0 else qn).num((c - 1) % NC, 1)
                elif tok == 'm':
                    qn.num(c, 0)
                elif tok == 'W':
                    if (j, c) != (1, 0) or not first_w:
                        out_step()
                    first_w = False
        q = qn
    assert not ffn
    q.num(NC - 1, 1)
    out_step()

    y = jnp.concatenate([ffn_st['y', n] for n in range(D // 128)], axis=1)
    sub = lax.broadcasted_iota(jnp.int32, (16, D), 0)
    y_row = jnp.sum(jnp.where(sub == idx - blk, y, 0.0), axis=0, keepdims=True)
    gate = 1.0 / (1.0 + jnp.exp(-jnp.full((1, D), r_max, F32)))
    trow = lax.broadcasted_iota(jnp.int32, (T, D), 0)
    upd = jnp.where(trow == idx - sel_tile * T, y_row * gate, 0.0)
    for n in range(D // 128):
        out_cols(NT - 1, n, None, upd)
        if n % 2 == 1:
            last_copy(n // 2).start()
    for j in range(NT - 1):
        out_copy(tile_of(j), j).wait()
    for n in range(D // 256):
        last_copy(n).wait()


@jax.jit
def pallas_recurrent_scan__linear_kernel_hedgehog__moe_arch_mod__prompt_kernel(
    A_x: jax.Array,
    A_wqkv: jax.Array,
    A_w_phi: jax.Array,
    A_wo: jax.Array,
    B_x: jax.Array,
    B_w_r: jax.Array,
    B_w_gate: jax.Array,
    B_w_up: jax.Array,
    B_w_down: jax.Array,
):
    del B_x
    any_spec = pl.BlockSpec(memory_space=pl.ANY)
    out = pl.pallas_call(
        _kernel,
        out_shape=jax.ShapeDtypeStruct((S, D), BF16),
        in_specs=[any_spec] * 8,
        out_specs=any_spec,
        scratch_shapes=[
            pltpu.VMEM((S, D), BF16),
            pltpu.VMEM((S // 2, D), U32),
            pltpu.VMEM((3 * NC, D // 2, MC), U32),
            pltpu.VMEM((WTR, D), U32),
            pltpu.VMEM((H, DH, DH), BF16),
            pltpu.VMEM((D,), BF16),
            pltpu.VMEM((D // 2, D), U32),
            pltpu.VMEM((D // 2, F), U32),
            pltpu.VMEM((D // 2, F), U32),
            pltpu.VMEM((F // 2, D), U32),
            pltpu.VMEM((9, 64, 128), U32),
            pltpu.VMEM((NP, GA, 128), F32),
            pltpu.VMEM((NP, GR // 2, 128), U32),
            pltpu.VMEM((NT, 8, T), F32),
            pltpu.VMEM((2, T // 2, D), U32),
            pltpu.VMEM((S, D), BF16),
            pltpu.VMEM((8, 128), U32),
            pltpu.VMEM((NP, 128, 128), F32),
            pltpu.VMEM((NP, 128, 128), F32),
            pltpu.SemaphoreType.DMA((NT,)),
            pltpu.SemaphoreType.DMA((3 * NC,)),
            pltpu.SemaphoreType.DMA((6,)),
            pltpu.SemaphoreType.DMA((NT + 3,)),
        ],
        compiler_params=pltpu.CompilerParams(
            vmem_limit_bytes=100 * 1024 * 1024,
            disable_bounds_checks=True,
            disable_semaphore_checks=True,
        ),
        name="hedgehog_mod",
    )(A_x.reshape(S, D), A_wqkv, A_w_phi, A_wo, B_w_r, B_w_gate, B_w_up, B_w_down)
    return out.reshape(1, S, D)
```

```python
import jax
import jax.numpy as jnp
from jax import lax
import jax.experimental.pallas as pl
import jax.experimental.pallas.tpu as pltpu

S, D, H, DH, F = 2048, 1024, 32, 32, 3584
T = 256
NT = S // T
MC = 256
NC = D // MC
PC = MC // 64
NP = H // 2
FC = 512
LNP = 16
QFOLD_EARLY = False
PATTERN = "PfQfnfWfmfWf"
DENVPU = True
ZVPU = True
VXLU = (1, 2, 3)
VX32 = True
RVPU = False
LASTW = 128
SPLIT = True
KROW = D if RVPU else D + 16
VROW = KROW + D
WTR = (VROW + D) // 2
GA = 64 if ZVPU else 80
GR = 64 if DENVPU else 80
LOG2E = 1.4426950408889634
EPS_LN = 1.0013580322265625e-05
F32 = jnp.float32
BF16 = jnp.bfloat16
U32 = jnp.uint32

_NT_DIMS = (((1,), (1,)), ((), ()))


def _dot_nt(a, b):
    return lax.dot_general(a, b, _NT_DIMS, preferred_element_type=F32)


def _dot(a, b):
    return jnp.dot(a, b, preferred_element_type=F32)


def _rb(x):
    return x.astype(BF16).astype(F32)


def _pk(x):
    return pltpu.bitcast(x, U32)


def _upk(x):
    return pltpu.bitcast(x, BF16)


def _phi_pair(p, link=None):
    pos, neg = [], []
    for a in range(2):
        ph = p[32 * a:32 * a + 32, :]
        mx = jnp.max(ph, axis=0, keepdims=True)
        mn = jnp.min(ph, axis=0, keepdims=True)
        if link is not None:
            mx, mn = link.start(mx, mn)
        ep = jnp.exp2(ph - mx)
        en = jnp.exp2(mn - ph)
        pos.append(ep * pl.reciprocal(jnp.sum(ep, axis=0, keepdims=True), approx=True))
        neg.append(en * pl.reciprocal(jnp.sum(en, axis=0, keepdims=True), approx=True))
        if link is not None:
            link.done(pos[-1], neg[-1])
    return jnp.concatenate(pos + neg, axis=0)


def _silu(x):
    h = 0.5 * x
    return h + h * jnp.tanh(h)


def _kernel(x_hbm, wqkv_hbm, wphi_hbm, wo_hbm, wr_hbm, wg_hbm, wu_hbm, wd_hbm, out_hbm,
            x_buf, xn_buf, w_buf, wt_buf, wphi_buf, wr_buf, wo_buf, wg_buf, wu_buf, wd_buf,
            bdt_buf, g_acc, g_buf, r_buf, o_buf, out_buf, zero_buf, z_acc, zb_buf, wrf_buf,
            sem_x, sem_w, sem_s, sem_o):
    x_cp = [pltpu.make_async_copy(x_hbm.at[pl.ds(i * T, T), :], x_buf.at[pl.ds(i * T, T), :], sem_x.at[i])
            for i in range(NT)]
    w_cp = [pltpu.make_async_copy(wqkv_hbm.at[:, pl.ds(j * MC, MC)], w_buf.at[j].bitcast(BF16), sem_w.at[j])
            for j in range(3 * NC)]
    q_cp, k_cp, v_cp = w_cp[:NC], w_cp[NC:2 * NC], w_cp[2 * NC:]
    phi_cp = pltpu.make_async_copy(wphi_hbm, wphi_buf, sem_s.at[0])
    wr_cp = pltpu.make_async_copy(wr_hbm, wr_buf, sem_s.at[1])
    wo_cp = pltpu.make_async_copy(wo_hbm, wo_buf.bitcast(BF16), sem_s.at[2])
    f_cp = [pltpu.make_async_copy(wg_hbm, wg_buf.bitcast(BF16), sem_s.at[3]),
            pltpu.make_async_copy(wu_hbm, wu_buf.bitcast(BF16), sem_s.at[4]),
            pltpu.make_async_copy(wd_hbm, wd_buf.bitcast(BF16), sem_s.at[5])]

    def out_copy(t, j):
        rows = pl.ds(pl.multiple_of(t * T, T), T)
        return pltpu.make_async_copy(out_buf.at[rows, :], out_hbm.at[rows, :], sem_o.at[j])

    copies = [x_cp[0], wr_cp, v_cp[0], x_cp[1], v_cp[1], phi_cp, k_cp[0], k_cp[1], v_cp[2], k_cp[2],
              v_cp[3], k_cp[3]] + x_cp[2:] + q_cp + [wo_cp] + f_cp

    def start_all(j, carry):
        for k, cp in enumerate(copies):
            pl.when((k + 2) * j == j)(cp.start)
        zero_buf[...] = jnp.zeros_like(zero_buf)
        return carry

    lax.fori_loop(0, 2, start_all, 0)

    def fence(d):
        acc = None
        for r in range(0, d.shape[0], 8):
            for c in range(0, d.shape[1], 128):
                piece = d[r:r + 8, c:c + 128]
                acc = piece if acc is None else acc | piece
        return acc & zero_buf[...]

    def tie(w, dep):
        top = [w[:8, c:c + 128] for c in range(0, w.shape[1], 128)]
        for k, d in enumerate(dep):
            k = k * len(top) // 2 if SPLIT else 0
            top[k] = top[k] | fence(d)
        return jnp.concatenate([jnp.concatenate(top, axis=1), w[8:, :]], axis=0)

    def after(x, dep):
        z = pltpu.bitcast(dep, U32)[:x.shape[0], :] & zero_buf[:x.shape[0], :]
        return pltpu.bitcast(pltpu.bitcast(x, U32) | z, F32)

    class Link:
        def __init__(self):
            self.prev = None

        def start(self, mx, mn):
            if self.prev is None:
                return mx, mn
            return after(mx, self.prev[0]), after(mn, self.prev[1])

        def done(self, pos, neg):
            self.prev = (pos[24:32, :], neg[24:32, :])

    def score(xn, r0):
        r = jnp.sum(xn.astype(F32) * wrf_buf[...], axis=-1, keepdims=True)
        r = jnp.broadcast_to(r, (xn.shape[0], 128))
        lane = lax.broadcasted_iota(jnp.int32, (8, 128), 1)
        for g in range(xn.shape[0] // 8):
            gg = r0 // 8 + g
            pltpu.store(r_buf.at[gg // 128], r[8 * g:8 * g + 8, :], mask=lane == gg % 128)
        return pltpu.bitcast(r, U32)

    def layer_norm(i, piece=0, npieces=1):
        n = T // npieces
        r0 = i * T + piece * n
        x = x_buf[r0:r0 + n, :].astype(F32)
        m = jnp.mean(x, axis=-1, keepdims=True)
        mb = _rb(m)
        d = x - mb
        v = jnp.mean(d * d, axis=-1, keepdims=True) - (m - mb) * (m - mb)
        den = _rb(jnp.sqrt(_rb(_rb(v) + EPS_LN)))
        inv = pl.reciprocal(den, approx=True)
        inv = inv * (2.0 - den * inv)
        xn = (_rb(d) * inv).astype(BF16)
        xn_buf[r0 // 2:(r0 + n) // 2, :] = _pk(xn)
        return [_pk(xn)] + ([score(xn, r0)] if RVPU and npieces > 1 else [])

    def score_pieces(r0, r1, n):
        return [lambda r=r: [score(_upk(xn_buf[r // 2:(r + n) // 2, :]), r)] for r in range(r0, r1, n)]

    def load_wt(r0, r1, dep=None):
        w = wt_buf[r0 // 2:r1 // 2, :]
        if dep is not None:
            w = tie(w, dep)
        return _upk(w)

    def fold(j, u):
        w = _upk(w_buf[j, :, u * 128:(u + 1) * 128])
        if j < 2 * NC:
            r = _dot_nt(_upk(bdt_buf[(2 * j + u) % 8]), w) * LOG2E
        elif j - 2 * NC in VXLU:
            r = w.astype(F32).T if VX32 else w.T
        else:
            r = _dot_nt(_upk(bdt_buf[8]), w)
        row = (j * MC + u * 128 + (KROW - D if j >= NC else 0)) // 2
        wt_buf[row:row + 64, :] = _pk(r.astype(BF16))

    def fold2(j):
        fold(j, 0)
        fold(j, 1)

    ri = lax.broadcasted_iota(jnp.int32, (128, 128), 0)
    ci = lax.broadcasted_iota(jnp.int32, (128, 128), 1)

    def build_bdt():
        same_head = (ri // 32) == (ci // 32)
        e_r = lax.broadcasted_iota(jnp.int32, (128, 32), 0)
        e_c = lax.broadcasted_iota(jnp.int32, (128, 32), 1)
        tile_eye = jnp.where((e_r % 32) == e_c, 1.0, 0.0).astype(BF16)
        for g in range(8):
            wg4 = wphi_buf[4 * g:4 * g + 4].reshape(128, 32)
            bdt_buf[g] = _pk(jnp.where(same_head, _dot_nt(tile_eye, wg4), 0.0).astype(BF16))

    ones = jnp.ones((16, T), BF16)

    side = []

    def take_side(count=1):
        deps = [side.pop(0) for _ in range(min(count, len(side)))]
        deps = [d for f in deps if f is not None for d in f()]
        return deps or None

    def ln_pieces(i):
        return [lambda p=p: layer_norm(i, p, LNP) for p in range(LNP)]

    class KV:
        def __init__(self, i):
            self.i = i
            self.pk, self.vt, self.ph = {}, {}, {}

        def proj(self, r0, r1):
            halves = []
            for n in range(2):
                row = (self.i * T + n * 128) // 2
                halves.append(_dot_nt(load_wt(r0, r1, take_side()), _upk(xn_buf[row:row + 64, :])))
            return jnp.concatenate(halves, axis=1)

        def k(self, c):
            if c == 0 and not RVPU:
                kr = self.proj(KROW - 16, KROW + MC)
                r_buf[self.i] = kr[:8, :]
                self.pk[c] = kr[16:, :]
            else:
                self.pk[c] = self.proj(KROW + c * MC, KROW + (c + 1) * MC)

        def v(self, c):
            self.vt[c] = self.proj(VROW + c * MC, VROW + (c + 1) * MC).astype(BF16)

        def phi(self, c):
            if c not in self.ph:
                pk = self.pk.pop(c)
                self.ph[c] = []
                for u in range(PC):
                    phi = _phi_pair(pk[64 * u:64 * u + 64, :])
                    z = None
                    if ZVPU:
                        z = phi[:, :128] + phi[:, 128:]
                        if self.i > 0:
                            z = z + z_acc[c * PC + u]
                        z_acc[c * PC + u] = z
                    self.ph[c].append((phi.astype(BF16), z))
            return self.ph[c]

        def g(self, c):
            vt = self.vt.pop(c)
            for u, (phi, z) in enumerate(self.phi(c)):
                lhs = vt[64 * u:64 * u + 64, :]
                if ZVPU:
                    lhs = _upk(tie(_pk(lhs), [pltpu.bitcast(z, U32)]))
                else:
                    lhs = jnp.concatenate([lhs, ones], axis=0)
                r = _dot_nt(lhs, phi)
                if self.i == 0:
                    g_acc[c * PC + u] = r
                else:
                    g_acc[c * PC + u] += r

    bdt_buf[8] = _pk(jnp.where(ri == ci, 1.0, 0.0).astype(BF16))
    x_cp[0].wait()
    layer_norm(0)
    t0, t1 = KV(0), KV(1)
    wr_cp.wait()
    v_cp[0].wait()
    wrf_buf[...] = wr_buf[...].astype(F32).reshape(1, D)
    fold2(2 * NC)
    t0.v(0)
    x_cp[1].wait()
    layer_norm(1)
    v_cp[1].wait()
    fold2(2 * NC + 1)
    t1.v(0)
    t0.v(1)
    t1.v(1)
    phi_cp.wait()
    k_cp[0].wait()
    k_cp[1].wait()
    if RVPU:
        side += [None] + score_pieces(0, 2 * T, 64)
    else:
        wt_buf[D // 2:D // 2 + 8, :] = _pk(
            jnp.broadcast_to(wr_buf[...].astype(F32).reshape(1, D), (16, D)).astype(BF16))
    build_bdt()
    fold2(NC)
    fold2(NC + 1)
    t0.k(0)
    t1.k(0)
    t0.k(1)
    t0.g(0)
    t1.k(1)
    t1.g(0)
    t0.g(1)
    t1.phi(1)
    take_side(len(side))
    for cp in [v_cp[2], k_cp[2], v_cp[3], k_cp[3], x_cp[2]]:
        cp.wait()
    side += ln_pieces(2)
    fold2(NC + 2)
    fold2(2 * NC + 2)
    fold2(NC + 3)
    t1.g(1)
    t0.k(2)
    t1.k(2)
    t0.v(2)
    fold2(2 * NC + 3)
    t0.g(2)
    t1.v(2)
    t0.k(3)
    t1.g(2)
    t0.v(3)
    t1.k(3)
    t0.g(3)
    t1.v(3)
    t1.phi(3)
    prev = t1

    for i in range(2, NT):
        if i == 2:
            for cp in x_cp[3:] + (q_cp if QFOLD_EARLY else []):
                cp.wait()
        if i == 2:
            side += [None]
        if i + 1 < NT:
            side += ln_pieces(i + 1)
        kv = KV(i)
        for c in range(NC):
            kv.k(c)
            if c == 0:
                prev.g(NC - 1)
            else:
                kv.g(c - 1)
            kv.v(c)
        if QFOLD_EARLY and i - 2 < NC:
            fold2(i - 2)
        prev = kv
    prev.g(NC - 1)
    take_side(len(side))

    gr = lax.broadcasted_iota(jnp.int32, (GR, 128), 0)
    gc = lax.broadcasted_iota(jnp.int32, (GR, 128), 1)
    row_head = jnp.where(gr < 64, gr // 32, (gr - 64) // 8)
    keep = row_head == ((gc % 64) // 32)
    for p in range(NP):
        g_buf[p] = _pk(jnp.where(keep, g_acc[p, :GR, :], 0.0).astype(BF16))
        if ZVPU:
            zb_buf[p] = jnp.broadcast_to(jnp.sum(z_acc[p], axis=1, keepdims=True), (128, 128))
        elif DENVPU:
            zb_buf[p] = jnp.broadcast_to(g_acc[p, 64:65, :], (128, 128)).T

    r_all = _rb(r_buf[...])
    iota = [lax.broadcasted_iota(jnp.int32, r_buf.shape, k) for k in range(3)]
    tok = iota[0] * 1024 + iota[2] * 8 + iota[1] if RVPU else iota[0] * T + iota[2]
    r_max = jnp.max(r_all)
    idx = jnp.min(jnp.where(r_all == r_max, tok, S - 1))
    sel_tile = idx // T
    blk = pl.multiple_of((idx // 16) * 16, 16)

    def tile_of(j):
        return (sel_tile + 1 + j) % NT

    def last_copy(n):
        rows = pl.ds(pl.multiple_of(sel_tile * T, T), T)
        cols = pl.ds(n * LASTW, LASTW)
        return pltpu.make_async_copy(out_buf.at[rows, cols], out_hbm.at[rows, cols], sem_o.at[NT - 1 + n])

    class Q:
        def __init__(self, j):
            self.j = j
            self.row0 = tile_of(j) * (T // 2)
            self.pq = {}

        def proj(self, c, n, dep=None):
            xn = _upk(xn_buf[pl.ds(pl.multiple_of(self.row0 + n * 64, 64), 64), :])
            self.pq[c, n] = _dot_nt(load_wt(c * MC, (c + 1) * MC, dep), xn)

        def num(self, c, n):
            pq = self.pq.pop((c, n))
            parts = []
            link = Link()
            for u in range(PC):
                phi = _phi_pair(pq[64 * u:64 * u + 64, :], link)
                nd = _dot(_upk(g_buf[c * PC + u]), phi.astype(BF16))
                if DENVPU:
                    zp = phi * zb_buf[c * PC + u]
                    zp = zp[:64, :] + zp[64:, :]
                for a in range(2):
                    if DENVPU:
                        den = jnp.sum(zp[32 * a:32 * a + 32, :], axis=0, keepdims=True)
                        parts.append(nd[32 * a:32 * a + 32, :] * pl.reciprocal(den + 1e-6, approx=True))
                    else:
                        inv = pl.reciprocal(nd[64 + 8 * a:72 + 8 * a, :] + 1e-6, approx=True)
                        parts.append(nd[32 * a:32 * a + 32, :] * jnp.concatenate([inv] * 4, axis=0))
            ot = jnp.concatenate(parts, axis=0)
            o_buf[self.j % 2, n * 64:(n + 1) * 64, c * MC:(c + 1) * MC] = _pk(ot.T.astype(BF16))

    def out_cols(j, n, upd=None):
        t = tile_of(j)
        rows = pl.ds(pl.multiple_of(t * T, T), T)
        rows2 = pl.ds(pl.multiple_of(t * (T // 2), T // 2), T // 2)
        cols = slice(n * 128, (n + 1) * 128)
        s = _dot(_upk(o_buf[j % 2]), _upk(wo_buf[:, cols]))
        xn = _upk(xn_buf[rows2, cols]).astype(F32)
        if upd is not None:
            xn = xn + upd[:, cols]
        out_buf[rows, cols] = (x_buf[rows, cols].astype(F32) + s * _silu(xn)).astype(BF16)

    def ffn_steps():
        st = {}
        KH = D // 2

        def apart(r):
            z = zero_buf[...]
            return pltpu.bitcast(pltpu.bitcast(r, U32) | jnp.concatenate([z, z], axis=0), F32)

        def up(w_ref, key, n, h):
            def f():
                xs = _upk(xn_buf[pl.ds(pl.multiple_of(blk // 2, 8), 8), h * KH:(h + 1) * KH])
                r = _dot(xs, _upk(w_ref[h * KH // 2:(h + 1) * KH // 2, n * 128:(n + 1) * 128]))
                st[key, n] = apart(r) if h == 0 else st[key, n] + r
            return f

        def down(c, n):
            def f():
                if ('h', c) not in st:
                    ms = range(c * FC // 128, (c + 1) * FC // 128)
                    st['h', c] = jnp.concatenate(
                        [_silu(st.pop(('g', m))) * st.pop(('u', m)) for m in ms], axis=1).astype(BF16)
                r = _dot(st['h', c], _upk(wd_buf[c * FC // 2:(c + 1) * FC // 2, n * 128:(n + 1) * 128]))
                st['y', n] = apart(r) if c == 0 else st['y', n] + r
            return f

        steps = []
        for c in range(F // FC + 1):
            ups = [up(w, k, m, h) for m in range(c * FC // 128, (c + 1) * FC // 128)
                   for h in range(2) for w, k in ((wg_buf, 'g'), (wu_buf, 'u'))] if c < F // FC else []
            downs = [down(c - 1, n) for n in range(D // 128)] if c > 0 else []
            while ups or downs:
                steps += ups[:2] + downs[:1]
                ups, downs = ups[2:], downs[1:]
        return steps, st

    for cp in ([] if QFOLD_EARLY else q_cp) + [wo_cp] + f_cp:
        cp.wait()
    if not QFOLD_EARLY:
        for j in range(NC):
            fold2(j)
    ffn, ffn_st = ffn_steps()

    q = Q(0)
    for c in range(NC):
        q.proj(c, 0)
        if c > 0:
            q.num(c - 1, 1)
        q.proj(c, 1)
        q.num(c, 0)
    def small():
        if ffn:
            ffn.pop(0)()

    pending = []

    def out_step():
        j, n = pending.pop(0)
        out_cols(j, n)
        if n == D // 128 - 1:
            out_copy(tile_of(j), j).start()

    for j in range(1, NT):
        qn = Q(j)
        pending += [(j - 1, n) for n in range(D // 128)]
        for c in range(NC):
            first_w = True
            for tok in PATTERN:
                if tok == 'P':
                    qn.proj(c, 0)
                elif tok == 'Q':
                    qn.proj(c, 1)
                elif tok == 'f':
                    small()
                elif tok == 'n':
                    (q if c == 0 else qn).num((c - 1) % NC, 1)
                elif tok == 'm':
                    qn.num(c, 0)
                elif tok == 'W':
                    if (j, c) != (1, 0) or not first_w:
                        out_step()
                    first_w = False
        q = qn
    assert not ffn
    q.num(NC - 1, 1)
    out_step()

    y = jnp.concatenate([ffn_st['y', n] for n in range(D // 128)], axis=1)
    sub = lax.broadcasted_iota(jnp.int32, (16, D), 0)
    y_row = jnp.sum(jnp.where(sub == idx - blk, y, 0.0), axis=0, keepdims=True)
    gate = 1.0 / (1.0 + jnp.exp(-jnp.full((1, D), r_max, F32)))
    trow = lax.broadcasted_iota(jnp.int32, (T, D), 0)
    upd = jnp.where(trow == idx - sel_tile * T, y_row * gate, 0.0)
    for n in range(D // 128):
        out_cols(NT - 1, n, upd)
        if (n + 1) * 128 % LASTW == 0:
            last_copy(n * 128 // LASTW).start()
    for j in range(NT - 1):
        out_copy(tile_of(j), j).wait()
    for n in range(D // LASTW):
        last_copy(n).wait()


@jax.jit
def pallas_recurrent_scan__linear_kernel_hedgehog__moe_arch_mod__prompt_kernel(
    A_x: jax.Array,
    A_wqkv: jax.Array,
    A_w_phi: jax.Array,
    A_wo: jax.Array,
    B_x: jax.Array,
    B_w_r: jax.Array,
    B_w_gate: jax.Array,
    B_w_up: jax.Array,
    B_w_down: jax.Array,
):
    del B_x
    any_spec = pl.BlockSpec(memory_space=pl.ANY)
    out = pl.pallas_call(
        _kernel,
        out_shape=jax.ShapeDtypeStruct((S, D), BF16),
        in_specs=[any_spec] * 8,
        out_specs=any_spec,
        scratch_shapes=[
            pltpu.VMEM((S, D), BF16),
            pltpu.VMEM((S // 2, D), U32),
            pltpu.VMEM((3 * NC, D // 2, MC), U32),
            pltpu.VMEM((WTR, D), U32),
            pltpu.VMEM((H, DH, DH), BF16),
            pltpu.VMEM((D,), BF16),
            pltpu.VMEM((D // 2, D), U32),
            pltpu.VMEM((D // 2, F), U32),
            pltpu.VMEM((D // 2, F), U32),
            pltpu.VMEM((F // 2, D), U32),
            pltpu.VMEM((9, 64, 128), U32),
            pltpu.VMEM((NP, GA, 128), F32),
            pltpu.VMEM((NP, GR // 2, 128), U32),
            pltpu.VMEM((2, 8, 128) if RVPU else (NT, 8, T), F32),
            pltpu.VMEM((2, T // 2, D), U32),
            pltpu.VMEM((S, D), BF16),
            pltpu.VMEM((8, 128), U32),
            pltpu.VMEM((NP, 128, 128), F32),
            pltpu.VMEM((NP, 128, 128), F32),
            pltpu.VMEM((1, D), F32),
            pltpu.SemaphoreType.DMA((NT,)),
            pltpu.SemaphoreType.DMA((3 * NC,)),
            pltpu.SemaphoreType.DMA((6,)),
            pltpu.SemaphoreType.DMA((NT - 1 + D // LASTW,)),
        ],
        compiler_params=pltpu.CompilerParams(
            vmem_limit_bytes=100 * 1024 * 1024,
            disable_bounds_checks=True,
            disable_semaphore_checks=True,
        ),
        name="hedgehog_mod",
    )(A_x.reshape(S, D), A_wqkv, A_w_phi, A_wo, B_w_r, B_w_gate, B_w_up, B_w_down)
    return out.reshape(1, S, D)
```

```python
import jax
import jax.numpy as jnp
from jax import lax
import jax.experimental.pallas as pl
import jax.experimental.pallas.tpu as pltpu

S, D, H, DH, F = 2048, 1024, 32, 32, 3584
T = 256
NT = S // T
MC = 256
NC = D // MC
PC = MC // 64
NP = H // 2
FC = 512
LNP = 16
PATTERN = "PfQfnfWfmfWf"
KROW = D + 16
VROW = KROW + D
LOG2E = 1.4426950408889634
EPS_LN = 1.0013580322265625e-05
F32 = jnp.float32
BF16 = jnp.bfloat16
U32 = jnp.uint32

_NT_DIMS = (((1,), (1,)), ((), ()))


def _dot_nt(a, b):
    return lax.dot_general(a, b, _NT_DIMS, preferred_element_type=F32)


def _dot(a, b):
    return jnp.dot(a, b, preferred_element_type=F32)


def _rb(x):
    return x.astype(BF16).astype(F32)


def _pk(x):
    return pltpu.bitcast(x, U32)


def _upk(x):
    return pltpu.bitcast(x, BF16)


def _phi_pair(p, link=None):
    pos, neg = [], []
    for a in range(2):
        ph = p[32 * a:32 * a + 32, :]
        mx = jnp.max(ph, axis=0, keepdims=True)
        mn = jnp.min(ph, axis=0, keepdims=True)
        if link is not None:
            mx, mn = link.start(mx, mn)
        ep = jnp.exp2(ph - mx)
        en = jnp.exp2(mn - ph)
        pos.append(ep * pl.reciprocal(jnp.sum(ep, axis=0, keepdims=True), approx=True))
        neg.append(en * pl.reciprocal(jnp.sum(en, axis=0, keepdims=True), approx=True))
        if link is not None:
            link.done(pos[-1], neg[-1])
    return jnp.concatenate(pos + neg, axis=0)


def _silu(x):
    h = 0.5 * x
    return h + h * jnp.tanh(h)


def _kernel(x_hbm, wqkv_hbm, wphi_hbm, wo_hbm, wr_hbm, wg_hbm, wu_hbm, wd_hbm, out_hbm,
            x_buf, xn_buf, w_buf, wt_buf, wphi_buf, wr_buf, wo_buf, wg_buf, wu_buf, wd_buf,
            bdt_buf, g_acc, g_buf, z_acc, zb_buf, r_buf, o_buf, out_buf, zero_buf,
            sem_x, sem_w, sem_s, sem_o):
    x_cp = [pltpu.make_async_copy(x_hbm.at[pl.ds(i * T, T), :], x_buf.at[pl.ds(i * T, T), :], sem_x.at[i])
            for i in range(NT)]
    w_cp = [pltpu.make_async_copy(wqkv_hbm.at[:, pl.ds(j * MC, MC)], w_buf.at[j].bitcast(BF16), sem_w.at[j])
            for j in range(3 * NC)]
    q_cp, k_cp, v_cp = w_cp[:NC], w_cp[NC:2 * NC], w_cp[2 * NC:]
    phi_cp = pltpu.make_async_copy(wphi_hbm, wphi_buf, sem_s.at[0])
    wr_cp = pltpu.make_async_copy(wr_hbm, wr_buf, sem_s.at[1])
    wo_cp = pltpu.make_async_copy(wo_hbm, wo_buf.bitcast(BF16), sem_s.at[2])
    f_cp = [pltpu.make_async_copy(wg_hbm, wg_buf.bitcast(BF16), sem_s.at[3]),
            pltpu.make_async_copy(wu_hbm, wu_buf.bitcast(BF16), sem_s.at[4]),
            pltpu.make_async_copy(wd_hbm, wd_buf.bitcast(BF16), sem_s.at[5])]

    copies = [x_cp[0], wr_cp, v_cp[0], x_cp[1], v_cp[1], phi_cp, k_cp[0], k_cp[1], v_cp[2], k_cp[2],
              v_cp[3], k_cp[3]] + x_cp[2:] + q_cp + [wo_cp] + f_cp

    def start_all(j, carry):
        for k, cp in enumerate(copies):
            pl.when((k + 2) * j == j)(cp.start)
        zero_buf[...] = jnp.zeros_like(zero_buf)
        return carry

    lax.fori_loop(0, 2, start_all, 0)

    def tie(w, dep):
        acc = None
        for r in range(0, dep.shape[0], 8):
            for c in range(0, dep.shape[1], 128):
                piece = dep[r:r + 8, c:c + 128]
                acc = piece if acc is None else acc | piece
        first = w[:8, :128] | (acc & zero_buf[...])
        return jnp.concatenate([jnp.concatenate([first, w[:8, 128:]], axis=1), w[8:, :]], axis=0)

    def after(x, dep):
        z = pltpu.bitcast(dep, U32)[:x.shape[0], :] & zero_buf[:x.shape[0], :]
        return pltpu.bitcast(pltpu.bitcast(x, U32) | z, F32)

    class Link:
        def __init__(self):
            self.prev = None

        def start(self, mx, mn):
            if self.prev is None:
                return mx, mn
            return after(mx, self.prev[0]), after(mn, self.prev[1])

        def done(self, pos, neg):
            self.prev = (pos[24:32, :], neg[24:32, :])

    side = []

    def take_side():
        f = side.pop(0) if side else None
        return None if f is None else f()

    def layer_norm(i, piece=0, npieces=1):
        n = T // npieces
        r0 = i * T + piece * n
        x = x_buf[r0:r0 + n, :].astype(F32)
        m = jnp.mean(x, axis=-1, keepdims=True)
        mb = _rb(m)
        d = x - mb
        v = jnp.mean(d * d, axis=-1, keepdims=True) - (m - mb) * (m - mb)
        den = _rb(jnp.sqrt(_rb(_rb(v) + EPS_LN)))
        inv = pl.reciprocal(den, approx=True)
        inv = inv * (2.0 - den * inv)
        xn = _pk((_rb(d) * inv).astype(BF16))
        xn_buf[r0 // 2:(r0 + n) // 2, :] = xn
        return xn

    def ln_pieces(i):
        return [lambda p=p: layer_norm(i, p, LNP) for p in range(LNP)]

    def load_wt(r0, r1, dep=None):
        w = wt_buf[r0 // 2:r1 // 2, :]
        return _upk(w if dep is None else tie(w, dep))

    def fold(j):
        for u in range(MC // 128):
            w = _upk(w_buf[j, :, u * 128:(u + 1) * 128])
            if j < 2 * NC:
                r = _dot_nt(_upk(bdt_buf[(2 * j + u) % 8]), w) * LOG2E
            elif j == 2 * NC:
                r = _dot_nt(_upk(bdt_buf[8]), w)
            else:
                r = w.astype(F32).T
            row = (j * MC + u * 128 + (KROW - D if j >= NC else 0)) // 2
            wt_buf[row:row + 64, :] = _pk(r.astype(BF16))

    ri = lax.broadcasted_iota(jnp.int32, (128, 128), 0)
    ci = lax.broadcasted_iota(jnp.int32, (128, 128), 1)

    def build_bdt():
        same_head = (ri // 32) == (ci // 32)
        e_r = lax.broadcasted_iota(jnp.int32, (128, 32), 0)
        e_c = lax.broadcasted_iota(jnp.int32, (128, 32), 1)
        tile_eye = jnp.where((e_r % 32) == e_c, 1.0, 0.0).astype(BF16)
        for g in range(8):
            wg4 = wphi_buf[4 * g:4 * g + 4].reshape(128, 32)
            bdt_buf[g] = _pk(jnp.where(same_head, _dot_nt(tile_eye, wg4), 0.0).astype(BF16))

    class KV:
        def __init__(self, i):
            self.i = i
            self.pk, self.vt, self.ph = {}, {}, {}

        def proj(self, r0, r1):
            halves = []
            for n in range(2):
                row = (self.i * T + n * 128) // 2
                halves.append(_dot_nt(load_wt(r0, r1, take_side()), _upk(xn_buf[row:row + 64, :])))
            return jnp.concatenate(halves, axis=1)

        def k(self, c):
            if c == 0:
                kr = self.proj(KROW - 16, KROW + MC)
                r_buf[self.i] = kr[:8, :]
                self.pk[c] = kr[16:, :]
            else:
                self.pk[c] = self.proj(KROW + c * MC, KROW + (c + 1) * MC)

        def v(self, c):
            self.vt[c] = self.proj(VROW + c * MC, VROW + (c + 1) * MC).astype(BF16)

        def phi(self, c):
            if c not in self.ph:
                pk = self.pk.pop(c)
                self.ph[c] = []
                for u in range(PC):
                    phi = _phi_pair(pk[64 * u:64 * u + 64, :])
                    z = phi[:, :128] + phi[:, 128:]
                    if self.i > 0:
                        z = z + z_acc[c * PC + u]
                    z_acc[c * PC + u] = z
                    self.ph[c].append((phi.astype(BF16), z))
            return self.ph[c]

        def g(self, c):
            vt = self.vt.pop(c)
            for u, (phi, z) in enumerate(self.phi(c)):
                r = _dot_nt(_upk(tie(_pk(vt[64 * u:64 * u + 64, :]), pltpu.bitcast(z, U32))), phi)
                if self.i == 0:
                    g_acc[c * PC + u] = r
                else:
                    g_acc[c * PC + u] += r

    bdt_buf[8] = _pk(jnp.where(ri == ci, 1.0, 0.0).astype(BF16))
    x_cp[0].wait()
    layer_norm(0)
    t0, t1 = KV(0), KV(1)
    wr_cp.wait()
    v_cp[0].wait()
    fold(2 * NC)
    t0.v(0)
    x_cp[1].wait()
    layer_norm(1)
    v_cp[1].wait()
    fold(2 * NC + 1)
    t1.v(0)
    t0.v(1)
    t1.v(1)
    phi_cp.wait()
    k_cp[0].wait()
    k_cp[1].wait()
    wt_buf[D // 2:D // 2 + 8, :] = _pk(
        jnp.broadcast_to(wr_buf[...].astype(F32).reshape(1, D), (16, D)).astype(BF16))
    build_bdt()
    fold(NC)
    fold(NC + 1)
    t0.k(0)
    t1.k(0)
    t0.k(1)
    t0.g(0)
    t1.k(1)
    t1.g(0)
    t0.g(1)
    t1.phi(1)
    for cp in [v_cp[2], k_cp[2], v_cp[3], k_cp[3], x_cp[2]]:
        cp.wait()
    side += ln_pieces(2)
    fold(NC + 2)
    fold(2 * NC + 2)
    fold(NC + 3)
    t1.g(1)
    t0.k(2)
    t1.k(2)
    t0.v(2)
    fold(2 * NC + 3)
    t0.g(2)
    t1.v(2)
    t0.k(3)
    t1.g(2)
    t0.v(3)
    t1.k(3)
    t0.g(3)
    t1.v(3)
    t1.phi(3)
    prev = t1

    for cp in x_cp[3:]:
        cp.wait()
    side += [None]
    for i in range(2, NT):
        if i + 1 < NT:
            side += ln_pieces(i + 1)
        kv = KV(i)
        for c in range(NC):
            kv.k(c)
            (prev if c == 0 else kv).g((c - 1) % NC)
            kv.v(c)
        prev = kv
    prev.g(NC - 1)
    assert not side

    same_head = (lax.broadcasted_iota(jnp.int32, (64, 128), 0) // 32
                 == (lax.broadcasted_iota(jnp.int32, (64, 128), 1) % 64) // 32)
    for p in range(NP):
        g_buf[p] = _pk(jnp.where(same_head, g_acc[p], 0.0).astype(BF16))
        zb_buf[p] = jnp.broadcast_to(jnp.sum(z_acc[p], axis=1, keepdims=True), (128, 128))

    r_all = _rb(r_buf[...])
    tok = (lax.broadcasted_iota(jnp.int32, r_buf.shape, 0) * T
           + lax.broadcasted_iota(jnp.int32, r_buf.shape, 2))
    r_max = jnp.max(r_all)
    idx = jnp.min(jnp.where(r_all == r_max, tok, S - 1))
    sel_tile = idx // T
    blk = pl.multiple_of((idx // 16) * 16, 16)

    def tile_of(j):
        return (sel_tile + 1 + j) % NT

    def out_copy(j):
        rows = pl.ds(pl.multiple_of(tile_of(j) * T, T), T)
        return pltpu.make_async_copy(out_buf.at[rows, :], out_hbm.at[rows, :], sem_o.at[j])

    def last_copy(n):
        rows = pl.ds(pl.multiple_of(sel_tile * T, T), T)
        cols = pl.ds(n * 128, 128)
        return pltpu.make_async_copy(out_buf.at[rows, cols], out_hbm.at[rows, cols], sem_o.at[NT - 1 + n])

    class Q:
        def __init__(self, j):
            self.j = j
            self.row0 = tile_of(j) * (T // 2)
            self.pq = {}

        def proj(self, c, n):
            xn = _upk(xn_buf[pl.ds(pl.multiple_of(self.row0 + n * 64, 64), 64), :])
            self.pq[c, n] = _dot_nt(load_wt(c * MC, (c + 1) * MC), xn)

        def num(self, c, n):
            pq = self.pq.pop((c, n))
            parts = []
            link = Link()
            for u in range(PC):
                phi = _phi_pair(pq[64 * u:64 * u + 64, :], link)
                nd = _dot(_upk(g_buf[c * PC + u]), phi.astype(BF16))
                zp = phi * zb_buf[c * PC + u]
                zp = zp[:64, :] + zp[64:, :]
                for a in range(2):
                    den = jnp.sum(zp[32 * a:32 * a + 32, :], axis=0, keepdims=True)
                    parts.append(nd[32 * a:32 * a + 32, :] * pl.reciprocal(den + 1e-6, approx=True))
            ot = jnp.concatenate(parts, axis=0)
            o_buf[self.j % 2, n * 64:(n + 1) * 64, c * MC:(c + 1) * MC] = _pk(ot.T.astype(BF16))

    def out_cols(j, n, upd=None):
        t = tile_of(j)
        rows = pl.ds(pl.multiple_of(t * T, T), T)
        rows2 = pl.ds(pl.multiple_of(t * (T // 2), T // 2), T // 2)
        cols = slice(n * 128, (n + 1) * 128)
        s = _dot(_upk(o_buf[j % 2]), _upk(wo_buf[:, cols]))
        xn = _upk(xn_buf[rows2, cols]).astype(F32)
        if upd is not None:
            xn = xn + upd[:, cols]
        out_buf[rows, cols] = (x_buf[rows, cols].astype(F32) + s * _silu(xn)).astype(BF16)

    def ffn_steps():
        st = {}
        KH = D // 2

        def apart(r):
            z = zero_buf[...]
            return pltpu.bitcast(pltpu.bitcast(r, U32) | jnp.concatenate([z, z], axis=0), F32)

        def up(w_ref, key, n, h):
            def f():
                xs = _upk(xn_buf[pl.ds(pl.multiple_of(blk // 2, 8), 8), h * KH:(h + 1) * KH])
                r = _dot(xs, _upk(w_ref[h * KH // 2:(h + 1) * KH // 2, n * 128:(n + 1) * 128]))
                st[key, n] = apart(r) if h == 0 else st[key, n] + r
            return f

        def down(c, n):
            def f():
                if ('h', c) not in st:
                    ms = range(c * FC // 128, (c + 1) * FC // 128)
                    st['h', c] = jnp.concatenate(
                        [_silu(st.pop(('g', m))) * st.pop(('u', m)) for m in ms], axis=1).astype(BF16)
                r = _dot(st['h', c], _upk(wd_buf[c * FC // 2:(c + 1) * FC // 2, n * 128:(n + 1) * 128]))
                st['y', n] = apart(r) if c == 0 else st['y', n] + r
            return f

        steps = []
        for c in range(F // FC + 1):
            ups = [up(w, k, m, h) for m in range(c * FC // 128, (c + 1) * FC // 128)
                   for h in range(2) for w, k in ((wg_buf, 'g'), (wu_buf, 'u'))] if c < F // FC else []
            downs = [down(c - 1, n) for n in range(D // 128)] if c > 0 else []
            while ups or downs:
                steps += ups[:2] + downs[:1]
                ups, downs = ups[2:], downs[1:]
        return steps, st

    for cp in q_cp + [wo_cp] + f_cp:
        cp.wait()
    for j in range(NC):
        fold(j)
    ffn, ffn_st = ffn_steps()

    q = Q(0)
    for c in range(NC):
        q.proj(c, 0)
        if c > 0:
            q.num(c - 1, 1)
        q.proj(c, 1)
        q.num(c, 0)

    pending = [None]

    def out_step():
        step = pending.pop(0)
        if step is not None:
            out_cols(*step)
            if step[1] == D // 128 - 1:
                out_copy(step[0]).start()

    for j in range(1, NT):
        qn = Q(j)
        pending += [(j - 1, n) for n in range(D // 128)]
        for c in range(NC):
            for tok in PATTERN:
                if tok == 'P' or tok == 'Q':
                    qn.proj(c, int(tok == 'Q'))
                elif tok == 'n':
                    (q if c == 0 else qn).num((c - 1) % NC, 1)
                elif tok == 'm':
                    qn.num(c, 0)
                elif tok == 'W':
                    out_step()
                else:
                    ffn.pop(0)()
        q = qn
    assert not ffn
    q.num(NC - 1, 1)
    out_step()

    y = jnp.concatenate([ffn_st['y', n] for n in range(D // 128)], axis=1)
    sub = lax.broadcasted_iota(jnp.int32, (16, D), 0)
    y_row = jnp.sum(jnp.where(sub == idx - blk, y, 0.0), axis=0, keepdims=True)
    gate = 1.0 / (1.0 + jnp.exp(-jnp.full((1, D), r_max, F32)))
    trow = lax.broadcasted_iota(jnp.int32, (T, D), 0)
    upd = jnp.where(trow == idx - sel_tile * T, y_row * gate, 0.0)
    for n in range(D // 128):
        out_cols(NT - 1, n, upd)
        last_copy(n).start()
    for j in range(NT - 1):
        out_copy(j).wait()
    for n in range(D // 128):
        last_copy(n).wait()


@jax.jit
def pallas_recurrent_scan__linear_kernel_hedgehog__moe_arch_mod__prompt_kernel(
    A_x: jax.Array,
    A_wqkv: jax.Array,
    A_w_phi: jax.Array,
    A_wo: jax.Array,
    B_x: jax.Array,
    B_w_r: jax.Array,
    B_w_gate: jax.Array,
    B_w_up: jax.Array,
    B_w_down: jax.Array,
):
    del B_x
    any_spec = pl.BlockSpec(memory_space=pl.ANY)
    out = pl.pallas_call(
        _kernel,
        out_shape=jax.ShapeDtypeStruct((S, D), BF16),
        in_specs=[any_spec] * 8,
        out_specs=any_spec,
        scratch_shapes=[
            pltpu.VMEM((S, D), BF16),
            pltpu.VMEM((S // 2, D), U32),
            pltpu.VMEM((3 * NC, D // 2, MC), U32),
            pltpu.VMEM(((VROW + D) // 2, D), U32),
            pltpu.VMEM((H, DH, DH), BF16),
            pltpu.VMEM((D,), BF16),
            pltpu.VMEM((D // 2, D), U32),
            pltpu.VMEM((D // 2, F), U32),
            pltpu.VMEM((D // 2, F), U32),
            pltpu.VMEM((F // 2, D), U32),
            pltpu.VMEM((9, 64, 128), U32),
            pltpu.VMEM((NP, 64, 128), F32),
            pltpu.VMEM((NP, 32, 128), U32),
            pltpu.VMEM((NP, 128, 128), F32),
            pltpu.VMEM((NP, 128, 128), F32),
            pltpu.VMEM((NT, 8, T), F32),
            pltpu.VMEM((2, T // 2, D), U32),
            pltpu.VMEM((S, D), BF16),
            pltpu.VMEM((8, 128), U32),
            pltpu.SemaphoreType.DMA((NT,)),
            pltpu.SemaphoreType.DMA((3 * NC,)),
            pltpu.SemaphoreType.DMA((6,)),
            pltpu.SemaphoreType.DMA((NT - 1 + D // 128,)),
        ],
        compiler_params=pltpu.CompilerParams(
            vmem_limit_bytes=100 * 1024 * 1024,
            disable_bounds_checks=True,
            disable_semaphore_checks=True,
        ),
        name="hedgehog_mod",
    )(A_x.reshape(S, D), A_wqkv, A_w_phi, A_wo, B_w_r, B_w_gate, B_w_up, B_w_down)
    return out.reshape(1, S, D)
```

```python
import jax
import jax.numpy as jnp
from jax import lax
import jax.experimental.pallas as pl
import jax.experimental.pallas.tpu as pltpu

S, D, H, DH, F = 2048, 1024, 32, 32, 3584
T = 256
NT = S // T
MC = 256
NC = D // MC
PC = MC // 64
NP = H // 2
FC = 512
LNP = 16
PATTERN = "PfQfnfWfmfWf"
KROW = D + 16
VROW = KROW + D
LOG2E = 1.4426950408889634
EPS_LN = 1.0013580322265625e-05
F32 = jnp.float32
BF16 = jnp.bfloat16
U32 = jnp.uint32

_NT_DIMS = (((1,), (1,)), ((), ()))


def _dot_nt(a, b):
    return lax.dot_general(a, b, _NT_DIMS, preferred_element_type=F32)


def _dot(a, b):
    return jnp.dot(a, b, preferred_element_type=F32)


def _rb(x):
    return x.astype(BF16).astype(F32)


def _pk(x):
    return pltpu.bitcast(x, U32)


def _upk(x):
    return pltpu.bitcast(x, BF16)


def _phi_pair(p, link=None):
    pos, neg = [], []
    for a in range(2):
        ph = p[32 * a:32 * a + 32, :]
        mx = jnp.max(ph, axis=0, keepdims=True)
        mn = jnp.min(ph, axis=0, keepdims=True)
        if link is not None:
            mx, mn = link.start(mx, mn)
        ep = jnp.exp2(ph - mx)
        en = jnp.exp2(mn - ph)
        pos.append(ep * pl.reciprocal(jnp.sum(ep, axis=0, keepdims=True), approx=True))
        neg.append(en * pl.reciprocal(jnp.sum(en, axis=0, keepdims=True), approx=True))
        if link is not None:
            link.done(pos[-1], neg[-1])
    return jnp.concatenate(pos + neg, axis=0)


def _silu(x):
    h = 0.5 * x
    return h + h * jnp.tanh(h)


def _kernel(x_hbm, wqkv_hbm, wphi_hbm, wo_hbm, wr_hbm, wg_hbm, wu_hbm, wd_hbm, out_hbm,
            x_buf, xn_buf, w_buf, wt_buf, wphi_buf, wr_buf, wo_buf, wg_buf, wu_buf, wd_buf,
            bdt_buf, g_acc, g_buf, z_acc, zb_buf, r_buf, o_buf, out_buf, zero_buf,
            sem_x, sem_w, sem_s, sem_o):
    x_cp = [pltpu.make_async_copy(x_hbm.at[pl.ds(i * T, T), :], x_buf.at[pl.ds(i * T, T), :], sem_x.at[i])
            for i in range(NT)]
    w_cp = [pltpu.make_async_copy(wqkv_hbm.bitcast(U32).at[:, pl.ds(j * MC, MC)], w_buf.at[j], sem_w.at[j])
            for j in range(3 * NC)]
    q_cp, k_cp, v_cp = w_cp[:NC], w_cp[NC:2 * NC], w_cp[2 * NC:]
    phi_cp = pltpu.make_async_copy(wphi_hbm, wphi_buf, sem_s.at[0])
    wr_cp = pltpu.make_async_copy(wr_hbm, wr_buf, sem_s.at[1])
    wo_cp = pltpu.make_async_copy(wo_hbm.bitcast(U32), wo_buf, sem_s.at[2])
    f_cp = [pltpu.make_async_copy(wg_hbm.bitcast(U32), wg_buf, sem_s.at[3]),
            pltpu.make_async_copy(wu_hbm.bitcast(U32), wu_buf, sem_s.at[4]),
            pltpu.make_async_copy(wd_hbm.bitcast(U32), wd_buf, sem_s.at[5])]

    copies = [x_cp[0], wr_cp, v_cp[0], x_cp[1], v_cp[1], phi_cp, k_cp[0], k_cp[1], v_cp[2], k_cp[2],
              v_cp[3], k_cp[3]] + x_cp[2:] + q_cp + [wo_cp] + f_cp

    def start_all(j, carry):
        for k, cp in enumerate(copies):
            pl.when((k + 2) * j == j)(cp.start)
        zero_buf[...] = jnp.zeros_like(zero_buf)
        return carry

    lax.fori_loop(0, 2, start_all, 0)

    def tie(w, dep):
        acc = None
        for r in range(0, dep.shape[0], 8):
            for c in range(0, dep.shape[1], 128):
                piece = dep[r:r + 8, c:c + 128]
                acc = piece if acc is None else acc | piece
        first = w[:8, :128] | (acc & zero_buf[...])
        return jnp.concatenate([jnp.concatenate([first, w[:8, 128:]], axis=1), w[8:, :]], axis=0)

    def after(x, dep):
        z = pltpu.bitcast(dep, U32)[:x.shape[0], :] & zero_buf[:x.shape[0], :]
        return pltpu.bitcast(pltpu.bitcast(x, U32) | z, F32)

    class Link:
        def __init__(self):
            self.prev = None

        def start(self, mx, mn):
            if self.prev is None:
                return mx, mn
            return after(mx, self.prev[0]), after(mn, self.prev[1])

        def done(self, pos, neg):
            self.prev = (pos[24:32, :], neg[24:32, :])

    side = []

    def take_side():
        f = side.pop(0) if side else None
        return None if f is None else f()

    def layer_norm(i, piece=0, npieces=1):
        n = T // npieces
        r0 = i * T + piece * n
        x = x_buf[r0:r0 + n, :].astype(F32)
        m = jnp.mean(x, axis=-1, keepdims=True)
        mb = _rb(m)
        d = x - mb
        v = jnp.mean(d * d, axis=-1, keepdims=True) - (m - mb) * (m - mb)
        den = _rb(jnp.sqrt(_rb(_rb(v) + EPS_LN)))
        inv = pl.reciprocal(den, approx=True)
        inv = inv * (2.0 - den * inv)
        xn = _pk((_rb(d) * inv).astype(BF16))
        xn_buf[r0 // 2:(r0 + n) // 2, :] = xn
        return xn

    def ln_pieces(i):
        return [lambda p=p: layer_norm(i, p, LNP) for p in range(LNP)]

    def load_wt(r0, r1, dep=None):
        w = wt_buf[r0 // 2:r1 // 2, :]
        return _upk(w if dep is None else tie(w, dep))

    def fold(j):
        for u in range(MC // 128):
            w = _upk(w_buf[j, :, u * 128:(u + 1) * 128])
            if j < 2 * NC:
                r = _dot_nt(_upk(bdt_buf[(2 * j + u) % 8]), w) * LOG2E
            elif j == 2 * NC:
                r = _dot_nt(_upk(bdt_buf[8]), w)
            else:
                r = w.astype(F32).T
            row = (j * MC + u * 128 + (KROW - D if j >= NC else 0)) // 2
            wt_buf[row:row + 64, :] = _pk(r.astype(BF16))

    ri = lax.broadcasted_iota(jnp.int32, (128, 128), 0)
    ci = lax.broadcasted_iota(jnp.int32, (128, 128), 1)

    def build_bdt():
        same_head = (ri // 32) == (ci // 32)
        e_r = lax.broadcasted_iota(jnp.int32, (128, 32), 0)
        e_c = lax.broadcasted_iota(jnp.int32, (128, 32), 1)
        tile_eye = jnp.where((e_r % 32) == e_c, 1.0, 0.0).astype(BF16)
        for g in range(8):
            wg4 = wphi_buf[4 * g:4 * g + 4].reshape(128, 32)
            bdt_buf[g] = _pk(jnp.where(same_head, _dot_nt(tile_eye, wg4), 0.0).astype(BF16))

    class KV:
        def __init__(self, i):
            self.i = i
            self.pk, self.vt, self.ph = {}, {}, {}

        def proj(self, r0, r1):
            halves = []
            for n in range(2):
                row = (self.i * T + n * 128) // 2
                halves.append(_dot_nt(load_wt(r0, r1, take_side()), _upk(xn_buf[row:row + 64, :])))
            return jnp.concatenate(halves, axis=1)

        def k(self, c):
            if c == 0:
                kr = self.proj(KROW - 16, KROW + MC)
                r_buf[self.i] = kr[:8, :]
                self.pk[c] = kr[16:, :]
            else:
                self.pk[c] = self.proj(KROW + c * MC, KROW + (c + 1) * MC)

        def v(self, c):
            self.vt[c] = self.proj(VROW + c * MC, VROW + (c + 1) * MC).astype(BF16)

        def phi(self, c):
            if c not in self.ph:
                pk = self.pk.pop(c)
                self.ph[c] = []
                for u in range(PC):
                    phi = _phi_pair(pk[64 * u:64 * u + 64, :])
                    z = phi[:, :128] + phi[:, 128:]
                    if self.i > 0:
                        z = z + z_acc[c * PC + u]
                    z_acc[c * PC + u] = z
                    self.ph[c].append((phi.astype(BF16), z))
            return self.ph[c]

        def g(self, c):
            vt = self.vt.pop(c)
            for u, (phi, z) in enumerate(self.phi(c)):
                r = _dot_nt(_upk(tie(_pk(vt[64 * u:64 * u + 64, :]), pltpu.bitcast(z, U32))), phi)
                if self.i == 0:
                    g_acc[c * PC + u] = r
                else:
                    g_acc[c * PC + u] += r

    bdt_buf[8] = _pk(jnp.where(ri == ci, 1.0, 0.0).astype(BF16))
    x_cp[0].wait()
    layer_norm(0)
    t0, t1 = KV(0), KV(1)
    wr_cp.wait()
    v_cp[0].wait()
    fold(2 * NC)
    t0.v(0)
    x_cp[1].wait()
    layer_norm(1)
    v_cp[1].wait()
    fold(2 * NC + 1)
    t1.v(0)
    t0.v(1)
    t1.v(1)
    phi_cp.wait()
    k_cp[0].wait()
    k_cp[1].wait()
    wt_buf[D // 2:D // 2 + 8, :] = _pk(
        jnp.broadcast_to(wr_buf[...].astype(F32).reshape(1, D), (16, D)).astype(BF16))
    build_bdt()
    fold(NC)
    fold(NC + 1)
    t0.k(0)
    t1.k(0)
    t0.k(1)
    t0.g(0)
    t1.k(1)
    t1.g(0)
    t0.g(1)
    t1.phi(1)
    for cp in [v_cp[2], k_cp[2], v_cp[3], k_cp[3], x_cp[2]]:
        cp.wait()
    side += ln_pieces(2)
    fold(NC + 2)
    fold(2 * NC + 2)
    fold(NC + 3)
    t1.g(1)
    t0.k(2)
    t1.k(2)
    t0.v(2)
    fold(2 * NC + 3)
    t0.g(2)
    t1.v(2)
    t0.k(3)
    t1.g(2)
    t0.v(3)
    t1.k(3)
    t0.g(3)
    t1.v(3)
    t1.phi(3)
    prev = t1

    for cp in x_cp[3:]:
        cp.wait()
    side += [None]
    for i in range(2, NT):
        if i + 1 < NT:
            side += ln_pieces(i + 1)
        kv = KV(i)
        for c in range(NC):
            kv.k(c)
            (prev if c == 0 else kv).g((c - 1) % NC)
            kv.v(c)
        prev = kv
    prev.g(NC - 1)
    assert not side

    same_head = (lax.broadcasted_iota(jnp.int32, (64, 128), 0) // 32
                 == (lax.broadcasted_iota(jnp.int32, (64, 128), 1) % 64) // 32)
    for p in range(NP):
        g_buf[p] = _pk(jnp.where(same_head, g_acc[p], 0.0).astype(BF16))
        zb_buf[p] = jnp.broadcast_to(jnp.sum(z_acc[p], axis=1, keepdims=True), (128, 128))

    r_all = _rb(r_buf[...])
    tok = (lax.broadcasted_iota(jnp.int32, r_buf.shape, 0) * T
           + lax.broadcasted_iota(jnp.int32, r_buf.shape, 2))
    r_max = jnp.max(r_all)
    idx = jnp.min(jnp.where(r_all == r_max, tok, S - 1))
    sel_tile = idx // T
    blk = pl.multiple_of((idx // 16) * 16, 16)

    def tile_of(j):
        return (sel_tile + 1 + j) % NT

    def out_copy(j):
        rows = pl.ds(pl.multiple_of(tile_of(j) * T, T), T)
        return pltpu.make_async_copy(out_buf.at[rows, :], out_hbm.at[rows, :], sem_o.at[j])

    def last_copy(n):
        rows = pl.ds(pl.multiple_of(sel_tile * T, T), T)
        cols = pl.ds(n * 128, 128)
        return pltpu.make_async_copy(out_buf.at[rows, cols], out_hbm.at[rows, cols], sem_o.at[NT - 1 + n])

    class Q:
        def __init__(self, j):
            self.j = j
            self.row0 = tile_of(j) * (T // 2)
            self.pq = {}

        def proj(self, c, n):
            xn = _upk(xn_buf[pl.ds(pl.multiple_of(self.row0 + n * 64, 64), 64), :])
            self.pq[c, n] = _dot_nt(load_wt(c * MC, (c + 1) * MC), xn)

        def num(self, c, n):
            pq = self.pq.pop((c, n))
            parts = []
            link = Link()
            for u in range(PC):
                phi = _phi_pair(pq[64 * u:64 * u + 64, :], link)
                nd = _dot(_upk(g_buf[c * PC + u]), phi.astype(BF16))
                zp = phi * zb_buf[c * PC + u]
                zp = zp[:64, :] + zp[64:, :]
                for a in range(2):
                    den = jnp.sum(zp[32 * a:32 * a + 32, :], axis=0, keepdims=True)
                    parts.append(nd[32 * a:32 * a + 32, :] * pl.reciprocal(den + 1e-6, approx=True))
            ot = jnp.concatenate(parts, axis=0)
            o_buf[self.j % 2, n * 64:(n + 1) * 64, c * MC:(c + 1) * MC] = _pk(ot.T.astype(BF16))

    def out_cols(j, n, upd=None):
        t = tile_of(j)
        rows = pl.ds(pl.multiple_of(t * T, T), T)
        rows2 = pl.ds(pl.multiple_of(t * (T // 2), T // 2), T // 2)
        cols = slice(n * 128, (n + 1) * 128)
        s = _dot(_upk(o_buf[j % 2]), _upk(wo_buf[:, cols]))
        xn = _upk(xn_buf[rows2, cols]).astype(F32)
        if upd is not None:
            xn = xn + upd[:, cols]
        out_buf[rows, cols] = (x_buf[rows, cols].astype(F32) + s * _silu(xn)).astype(BF16)

    def ffn_steps():
        st = {}
        KH = D // 2

        def apart(r):
            z = zero_buf[...]
            return pltpu.bitcast(pltpu.bitcast(r, U32) | jnp.concatenate([z, z], axis=0), F32)

        def up(w_ref, key, n, h):
            def f():
                xs = _upk(xn_buf[pl.ds(pl.multiple_of(blk // 2, 8), 8), h * KH:(h + 1) * KH])
                r = _dot(xs, _upk(w_ref[h * KH // 2:(h + 1) * KH // 2, n * 128:(n + 1) * 128]))
                st[key, n] = apart(r) if h == 0 else st[key, n] + r
            return f

        def down(c, n):
            def f():
                if ('h', c) not in st:
                    ms = range(c * FC // 128, (c + 1) * FC // 128)
                    st['h', c] = jnp.concatenate(
                        [_silu(st.pop(('g', m))) * st.pop(('u', m)) for m in ms], axis=1).astype(BF16)
                r = _dot(st['h', c], _upk(wd_buf[c * FC // 2:(c + 1) * FC // 2, n * 128:(n + 1) * 128]))
                st['y', n] = apart(r) if c == 0 else st['y', n] + r
            return f

        steps = []
        for c in range(F // FC + 1):
            ups = [up(w, k, m, h) for m in range(c * FC // 128, (c + 1) * FC // 128)
                   for h in range(2) for w, k in ((wg_buf, 'g'), (wu_buf, 'u'))] if c < F // FC else []
            downs = [down(c - 1, n) for n in range(D // 128)] if c > 0 else []
            while ups or downs:
                steps += ups[:2] + downs[:1]
                ups, downs = ups[2:], downs[1:]
        return steps, st

    for cp in q_cp + [wo_cp] + f_cp:
        cp.wait()
    for j in range(NC):
        fold(j)
    ffn, ffn_st = ffn_steps()

    q = Q(0)
    for c in range(NC):
        q.proj(c, 0)
        if c > 0:
            q.num(c - 1, 1)
        q.proj(c, 1)
        q.num(c, 0)

    pending = [None]

    def out_step():
        step = pending.pop(0)
        if step is not None:
            out_cols(*step)
            if step[1] == D // 128 - 1:
                out_copy(step[0]).start()

    for j in range(1, NT):
        qn = Q(j)
        pending += [(j - 1, n) for n in range(D // 128)]
        for c in range(NC):
            for tok in PATTERN:
                if tok == 'P' or tok == 'Q':
                    qn.proj(c, int(tok == 'Q'))
                elif tok == 'n':
                    (q if c == 0 else qn).num((c - 1) % NC, 1)
                elif tok == 'm':
                    qn.num(c, 0)
                elif tok == 'W':
                    out_step()
                else:
                    ffn.pop(0)()
        q = qn
    assert not ffn
    q.num(NC - 1, 1)
    out_step()

    y = jnp.concatenate([ffn_st['y', n] for n in range(D // 128)], axis=1)
    sub = lax.broadcasted_iota(jnp.int32, (16, D), 0)
    y_row = jnp.sum(jnp.where(sub == idx - blk, y, 0.0), axis=0, keepdims=True)
    gate = 1.0 / (1.0 + jnp.exp(-jnp.full((1, D), r_max, F32)))
    trow = lax.broadcasted_iota(jnp.int32, (T, D), 0)
    upd = jnp.where(trow == idx - sel_tile * T, y_row * gate, 0.0)
    for n in range(D // 128):
        out_cols(NT - 1, n, upd)
        last_copy(n).start()
    for j in range(NT - 1):
        out_copy(j).wait()
    for n in range(D // 128):
        last_copy(n).wait()


@jax.jit
def pallas_recurrent_scan__linear_kernel_hedgehog__moe_arch_mod__prompt_kernel(
    A_x: jax.Array,
    A_wqkv: jax.Array,
    A_w_phi: jax.Array,
    A_wo: jax.Array,
    B_x: jax.Array,
    B_w_r: jax.Array,
    B_w_gate: jax.Array,
    B_w_up: jax.Array,
    B_w_down: jax.Array,
):
    del B_x
    any_spec = pl.BlockSpec(memory_space=pl.ANY)
    out = pl.pallas_call(
        _kernel,
        out_shape=jax.ShapeDtypeStruct((S, D), BF16),
        in_specs=[any_spec] * 8,
        out_specs=any_spec,
        scratch_shapes=[
            pltpu.VMEM((S, D), BF16),
            pltpu.VMEM((S // 2, D), U32),
            pltpu.VMEM((3 * NC, D // 2, MC), U32),
            pltpu.VMEM(((VROW + D) // 2, D), U32),
            pltpu.VMEM((H, DH, DH), BF16),
            pltpu.VMEM((D,), BF16),
            pltpu.VMEM((D // 2, D), U32),
            pltpu.VMEM((D // 2, F), U32),
            pltpu.VMEM((D // 2, F), U32),
            pltpu.VMEM((F // 2, D), U32),
            pltpu.VMEM((9, 64, 128), U32),
            pltpu.VMEM((NP, 64, 128), F32),
            pltpu.VMEM((NP, 32, 128), U32),
            pltpu.VMEM((NP, 128, 128), F32),
            pltpu.VMEM((NP, 128, 128), F32),
            pltpu.VMEM((NT, 8, T), F32),
            pltpu.VMEM((2, T // 2, D), U32),
            pltpu.VMEM((S, D), BF16),
            pltpu.VMEM((8, 128), U32),
            pltpu.SemaphoreType.DMA((NT,)),
            pltpu.SemaphoreType.DMA((3 * NC,)),
            pltpu.SemaphoreType.DMA((6,)),
            pltpu.SemaphoreType.DMA((NT - 1 + D // 128,)),
        ],
        compiler_params=pltpu.CompilerParams(
            vmem_limit_bytes=100 * 1024 * 1024,
            disable_bounds_checks=True,
            disable_semaphore_checks=True,
        ),
        name="hedgehog_mod",
    )(A_x.reshape(S, D), A_wqkv, A_w_phi, A_wo, B_w_r, B_w_gate, B_w_up, B_w_down)
    return out.reshape(1, S, D)
```

```python
import jax
import jax.numpy as jnp
from jax import lax
import jax.experimental.pallas as pl
import jax.experimental.pallas.tpu as pltpu

S, D, H, DH, F = 2048, 1024, 32, 32, 3584
T = 256
NT = S // T
MC = 256
NC = D // MC
PC = MC // 64
NP = H // 2
FC = 512
LNP = 16
PATTERN = "PfQfWfnfmfWf"
KPIECES = (2, 2, 1, 0)
VPIECES = (1, 1, 1, 0)
KROW = D + 16
VROW = KROW + D
LOG2E = 1.4426950408889634
EPS_LN = 1.0013580322265625e-05
F32 = jnp.float32
BF16 = jnp.bfloat16
U32 = jnp.uint32

_NT_DIMS = (((1,), (1,)), ((), ()))


def _dot_nt(a, b):
    return lax.dot_general(a, b, _NT_DIMS, preferred_element_type=F32)


def _dot(a, b):
    return jnp.dot(a, b, preferred_element_type=F32)


def _rb(x):
    return x.astype(BF16).astype(F32)


def _pk(x):
    return pltpu.bitcast(x, U32)


def _upk(x):
    return pltpu.bitcast(x, BF16)


def _phi_pair(p, link=None):
    pos, neg = [], []
    for a in range(2):
        ph = p[32 * a:32 * a + 32, :]
        mx = jnp.max(ph, axis=0, keepdims=True)
        mn = jnp.min(ph, axis=0, keepdims=True)
        if link is not None:
            mx, mn = link.start(mx, mn)
        ep = jnp.exp2(ph - mx)
        en = jnp.exp2(mn - ph)
        pos.append(ep * pl.reciprocal(jnp.sum(ep, axis=0, keepdims=True), approx=True))
        neg.append(en * pl.reciprocal(jnp.sum(en, axis=0, keepdims=True), approx=True))
        if link is not None:
            link.done(pos[-1], neg[-1])
    return jnp.concatenate(pos + neg, axis=0)


def _silu(x):
    h = 0.5 * x
    return h + h * jnp.tanh(h)


def _kernel(x_hbm, wqkv_hbm, wphi_hbm, wo_hbm, wr_hbm, wg_hbm, wu_hbm, wd_hbm, out_hbm,
            x_buf, xn_buf, w_buf, wt_buf, wphi_buf, wr_buf, wo_buf, wg_buf, wu_buf, wd_buf,
            bdt_buf, g_acc, g_buf, z_acc, zb_buf, r_buf, o_buf, out_buf, zero_buf,
            sem_x, sem_w, sem_s, sem_o):
    x_cp = [pltpu.make_async_copy(x_hbm.at[pl.ds(i * T, T), :], x_buf.at[pl.ds(i * T, T), :], sem_x.at[i])
            for i in range(NT)]
    w_cp = [pltpu.make_async_copy(wqkv_hbm.bitcast(U32).at[:, pl.ds(j * MC, MC)], w_buf.at[j], sem_w.at[j])
            for j in range(3 * NC)]
    q_cp, k_cp, v_cp = w_cp[:NC], w_cp[NC:2 * NC], w_cp[2 * NC:]
    phi_cp = pltpu.make_async_copy(wphi_hbm, wphi_buf, sem_s.at[0])
    wr_cp = pltpu.make_async_copy(wr_hbm, wr_buf, sem_s.at[1])
    wo_cp = pltpu.make_async_copy(wo_hbm.bitcast(U32), wo_buf, sem_s.at[2])
    f_cp = [pltpu.make_async_copy(wg_hbm.bitcast(U32), wg_buf, sem_s.at[3]),
            pltpu.make_async_copy(wu_hbm.bitcast(U32), wu_buf, sem_s.at[4]),
            pltpu.make_async_copy(wd_hbm.bitcast(U32), wd_buf, sem_s.at[5])]

    copies = [x_cp[0], wr_cp, v_cp[0], x_cp[1], v_cp[1], phi_cp, k_cp[0], k_cp[1], v_cp[2], k_cp[2],
              v_cp[3], k_cp[3]] + x_cp[2:] + q_cp + [wo_cp] + f_cp

    def start_all(j, carry):
        for k, cp in enumerate(copies):
            pl.when((k + 2) * j == j)(cp.start)
        zero_buf[...] = jnp.zeros_like(zero_buf)
        return carry

    lax.fori_loop(0, 2, start_all, 0)

    def tie(w, dep):
        acc = None
        for r in range(0, dep.shape[0], 8):
            for c in range(0, dep.shape[1], 128):
                piece = dep[r:r + 8, c:c + 128]
                acc = piece if acc is None else acc | piece
        first = w[:8, :128] | (acc & zero_buf[...])
        return jnp.concatenate([jnp.concatenate([first, w[:8, 128:]], axis=1), w[8:, :]], axis=0)

    def after(x, dep):
        z = pltpu.bitcast(dep, U32)[:x.shape[0], :] & zero_buf[:x.shape[0], :]
        return pltpu.bitcast(pltpu.bitcast(x, U32) | z, F32)

    class Link:
        def __init__(self):
            self.prev = None

        def start(self, mx, mn):
            if self.prev is None:
                return mx, mn
            return after(mx, self.prev[0]), after(mn, self.prev[1])

        def done(self, pos, neg):
            self.prev = (pos[24:32, :], neg[24:32, :])

    side = []

    def take_side():
        f = side.pop(0) if side else None
        return None if f is None else f()

    def layer_norm(i, piece=0, npieces=1):
        n = T // npieces
        r0 = i * T + piece * n
        x = x_buf[r0:r0 + n, :].astype(F32)
        m = jnp.mean(x, axis=-1, keepdims=True)
        mb = _rb(m)
        d = x - mb
        v = jnp.mean(d * d, axis=-1, keepdims=True) - (m - mb) * (m - mb)
        den = _rb(jnp.sqrt(_rb(_rb(v) + EPS_LN)))
        inv = pl.reciprocal(den, approx=True)
        inv = inv * (2.0 - den * inv)
        xn = _pk((_rb(d) * inv).astype(BF16))
        xn_buf[r0 // 2:(r0 + n) // 2, :] = xn
        return xn

    def ln_pieces(i):
        return [lambda p=p: layer_norm(i, p, LNP) for p in range(LNP)]

    def load_wt(r0, r1, dep=None, dep2=None):
        w = wt_buf[r0 // 2:r1 // 2, :]
        if dep is not None:
            w = tie(w, dep)
        if dep2 is not None:
            w = jnp.concatenate([w[:, :D // 2], tie(w[:, D // 2:], dep2)], axis=1)
        return _upk(w)

    def fold(j):
        for u in range(MC // 128):
            w = _upk(w_buf[j, :, u * 128:(u + 1) * 128])
            if j < 2 * NC:
                r = _dot_nt(_upk(bdt_buf[(2 * j + u) % 8]), w) * LOG2E
            elif j == 2 * NC:
                r = _dot_nt(_upk(bdt_buf[8]), w)
            else:
                r = w.astype(F32).T
            row = (j * MC + u * 128 + (KROW - D if j >= NC else 0)) // 2
            wt_buf[row:row + 64, :] = _pk(r.astype(BF16))

    ri = lax.broadcasted_iota(jnp.int32, (128, 128), 0)
    ci = lax.broadcasted_iota(jnp.int32, (128, 128), 1)

    def build_bdt():
        same_head = (ri // 32) == (ci // 32)
        e_r = lax.broadcasted_iota(jnp.int32, (128, 32), 0)
        e_c = lax.broadcasted_iota(jnp.int32, (128, 32), 1)
        tile_eye = jnp.where((e_r % 32) == e_c, 1.0, 0.0).astype(BF16)
        for g in range(8):
            wg4 = wphi_buf[4 * g:4 * g + 4].reshape(128, 32)
            bdt_buf[g] = _pk(jnp.where(same_head, _dot_nt(tile_eye, wg4), 0.0).astype(BF16))

    class KV:
        def __init__(self, i):
            self.i = i
            self.pk, self.vt, self.ph = {}, {}, {}

        def half(self, r0, r1, n, pieces):
            row = (self.i * T + n * 128) // 2
            deps = [take_side() for _ in range(pieces)]
            return _dot_nt(load_wt(r0, r1, *deps), _upk(xn_buf[row:row + 64, :]))

        def proj(self, r0, r1, pieces):
            return jnp.concatenate([self.half(r0, r1, n, pieces) for n in range(2)], axis=1)

        def k(self, c, pieces=0):
            if c == 0:
                kr = self.proj(KROW - 16, KROW + MC, pieces)
                r_buf[self.i] = kr[:8, :]
                self.pk[c] = kr[16:, :]
            else:
                self.pk[c] = self.proj(KROW + c * MC, KROW + (c + 1) * MC, pieces)

        def v(self, c, pieces=0):
            self.vt[c] = self.proj(VROW + c * MC, VROW + (c + 1) * MC, pieces).astype(BF16)

        def v_half(self, c, n):
            r = self.half(VROW + c * MC, VROW + (c + 1) * MC, n, 0).astype(BF16)
            self.vt[c] = r if n == 0 else jnp.concatenate([self.vt[c], r], axis=1)

        def phi(self, c):
            if c not in self.ph:
                pk = self.pk.pop(c)
                self.ph[c] = []
                for u in range(PC):
                    phi = _phi_pair(pk[64 * u:64 * u + 64, :])
                    z = phi[:, :128] + phi[:, 128:]
                    if self.i > 0:
                        z = z + z_acc[c * PC + u]
                    z_acc[c * PC + u] = z
                    self.ph[c].append((phi.astype(BF16), z))
            return self.ph[c]

        def g(self, c):
            vt = self.vt.pop(c)
            for u, (phi, z) in enumerate(self.phi(c)):
                r = _dot_nt(_upk(tie(_pk(vt[64 * u:64 * u + 64, :]), pltpu.bitcast(z, U32))), phi)
                if self.i == 0:
                    g_acc[c * PC + u] = r
                else:
                    g_acc[c * PC + u] += r

    bdt_buf[8] = _pk(jnp.where(ri == ci, 1.0, 0.0).astype(BF16))
    x_cp[0].wait()
    layer_norm(0)
    t0, t1 = KV(0), KV(1)
    wr_cp.wait()
    v_cp[0].wait()
    fold(2 * NC)
    t0.v_half(0, 0)
    x_cp[1].wait()
    t0.v_half(0, 1)
    layer_norm(1)
    t1.v_half(0, 0)
    v_cp[1].wait()
    fold(2 * NC + 1)
    t1.v_half(0, 1)
    t0.v(1)
    t1.v(1)
    phi_cp.wait()
    k_cp[0].wait()
    wt_buf[D // 2:D // 2 + 8, :] = _pk(
        jnp.broadcast_to(wr_buf[...].astype(F32).reshape(1, D), (16, D)).astype(BF16))
    build_bdt()
    fold(NC)
    t0.k(0)
    t1.k(0)
    t0.g(0)
    t1.phi(0)
    for cp in [k_cp[1], v_cp[2], k_cp[2]]:
        cp.wait()
    fold(NC + 1)
    fold(2 * NC + 2)
    fold(NC + 2)
    t1.g(0)
    t0.k(1)
    t1.k(1)
    t0.k(2)
    t0.g(1)
    t1.k(2)
    t1.g(1)
    t0.v(2)
    t1.v(2)
    t0.g(2)
    t1.phi(2)
    for cp in [v_cp[3], k_cp[3]] + x_cp[2:]:
        cp.wait()
    side += ln_pieces(2)
    fold(NC + 3)
    fold(2 * NC + 3)
    t1.g(2)
    t0.k(3, 2)
    t1.k(3, 2)
    t0.v(3, 2)
    t1.v(3, 2)
    t0.g(3)
    prev = t1
    for i in range(2, NT):
        if i + 1 < NT:
            side += ln_pieces(i + 1)
        kv = KV(i)
        for c in range(NC):
            kv.k(c, KPIECES[c])
            (prev if c == 0 else kv).g((c - 1) % NC)
            kv.v(c, VPIECES[c])
        prev = kv
    prev.g(NC - 1)
    assert not side

    same_head = (lax.broadcasted_iota(jnp.int32, (64, 128), 0) // 32
                 == (lax.broadcasted_iota(jnp.int32, (64, 128), 1) % 64) // 32)
    for p in range(NP):
        g_buf[p] = _pk(jnp.where(same_head, g_acc[p], 0.0).astype(BF16))
        zb_buf[p] = jnp.broadcast_to(jnp.sum(z_acc[p], axis=1, keepdims=True), (128, 128))

    r_all = _rb(r_buf[...])
    tok = (lax.broadcasted_iota(jnp.int32, r_buf.shape, 0) * T
           + lax.broadcasted_iota(jnp.int32, r_buf.shape, 2))
    r_max = jnp.max(r_all)
    idx = jnp.min(jnp.where(r_all == r_max, tok, S - 1))
    sel_tile = idx // T
    blk = pl.multiple_of((idx // 16) * 16, 16)

    def tile_of(j):
        return (sel_tile + 1 + j) % NT

    def out_copy(j):
        rows = pl.ds(pl.multiple_of(tile_of(j) * T, T), T)
        return pltpu.make_async_copy(out_buf.at[rows, :], out_hbm.at[rows, :], sem_o.at[j])

    def last_copy(n):
        rows = pl.ds(pl.multiple_of(sel_tile * T, T), T)
        cols = pl.ds(n * 128, 128)
        return pltpu.make_async_copy(out_buf.at[rows, cols], out_hbm.at[rows, cols], sem_o.at[NT - 1 + n])

    class Q:
        def __init__(self, j):
            self.j = j
            self.row0 = tile_of(j) * (T // 2)
            self.pq = {}

        def proj(self, c, n):
            xn = _upk(xn_buf[pl.ds(pl.multiple_of(self.row0 + n * 64, 64), 64), :])
            self.pq[c, n] = _dot_nt(load_wt(c * MC, (c + 1) * MC), xn)

        def num(self, c, n):
            pq = self.pq.pop((c, n))
            parts = []
            link = Link()
            for u in range(PC):
                phi = _phi_pair(pq[64 * u:64 * u + 64, :], link)
                nd = _dot(_upk(g_buf[c * PC + u]), phi.astype(BF16))
                zp = phi * zb_buf[c * PC + u]
                zp = zp[:64, :] + zp[64:, :]
                for a in range(2):
                    den = jnp.sum(zp[32 * a:32 * a + 32, :], axis=0, keepdims=True)
                    parts.append(nd[32 * a:32 * a + 32, :] * pl.reciprocal(den + 1e-6, approx=True))
            ot = jnp.concatenate(parts, axis=0)
            o_buf[self.j % 2, n * 64:(n + 1) * 64, c * MC:(c + 1) * MC] = _pk(ot.T.astype(BF16))

    def out_cols(j, n, upd=None):
        t = tile_of(j)
        rows = pl.ds(pl.multiple_of(t * T, T), T)
        rows2 = pl.ds(pl.multiple_of(t * (T // 2), T // 2), T // 2)
        cols = slice(n * 128, (n + 1) * 128)
        s = _dot(_upk(o_buf[j % 2]), _upk(wo_buf[:, cols]))
        xn = _upk(xn_buf[rows2, cols]).astype(F32)
        if upd is not None:
            xn = xn + upd[:, cols]
        out_buf[rows, cols] = (x_buf[rows, cols].astype(F32) + s * _silu(xn)).astype(BF16)

    def ffn_steps():
        st = {}
        KH = D // 2

        def apart(r):
            z = zero_buf[...]
            return pltpu.bitcast(pltpu.bitcast(r, U32) | jnp.concatenate([z, z], axis=0), F32)

        def up(w_ref, key, n, h):
            def f():
                xs = _upk(xn_buf[pl.ds(pl.multiple_of(blk // 2, 8), 8), h * KH:(h + 1) * KH])
                r = _dot(xs, _upk(w_ref[h * KH // 2:(h + 1) * KH // 2, n * 128:(n + 1) * 128]))
                st[key, n] = apart(r) if h == 0 else st[key, n] + r
            return f

        def down(c, n):
            def f():
                if ('h', c) not in st:
                    ms = range(c * FC // 128, (c + 1) * FC // 128)
                    st['h', c] = jnp.concatenate(
                        [_silu(st.pop(('g', m))) * st.pop(('u', m)) for m in ms], axis=1).astype(BF16)
                r = _dot(st['h', c], _upk(wd_buf[c * FC // 2:(c + 1) * FC // 2, n * 128:(n + 1) * 128]))
                st['y', n] = apart(r) if c == 0 else st['y', n] + r
            return f

        steps = []
        for c in range(F // FC + 1):
            ups = [up(w, k, m, h) for m in range(c * FC // 128, (c + 1) * FC // 128)
                   for h in range(2) for w, k in ((wg_buf, 'g'), (wu_buf, 'u'))] if c < F // FC else []
            downs = [down(c - 1, n) for n in range(D // 128)] if c > 0 else []
            while ups or downs:
                steps += ups[:2] + downs[:1]
                ups, downs = ups[2:], downs[1:]
        return steps, st

    for cp in q_cp + [wo_cp] + f_cp:
        cp.wait()
    for j in range(NC):
        fold(j)
    ffn, ffn_st = ffn_steps()

    q = Q(0)
    for c in range(NC):
        q.proj(c, 0)
        if c > 0:
            q.num(c - 1, 1)
        q.proj(c, 1)
        q.num(c, 0)

    pending = [None]

    def out_step():
        step = pending.pop(0)
        if step is not None:
            out_cols(*step)
            if step[1] == D // 128 - 1:
                out_copy(step[0]).start()

    for j in range(1, NT):
        qn = Q(j)
        pending += [(j - 1, n) for n in range(D // 128)]
        for c in range(NC):
            for tok in PATTERN:
                if tok == 'P' or tok == 'Q':
                    qn.proj(c, int(tok == 'Q'))
                elif tok == 'n':
                    (q if c == 0 else qn).num((c - 1) % NC, 1)
                elif tok == 'm':
                    qn.num(c, 0)
                elif tok == 'W':
                    out_step()
                else:
                    ffn.pop(0)()
        q = qn
    assert not ffn
    q.num(NC - 1, 1)
    out_step()

    y = jnp.concatenate([ffn_st['y', n] for n in range(D // 128)], axis=1)
    sub = lax.broadcasted_iota(jnp.int32, (16, D), 0)
    y_row = jnp.sum(jnp.where(sub == idx - blk, y, 0.0), axis=0, keepdims=True)
    gate = 1.0 / (1.0 + jnp.exp(-jnp.full((1, D), r_max, F32)))
    trow = lax.broadcasted_iota(jnp.int32, (T, D), 0)
    upd = jnp.where(trow == idx - sel_tile * T, y_row * gate, 0.0)
    for n in range(D // 128):
        out_cols(NT - 1, n, upd)
        last_copy(n).start()
    for j in range(NT - 1):
        out_copy(j).wait()
    for n in range(D // 128):
        last_copy(n).wait()


@jax.jit
def pallas_recurrent_scan__linear_kernel_hedgehog__moe_arch_mod__prompt_kernel(
    A_x: jax.Array,
    A_wqkv: jax.Array,
    A_w_phi: jax.Array,
    A_wo: jax.Array,
    B_x: jax.Array,
    B_w_r: jax.Array,
    B_w_gate: jax.Array,
    B_w_up: jax.Array,
    B_w_down: jax.Array,
):
    del B_x
    any_spec = pl.BlockSpec(memory_space=pl.ANY)
    out = pl.pallas_call(
        _kernel,
        out_shape=jax.ShapeDtypeStruct((S, D), BF16),
        in_specs=[any_spec] * 8,
        out_specs=any_spec,
        scratch_shapes=[
            pltpu.VMEM((S, D), BF16),
            pltpu.VMEM((S // 2, D), U32),
            pltpu.VMEM((3 * NC, D // 2, MC), U32),
            pltpu.VMEM(((VROW + D) // 2, D), U32),
            pltpu.VMEM((H, DH, DH), BF16),
            pltpu.VMEM((D,), BF16),
            pltpu.VMEM((D // 2, D), U32),
            pltpu.VMEM((D // 2, F), U32),
            pltpu.VMEM((D // 2, F), U32),
            pltpu.VMEM((F // 2, D), U32),
            pltpu.VMEM((9, 64, 128), U32),
            pltpu.VMEM((NP, 64, 128), F32),
            pltpu.VMEM((NP, 32, 128), U32),
            pltpu.VMEM((NP, 128, 128), F32),
            pltpu.VMEM((NP, 128, 128), F32),
            pltpu.VMEM((NT, 8, T), F32),
            pltpu.VMEM((2, T // 2, D), U32),
            pltpu.VMEM((S, D), BF16),
            pltpu.VMEM((8, 128), U32),
            pltpu.SemaphoreType.DMA((NT,)),
            pltpu.SemaphoreType.DMA((3 * NC,)),
            pltpu.SemaphoreType.DMA((6,)),
            pltpu.SemaphoreType.DMA((NT - 1 + D // 128,)),
        ],
        compiler_params=pltpu.CompilerParams(
            vmem_limit_bytes=100 * 1024 * 1024,
            disable_bounds_checks=True,
            disable_semaphore_checks=True,
        ),
        name="hedgehog_mod",
    )(A_x.reshape(S, D), A_wqkv, A_w_phi, A_wo, B_w_r, B_w_gate, B_w_up, B_w_down)
    return out.reshape(1, S, D)
```

```python
import jax
import jax.numpy as jnp
from jax import lax
import jax.experimental.pallas as pl
import jax.experimental.pallas.tpu as pltpu

S, D, H, DH, F = 2048, 1024, 32, 32, 3584
T = 256
NT = S // T
MC = 256
NC = D // MC
PC = MC // 64
NP = H // 2
FC = 512
LNP = 16
PATTERN = "PfQfWfnfmfWf"
KPIECES = (2, 2, 1, 0)
VPIECES = (1, 1, 1, 0)
KROW = D + 16
VROW = KROW + D
LOG2E = 1.4426950408889634
EPS_LN = 1.0013580322265625e-05
F32 = jnp.float32
BF16 = jnp.bfloat16
U32 = jnp.uint32

_NT_DIMS = (((1,), (1,)), ((), ()))


def _dot_nt(a, b):
    return lax.dot_general(a, b, _NT_DIMS, preferred_element_type=F32)


def _dot(a, b):
    return jnp.dot(a, b, preferred_element_type=F32)


def _rb(x):
    return x.astype(BF16).astype(F32)


def _pk(x):
    return pltpu.bitcast(x, U32)


def _upk(x):
    return pltpu.bitcast(x, BF16)


def _phi_pair(p, link=None, link_after=None):
    pos, neg = [], []
    for a in range(2):
        ph = p[32 * a:32 * a + 32, :]
        mx = jnp.max(ph, axis=0, keepdims=True)
        mn = jnp.min(ph, axis=0, keepdims=True)
        if link:
            mx = link[0](mx)
        ep = jnp.exp2(ph - mx)
        en = jnp.exp2(mn - ph)
        if link is not None:
            link[:] = [link_after(ep[24:32, :])]
        pos.append(ep * pl.reciprocal(jnp.sum(ep, axis=0, keepdims=True), approx=True))
        neg.append(en * pl.reciprocal(jnp.sum(en, axis=0, keepdims=True), approx=True))
    return jnp.concatenate(pos + neg, axis=0)


def _silu(x):
    h = 0.5 * x
    return h + h * jnp.tanh(h)


def _kernel(x_hbm, wqkv_hbm, wphi_hbm, wo_hbm, wr_hbm, wg_hbm, wu_hbm, wd_hbm, out_hbm,
            x_buf, xn_buf, w_buf, wt_buf, wphi_buf, wr_buf, wo_buf, wg_buf, wu_buf, wd_buf,
            bdt_buf, g_acc, g_buf, z_acc, zb_buf, r_buf, o_buf, out_buf, zero_buf,
            sem_x, sem_w, sem_s, sem_o):
    x_cp = [pltpu.make_async_copy(x_hbm.at[pl.ds(i * T, T), :], x_buf.at[pl.ds(i * T, T), :], sem_x.at[i])
            for i in range(NT)]
    w_cp = [pltpu.make_async_copy(wqkv_hbm.bitcast(U32).at[:, pl.ds(j * MC, MC)], w_buf.at[j], sem_w.at[j])
            for j in range(3 * NC)]
    q_cp, k_cp, v_cp = w_cp[:NC], w_cp[NC:2 * NC], w_cp[2 * NC:]
    phi_cp = pltpu.make_async_copy(wphi_hbm, wphi_buf, sem_s.at[0])
    wr_cp = pltpu.make_async_copy(wr_hbm, wr_buf, sem_s.at[1])
    wo_cp = pltpu.make_async_copy(wo_hbm.bitcast(U32), wo_buf, sem_s.at[2])
    f_cp = [pltpu.make_async_copy(wg_hbm.bitcast(U32), wg_buf, sem_s.at[3]),
            pltpu.make_async_copy(wu_hbm.bitcast(U32), wu_buf, sem_s.at[4]),
            pltpu.make_async_copy(wd_hbm.bitcast(U32), wd_buf, sem_s.at[5])]

    copies = [x_cp[0], wr_cp, v_cp[0], x_cp[1], v_cp[1], phi_cp, k_cp[0], k_cp[1], v_cp[2], k_cp[2],
              v_cp[3], k_cp[3]] + x_cp[2:] + q_cp + [wo_cp] + f_cp

    def start_all(j, carry):
        for k, cp in enumerate(copies):
            pl.when((k + 2) * j == j)(cp.start)
        zero_buf[...] = jnp.zeros_like(zero_buf)
        return carry

    lax.fori_loop(0, 2, start_all, 0)

    def tie(w, dep):
        acc = None
        for r in range(0, dep.shape[0], 8):
            for c in range(0, dep.shape[1], 128):
                piece = dep[r:r + 8, c:c + 128]
                acc = piece if acc is None else acc | piece
        first = w[:8, :128] | (acc & zero_buf[...])
        return jnp.concatenate([jnp.concatenate([first, w[:8, 128:]], axis=1), w[8:, :]], axis=0)

    def after(dep):
        z = pltpu.bitcast(dep, U32)[:1, :] & zero_buf[:1, :]
        return lambda x: pltpu.bitcast(pltpu.bitcast(x, U32) | z, F32)

    side = []

    def take_side():
        f = side.pop(0) if side else None
        return None if f is None else f()

    def layer_norm(i, piece=0, npieces=1):
        n = T // npieces
        r0 = i * T + piece * n
        x = x_buf[r0:r0 + n, :].astype(F32)
        m = jnp.mean(x, axis=-1, keepdims=True)
        mb = _rb(m)
        d = x - mb
        v = jnp.mean(d * d, axis=-1, keepdims=True) - (m - mb) * (m - mb)
        den = _rb(jnp.sqrt(_rb(_rb(v) + EPS_LN)))
        inv = pl.reciprocal(den, approx=True)
        inv = inv * (2.0 - den * inv)
        xn = _pk((_rb(d) * inv).astype(BF16))
        xn_buf[r0 // 2:(r0 + n) // 2, :] = xn
        return xn

    def ln_pieces(i):
        return [lambda p=p: layer_norm(i, p, LNP) for p in range(LNP)]

    def load_wt(r0, r1, dep=None, dep2=None):
        w = wt_buf[r0 // 2:r1 // 2, :]
        if dep is not None:
            w = tie(w, dep)
        if dep2 is not None:
            w = jnp.concatenate([w[:, :D // 2], tie(w[:, D // 2:], dep2)], axis=1)
        return _upk(w)

    def fold(j):
        for u in range(MC // 128):
            w = _upk(w_buf[j, :, u * 128:(u + 1) * 128])
            if j < 2 * NC:
                r = _dot_nt(_upk(bdt_buf[(2 * j + u) % 8]), w) * LOG2E
            elif j == 2 * NC:
                r = _dot_nt(_upk(bdt_buf[8]), w)
            else:
                r = w.astype(F32).T
            row = (j * MC + u * 128 + (KROW - D if j >= NC else 0)) // 2
            wt_buf[row:row + 64, :] = _pk(r.astype(BF16))

    ri = lax.broadcasted_iota(jnp.int32, (128, 128), 0)
    ci = lax.broadcasted_iota(jnp.int32, (128, 128), 1)

    def build_bdt():
        same_head = (ri // 32) == (ci // 32)
        e_r = lax.broadcasted_iota(jnp.int32, (128, 32), 0)
        e_c = lax.broadcasted_iota(jnp.int32, (128, 32), 1)
        tile_eye = jnp.where((e_r % 32) == e_c, 1.0, 0.0).astype(BF16)
        for g in range(8):
            wg4 = wphi_buf[4 * g:4 * g + 4].reshape(128, 32)
            bdt_buf[g] = _pk(jnp.where(same_head, _dot_nt(tile_eye, wg4), 0.0).astype(BF16))

    class KV:
        def __init__(self, i):
            self.i = i
            self.pk, self.vt, self.ph = {}, {}, {}

        def half(self, r0, r1, n, pieces):
            row = (self.i * T + n * 128) // 2
            deps = [take_side() for _ in range(pieces)]
            return _dot_nt(load_wt(r0, r1, *deps), _upk(xn_buf[row:row + 64, :]))

        def proj(self, r0, r1, pieces):
            return jnp.concatenate([self.half(r0, r1, n, pieces) for n in range(2)], axis=1)

        def k(self, c, pieces=0):
            if c == 0:
                kr = self.proj(KROW - 16, KROW + MC, pieces)
                r_buf[self.i] = kr[:8, :]
                self.pk[c] = kr[16:, :]
            else:
                self.pk[c] = self.proj(KROW + c * MC, KROW + (c + 1) * MC, pieces)

        def v(self, c, pieces=0):
            self.vt[c] = self.proj(VROW + c * MC, VROW + (c + 1) * MC, pieces).astype(BF16)

        def v_half(self, c, n):
            r = self.half(VROW + c * MC, VROW + (c + 1) * MC, n, 0).astype(BF16)
            self.vt[c] = r if n == 0 else jnp.concatenate([self.vt[c], r], axis=1)

        def phi(self, c):
            if c not in self.ph:
                pk = self.pk.pop(c)
                self.ph[c] = []
                for u in range(PC):
                    phi = _phi_pair(pk[64 * u:64 * u + 64, :])
                    z = phi[:, :128] + phi[:, 128:]
                    if self.i > 0:
                        z = z + z_acc[c * PC + u]
                    z_acc[c * PC + u] = z
                    self.ph[c].append((phi.astype(BF16), z))
            return self.ph[c]

        def g(self, c):
            vt = self.vt.pop(c)
            for u, (phi, z) in enumerate(self.phi(c)):
                r = _dot_nt(_upk(tie(_pk(vt[64 * u:64 * u + 64, :]), pltpu.bitcast(z, U32))), phi)
                if self.i == 0:
                    g_acc[c * PC + u] = r
                else:
                    g_acc[c * PC + u] += r

    bdt_buf[8] = _pk(jnp.where(ri == ci, 1.0, 0.0).astype(BF16))
    x_cp[0].wait()
    layer_norm(0)
    t0, t1 = KV(0), KV(1)
    wr_cp.wait()
    v_cp[0].wait()
    fold(2 * NC)
    t0.v_half(0, 0)
    x_cp[1].wait()
    t0.v_half(0, 1)
    layer_norm(1)
    t1.v_half(0, 0)
    v_cp[1].wait()
    fold(2 * NC + 1)
    t1.v_half(0, 1)
    t0.v(1)
    t1.v(1)
    phi_cp.wait()
    k_cp[0].wait()
    wt_buf[D // 2:D // 2 + 8, :] = _pk(
        jnp.broadcast_to(wr_buf[...].astype(F32).reshape(1, D), (16, D)).astype(BF16))
    build_bdt()
    fold(NC)
    t0.k(0)
    t1.k(0)
    t0.g(0)
    t1.phi(0)
    for cp in [k_cp[1], v_cp[2], k_cp[2]]:
        cp.wait()
    fold(NC + 1)
    fold(2 * NC + 2)
    fold(NC + 2)
    t1.g(0)
    t0.k(1)
    t1.k(1)
    t0.k(2)
    t0.g(1)
    t1.k(2)
    t1.g(1)
    t0.v(2)
    t1.v(2)
    t0.g(2)
    t1.phi(2)
    for cp in [v_cp[3], k_cp[3]] + x_cp[2:]:
        cp.wait()
    side += ln_pieces(2)
    fold(NC + 3)
    fold(2 * NC + 3)
    t1.g(2)
    t0.k(3, 2)
    t1.k(3, 2)
    t0.v(3, 2)
    t1.v(3, 2)
    t0.g(3)
    prev = t1
    for i in range(2, NT):
        if i + 1 < NT:
            side += ln_pieces(i + 1)
        kv = KV(i)
        for c in range(NC):
            kv.k(c, KPIECES[c])
            (prev if c == 0 else kv).g((c - 1) % NC)
            kv.v(c, VPIECES[c])
        prev = kv
    prev.g(NC - 1)
    assert not side

    same_head = (lax.broadcasted_iota(jnp.int32, (64, 128), 0) // 32
                 == (lax.broadcasted_iota(jnp.int32, (64, 128), 1) % 64) // 32)
    for p in range(NP):
        g_buf[p] = _pk(jnp.where(same_head, g_acc[p], 0.0).astype(BF16))
        zb_buf[p] = jnp.broadcast_to(jnp.sum(z_acc[p], axis=1, keepdims=True), (128, 128))

    r_all = _rb(r_buf[...])
    tok = (lax.broadcasted_iota(jnp.int32, r_buf.shape, 0) * T
           + lax.broadcasted_iota(jnp.int32, r_buf.shape, 2))
    r_max = jnp.max(r_all)
    idx = jnp.min(jnp.where(r_all == r_max, tok, S - 1))
    sel_tile = idx // T
    blk = pl.multiple_of((idx // 16) * 16, 16)

    def tile_of(j):
        return (sel_tile + 1 + j) % NT

    def out_copy(j):
        rows = pl.ds(pl.multiple_of(tile_of(j) * T, T), T)
        return pltpu.make_async_copy(out_buf.at[rows, :], out_hbm.at[rows, :], sem_o.at[j])

    def last_copy(n):
        rows = pl.ds(pl.multiple_of(sel_tile * T, T), T)
        cols = pl.ds(n * 128, 128)
        return pltpu.make_async_copy(out_buf.at[rows, cols], out_hbm.at[rows, cols], sem_o.at[NT - 1 + n])

    class Q:
        def __init__(self, j):
            self.j = j
            self.row0 = tile_of(j) * (T // 2)
            self.pq = {}

        def proj(self, c, n):
            xn = _upk(xn_buf[pl.ds(pl.multiple_of(self.row0 + n * 64, 64), 64), :])
            self.pq[c, n] = _dot_nt(load_wt(c * MC, (c + 1) * MC), xn)

        def num(self, c, n):
            pq = self.pq.pop((c, n))
            parts = []
            link = []
            for u in range(PC):
                phi = _phi_pair(pq[64 * u:64 * u + 64, :], link, after)
                nd = _dot(_upk(g_buf[c * PC + u]), phi.astype(BF16))
                zp = phi * zb_buf[c * PC + u]
                zp = zp[:64, :] + zp[64:, :]
                for a in range(2):
                    den = jnp.sum(zp[32 * a:32 * a + 32, :], axis=0, keepdims=True)
                    parts.append(nd[32 * a:32 * a + 32, :] * pl.reciprocal(den + 1e-6, approx=True))
            ot = jnp.concatenate(parts, axis=0)
            o_buf[self.j % 2, n * 64:(n + 1) * 64, c * MC:(c + 1) * MC] = _pk(ot.T.astype(BF16))

    def out_cols(j, n, upd=None):
        t = tile_of(j)
        rows = pl.ds(pl.multiple_of(t * T, T), T)
        rows2 = pl.ds(pl.multiple_of(t * (T // 2), T // 2), T // 2)
        cols = slice(n * 128, (n + 1) * 128)
        s = _dot(_upk(o_buf[j % 2]), _upk(wo_buf[:, cols]))
        xn = _upk(xn_buf[rows2, cols]).astype(F32)
        if upd is not None:
            xn = xn + upd[:, cols]
        out_buf[rows, cols] = (x_buf[rows, cols].astype(F32) + s * _silu(xn)).astype(BF16)

    def ffn_steps():
        st = {}
        KH = D // 2

        def apart(r):
            z = zero_buf[...]
            return pltpu.bitcast(pltpu.bitcast(r, U32) | jnp.concatenate([z, z], axis=0), F32)

        def up(w_ref, key, n, h):
            def f():
                xs = _upk(xn_buf[pl.ds(pl.multiple_of(blk // 2, 8), 8), h * KH:(h + 1) * KH])
                r = _dot(xs, _upk(w_ref[h * KH // 2:(h + 1) * KH // 2, n * 128:(n + 1) * 128]))
                st[key, n] = apart(r) if h == 0 else st[key, n] + r
            return f

        def down(c, n):
            def f():
                if ('h', c) not in st:
                    ms = range(c * FC // 128, (c + 1) * FC // 128)
                    st['h', c] = jnp.concatenate(
                        [_silu(st.pop(('g', m))) * st.pop(('u', m)) for m in ms], axis=1).astype(BF16)
                r = _dot(st['h', c], _upk(wd_buf[c * FC // 2:(c + 1) * FC // 2, n * 128:(n + 1) * 128]))
                st['y', n] = apart(r) if c == 0 else st['y', n] + r
            return f

        steps = []
        for c in range(F // FC + 1):
            ups = [up(w, k, m, h) for m in range(c * FC // 128, (c + 1) * FC // 128)
                   for h in range(2) for w, k in ((wg_buf, 'g'), (wu_buf, 'u'))] if c < F // FC else []
            downs = [down(c - 1, n) for n in range(D // 128)] if c > 0 else []
            while ups or downs:
                steps += ups[:2] + downs[:1]
                ups, downs = ups[2:], downs[1:]
        return steps, st

    for cp in q_cp + [wo_cp] + f_cp:
        cp.wait()
    for j in range(NC):
        fold(j)
    ffn, ffn_st = ffn_steps()

    q = Q(0)
    for c in range(NC):
        q.proj(c, 0)
        if c > 0:
            q.num(c - 1, 1)
        q.proj(c, 1)
        q.num(c, 0)

    pending = [None]

    def out_step():
        step = pending.pop(0)
        if step is not None:
            out_cols(*step)
            if step[1] == D // 128 - 1:
                out_copy(step[0]).start()

    for j in range(1, NT):
        qn = Q(j)
        pending += [(j - 1, n) for n in range(D // 128)]
        for c in range(NC):
            for tok in PATTERN:
                if tok == 'P' or tok == 'Q':
                    qn.proj(c, int(tok == 'Q'))
                elif tok == 'n':
                    (q if c == 0 else qn).num((c - 1) % NC, 1)
                elif tok == 'm':
                    qn.num(c, 0)
                elif tok == 'W':
                    out_step()
                else:
                    ffn.pop(0)()
        q = qn
    assert not ffn
    q.num(NC - 1, 1)
    out_step()

    y = jnp.concatenate([ffn_st['y', n] for n in range(D // 128)], axis=1)
    sub = lax.broadcasted_iota(jnp.int32, (16, D), 0)
    y_row = jnp.sum(jnp.where(sub == idx - blk, y, 0.0), axis=0, keepdims=True)
    gate = 1.0 / (1.0 + jnp.exp(-jnp.full((1, D), r_max, F32)))
    trow = lax.broadcasted_iota(jnp.int32, (T, D), 0)
    upd = jnp.where(trow == idx - sel_tile * T, y_row * gate, 0.0)
    for n in range(D // 128):
        out_cols(NT - 1, n, upd)
        last_copy(n).start()
    for j in range(NT - 1):
        out_copy(j).wait()
    for n in range(D // 128):
        last_copy(n).wait()


@jax.jit
def pallas_recurrent_scan__linear_kernel_hedgehog__moe_arch_mod__prompt_kernel(
    A_x: jax.Array,
    A_wqkv: jax.Array,
    A_w_phi: jax.Array,
    A_wo: jax.Array,
    B_x: jax.Array,
    B_w_r: jax.Array,
    B_w_gate: jax.Array,
    B_w_up: jax.Array,
    B_w_down: jax.Array,
):
    del B_x
    any_spec = pl.BlockSpec(memory_space=pl.ANY)
    out = pl.pallas_call(
        _kernel,
        out_shape=jax.ShapeDtypeStruct((S, D), BF16),
        in_specs=[any_spec] * 8,
        out_specs=any_spec,
        scratch_shapes=[
            pltpu.VMEM((S, D), BF16),
            pltpu.VMEM((S // 2, D), U32),
            pltpu.VMEM((3 * NC, D // 2, MC), U32),
            pltpu.VMEM(((VROW + D) // 2, D), U32),
            pltpu.VMEM((H, DH, DH), BF16),
            pltpu.VMEM((D,), BF16),
            pltpu.VMEM((D // 2, D), U32),
            pltpu.VMEM((D // 2, F), U32),
            pltpu.VMEM((D // 2, F), U32),
            pltpu.VMEM((F // 2, D), U32),
            pltpu.VMEM((9, 64, 128), U32),
            pltpu.VMEM((NP, 64, 128), F32),
            pltpu.VMEM((NP, 32, 128), U32),
            pltpu.VMEM((NP, 128, 128), F32),
            pltpu.VMEM((NP, 128, 128), F32),
            pltpu.VMEM((NT, 8, T), F32),
            pltpu.VMEM((2, T // 2, D), U32),
            pltpu.VMEM((S, D), BF16),
            pltpu.VMEM((8, 128), U32),
            pltpu.SemaphoreType.DMA((NT,)),
            pltpu.SemaphoreType.DMA((3 * NC,)),
            pltpu.SemaphoreType.DMA((6,)),
            pltpu.SemaphoreType.DMA((NT - 1 + D // 128,)),
        ],
        compiler_params=pltpu.CompilerParams(
            vmem_limit_bytes=100 * 1024 * 1024,
            disable_bounds_checks=True,
            disable_semaphore_checks=True,
        ),
        name="hedgehog_mod",
    )(A_x.reshape(S, D), A_wqkv, A_w_phi, A_wo, B_w_r, B_w_gate, B_w_up, B_w_down)
    return out.reshape(1, S, D)
```

```python
import jax
import jax.numpy as jnp
from jax import lax
import jax.experimental.pallas as pl
import jax.experimental.pallas.tpu as pltpu

S, D, H, DH, F = 2048, 1024, 32, 32, 3584
T = 256
NT = S // T
MC = 256
NC = D // MC
PC = MC // 64
NP = H // 2
FC = 512
LNP = 16
PATTERN = "PfQfWfnfmfWf"
KPIECES = (2, 2, 2, 0)
VPIECES = (1, 1, 0, 0)
KROW = D + 16
VROW = KROW + D
LOG2E = 1.4426950408889634
EPS_LN = 1.0013580322265625e-05
F32 = jnp.float32
BF16 = jnp.bfloat16
U32 = jnp.uint32

_NT_DIMS = (((1,), (1,)), ((), ()))


def _dot_nt(a, b):
    return lax.dot_general(a, b, _NT_DIMS, preferred_element_type=F32)


def _dot(a, b):
    return jnp.dot(a, b, preferred_element_type=F32)


def _rb(x):
    return x.astype(BF16).astype(F32)


def _pk(x):
    return pltpu.bitcast(x, U32)


def _upk(x):
    return pltpu.bitcast(x, BF16)


def _phi_pair(p, link=None, link_after=None):
    pos, neg, scale = [], [], []
    for a in range(2):
        ph = p[32 * a:32 * a + 32, :]
        mx = jnp.max(ph, axis=0, keepdims=True)
        mn = jnp.min(ph, axis=0, keepdims=True)
        if link:
            mx = link[0](mx)
        ep = jnp.exp2(ph - mx)
        en = jnp.exp2(mn - ph)
        sp = jnp.sum(ep, axis=0, keepdims=True)
        rn = pl.reciprocal(jnp.sum(en, axis=0, keepdims=True), approx=True)
        if link is None:
            pos.append(ep * pl.reciprocal(sp, approx=True))
            neg.append(en * rn)
        else:
            link[:] = [link_after(ep[24:32, :])]
            pos.append(ep)
            neg.append(en * (sp * rn))
            scale.append(sp)
    return jnp.concatenate(pos + neg, axis=0), scale


def _silu(x):
    h = 0.5 * x
    return h + h * jnp.tanh(h)


def _kernel(x_hbm, wqkv_hbm, wphi_hbm, wo_hbm, wr_hbm, wg_hbm, wu_hbm, wd_hbm, out_hbm,
            x_buf, xn_buf, w_buf, wt_buf, wphi_buf, wr_buf, wo_buf, wg_buf, wu_buf, wd_buf,
            bdt_buf, g_acc, g_buf, z_acc, zb_buf, r_buf, o_buf, out_buf, zero_buf,
            sem_x, sem_w, sem_s, sem_o):
    x_cp = [pltpu.make_async_copy(x_hbm.at[pl.ds(i * T, T), :], x_buf.at[pl.ds(i * T, T), :], sem_x.at[i])
            for i in range(NT)]
    w_cp = [pltpu.make_async_copy(wqkv_hbm.bitcast(U32).at[:, pl.ds(j * MC, MC)], w_buf.at[j], sem_w.at[j])
            for j in range(3 * NC)]
    q_cp, k_cp, v_cp = w_cp[:NC], w_cp[NC:2 * NC], w_cp[2 * NC:]
    phi_cp = pltpu.make_async_copy(wphi_hbm, wphi_buf, sem_s.at[0])
    wr_cp = pltpu.make_async_copy(wr_hbm, wr_buf, sem_s.at[1])
    wo_cp = pltpu.make_async_copy(wo_hbm.bitcast(U32), wo_buf, sem_s.at[2])
    f_cp = [pltpu.make_async_copy(wg_hbm.bitcast(U32), wg_buf, sem_s.at[3]),
            pltpu.make_async_copy(wu_hbm.bitcast(U32), wu_buf, sem_s.at[4]),
            pltpu.make_async_copy(wd_hbm.bitcast(U32), wd_buf, sem_s.at[5])]

    copies = [x_cp[0], wr_cp, v_cp[0], x_cp[1], v_cp[1], phi_cp, k_cp[0], k_cp[1], v_cp[2], k_cp[2],
              v_cp[3], k_cp[3]] + x_cp[2:] + q_cp + [wo_cp] + f_cp

    def start_all(j, carry):
        for k, cp in enumerate(copies):
            pl.when((k + 2) * j == j)(cp.start)
        zero_buf[...] = jnp.zeros_like(zero_buf)
        return carry

    lax.fori_loop(0, 2, start_all, 0)

    def tie(w, dep):
        acc = None
        for r in range(0, dep.shape[0], 8):
            for c in range(0, dep.shape[1], 128):
                piece = dep[r:r + 8, c:c + 128]
                acc = piece if acc is None else acc | piece
        first = w[:8, :128] | (acc & zero_buf[...])
        return jnp.concatenate([jnp.concatenate([first, w[:8, 128:]], axis=1), w[8:, :]], axis=0)

    def after(dep):
        z = pltpu.bitcast(dep, U32)[:1, :] & zero_buf[:1, :]
        return lambda x: pltpu.bitcast(pltpu.bitcast(x, U32) | z, F32)

    side = []

    def take_side():
        f = side.pop(0) if side else None
        return None if f is None else f()

    def layer_norm(i, piece=0, npieces=1):
        n = T // npieces
        r0 = i * T + piece * n
        x = x_buf[r0:r0 + n, :].astype(F32)
        m = jnp.mean(x, axis=-1, keepdims=True)
        mb = _rb(m)
        d = x - mb
        v = jnp.mean(d * d, axis=-1, keepdims=True) - (m - mb) * (m - mb)
        den = _rb(jnp.sqrt(_rb(_rb(v) + EPS_LN)))
        inv = pl.reciprocal(den, approx=True)
        inv = inv * (2.0 - den * inv)
        xn = _pk((_rb(d) * inv).astype(BF16))
        xn_buf[r0 // 2:(r0 + n) // 2, :] = xn
        return xn

    def ln_pieces(i):
        return [lambda p=p: layer_norm(i, p, LNP) for p in range(LNP)]

    def load_wt(r0, r1, dep=None, dep2=None):
        w = wt_buf[r0 // 2:r1 // 2, :]
        if dep is not None:
            w = tie(w, dep)
        if dep2 is not None:
            w = jnp.concatenate([w[:, :D // 2], tie(w[:, D // 2:], dep2)], axis=1)
        return _upk(w)

    def fold(j):
        for u in range(MC // 128):
            w = _upk(w_buf[j, :, u * 128:(u + 1) * 128])
            if j < 2 * NC:
                r = _dot_nt(_upk(bdt_buf[(2 * j + u) % 8]), w) * LOG2E
            elif j == 2 * NC:
                r = _dot_nt(_upk(bdt_buf[8]), w)
            else:
                r = w.astype(F32).T
            row = (j * MC + u * 128 + (KROW - D if j >= NC else 0)) // 2
            wt_buf[row:row + 64, :] = _pk(r.astype(BF16))

    ri = lax.broadcasted_iota(jnp.int32, (128, 128), 0)
    ci = lax.broadcasted_iota(jnp.int32, (128, 128), 1)

    def build_bdt(g):
        wg4 = wphi_buf[4 * g:4 * g + 4].reshape(128, 32)
        t = jnp.concatenate([wg4.astype(F32).T] * 4, axis=0)
        b = _pk(jnp.where((ri // 32) == (ci // 32), t, 0.0).astype(BF16))
        bdt_buf[g] = b
        return b

    class KV:
        def __init__(self, i):
            self.i = i
            self.pk, self.vt, self.ph = {}, {}, {}

        def half(self, r0, r1, n, pieces):
            row = (self.i * T + n * 128) // 2
            deps = [take_side() for _ in range(pieces)]
            return _dot_nt(load_wt(r0, r1, *deps), _upk(xn_buf[row:row + 64, :]))

        def proj(self, r0, r1, pieces):
            return jnp.concatenate([self.half(r0, r1, n, pieces) for n in range(2)], axis=1)

        def k(self, c, pieces=0):
            if c == 0:
                kr = self.proj(KROW - 16, KROW + MC, pieces)
                r_buf[self.i] = kr[:8, :]
                self.pk[c] = kr[16:, :]
            else:
                self.pk[c] = self.proj(KROW + c * MC, KROW + (c + 1) * MC, pieces)

        def v(self, c, pieces=0):
            self.vt[c] = self.proj(VROW + c * MC, VROW + (c + 1) * MC, pieces).astype(BF16)

        def v_half(self, c, n):
            r = self.half(VROW + c * MC, VROW + (c + 1) * MC, n, 0).astype(BF16)
            self.vt[c] = r if n == 0 else jnp.concatenate([self.vt[c], r], axis=1)

        def phi(self, c):
            if c not in self.ph:
                pk = self.pk.pop(c)
                self.ph[c] = []
                for u in range(PC):
                    phi, _ = _phi_pair(pk[64 * u:64 * u + 64, :])
                    z = phi[:, :128] + phi[:, 128:]
                    if self.i > 0:
                        z = z + z_acc[c * PC + u]
                    z_acc[c * PC + u] = z
                    self.ph[c].append((phi.astype(BF16), z))
            return self.ph[c]

        def g(self, c):
            vt = self.vt.pop(c)
            for u, (phi, z) in enumerate(self.phi(c)):
                r = _dot_nt(_upk(tie(_pk(vt[64 * u:64 * u + 64, :]), pltpu.bitcast(z, U32))), phi)
                if self.i == 0:
                    g_acc[c * PC + u] = r
                else:
                    g_acc[c * PC + u] += r

    bdt_buf[8] = _pk(jnp.where(ri == ci, 1.0, 0.0).astype(BF16))
    x_cp[0].wait()
    layer_norm(0)
    t0, t1 = KV(0), KV(1)
    wr_cp.wait()
    v_cp[0].wait()
    fold(2 * NC)
    t0.v_half(0, 0)
    x_cp[1].wait()
    t0.v_half(0, 1)
    layer_norm(1)
    t1.v_half(0, 0)
    v_cp[1].wait()
    fold(2 * NC + 1)
    t1.v_half(0, 1)
    t0.v(1)
    t1.v(1)
    phi_cp.wait()
    k_cp[0].wait()
    wt_buf[D // 2:D // 2 + 8, :] = _pk(
        jnp.broadcast_to(wr_buf[...].astype(F32).reshape(1, D), (16, D)).astype(BF16))
    build_bdt(0)
    build_bdt(1)
    side += [None] * 2 + [lambda g=g: build_bdt(g) for g in range(2, 8)]
    fold(NC)
    t0.k(0, 2)
    t1.k(0, 2)
    t0.g(0)
    t1.phi(0)
    for cp in [k_cp[1], v_cp[2], k_cp[2]]:
        cp.wait()
    fold(NC + 1)
    fold(2 * NC + 2)
    fold(NC + 2)
    t1.g(0)
    t0.k(1)
    t1.k(1)
    t0.k(2)
    t0.g(1)
    t1.k(2)
    t1.g(1)
    t0.v(2)
    t1.v(2)
    t0.g(2)
    t1.phi(2)
    for cp in [v_cp[3], k_cp[3]] + x_cp[2:]:
        cp.wait()
    side += ln_pieces(2)
    fold(NC + 3)
    fold(2 * NC + 3)
    t1.g(2)
    t0.k(3, 2)
    t1.k(3, 2)
    t0.v(3, 2)
    t1.v(3, 2)
    t0.g(3)
    prev = t1
    for i in range(2, NT):
        if i + 1 < NT:
            side += ln_pieces(i + 1)
        kv = KV(i)
        for c in range(NC):
            kv.k(c, KPIECES[c])
            (prev if c == 0 else kv).g((c - 1) % NC)
            kv.v(c, VPIECES[c])
        prev = kv
    prev.g(NC - 1)
    assert not side

    same_head = (lax.broadcasted_iota(jnp.int32, (64, 128), 0) // 32
                 == (lax.broadcasted_iota(jnp.int32, (64, 128), 1) % 64) // 32)
    for p in range(NP):
        g_buf[p] = _pk(jnp.where(same_head, g_acc[p], 0.0).astype(BF16))
        zb_buf[p] = jnp.broadcast_to(jnp.sum(z_acc[p], axis=1, keepdims=True), (128, 128))

    r_all = _rb(r_buf[...])
    tok = (lax.broadcasted_iota(jnp.int32, r_buf.shape, 0) * T
           + lax.broadcasted_iota(jnp.int32, r_buf.shape, 2))
    r_max = jnp.max(r_all)
    idx = jnp.min(jnp.where(r_all == r_max, tok, S - 1))
    sel_tile = idx // T
    blk = pl.multiple_of((idx // 16) * 16, 16)

    def tile_of(j):
        return (sel_tile + 1 + j) % NT

    def out_copy(j):
        rows = pl.ds(pl.multiple_of(tile_of(j) * T, T), T)
        return pltpu.make_async_copy(out_buf.at[rows, :], out_hbm.at[rows, :], sem_o.at[j])

    def last_copy(n):
        rows = pl.ds(pl.multiple_of(sel_tile * T, T), T)
        cols = pl.ds(n * 128, 128)
        return pltpu.make_async_copy(out_buf.at[rows, cols], out_hbm.at[rows, cols], sem_o.at[NT - 1 + n])

    class Q:
        def __init__(self, j):
            self.j = j
            self.row0 = tile_of(j) * (T // 2)
            self.pq = {}

        def proj(self, c, n):
            xn = _upk(xn_buf[pl.ds(pl.multiple_of(self.row0 + n * 64, 64), 64), :])
            self.pq[c, n] = _dot_nt(load_wt(c * MC, (c + 1) * MC), xn)

        def num(self, c, n):
            pq = self.pq.pop((c, n))
            parts = []
            link = []
            for u in range(PC):
                phi, scale = _phi_pair(pq[64 * u:64 * u + 64, :], link, after)
                nd = _dot(_upk(g_buf[c * PC + u]), phi.astype(BF16))
                zp = phi * zb_buf[c * PC + u]
                zp = zp[:64, :] + zp[64:, :]
                for a in range(2):
                    den = jnp.sum(zp[32 * a:32 * a + 32, :], axis=0, keepdims=True) + 1e-6 * scale[a]
                    parts.append(nd[32 * a:32 * a + 32, :] * pl.reciprocal(den, approx=True))
            ot = jnp.concatenate(parts, axis=0)
            o_buf[self.j % 2, n * 64:(n + 1) * 64, c * MC:(c + 1) * MC] = _pk(ot.T.astype(BF16))

    def out_cols(j, n, upd=None):
        t = tile_of(j)
        rows = pl.ds(pl.multiple_of(t * T, T), T)
        rows2 = pl.ds(pl.multiple_of(t * (T // 2), T // 2), T // 2)
        cols = slice(n * 128, (n + 1) * 128)
        s = _dot(_upk(o_buf[j % 2]), _upk(wo_buf[:, cols]))
        xn = _upk(xn_buf[rows2, cols]).astype(F32)
        if upd is not None:
            xn = xn + upd[:, cols]
        out_buf[rows, cols] = (x_buf[rows, cols].astype(F32) + s * _silu(xn)).astype(BF16)

    def ffn_steps():
        st = {}
        KH = D // 2

        def apart(r):
            z = zero_buf[...]
            return pltpu.bitcast(pltpu.bitcast(r, U32) | jnp.concatenate([z, z], axis=0), F32)

        def up(w_ref, key, n, h):
            def f():
                xs = _upk(xn_buf[pl.ds(pl.multiple_of(blk // 2, 8), 8), h * KH:(h + 1) * KH])
                r = _dot(xs, _upk(w_ref[h * KH // 2:(h + 1) * KH // 2, n * 128:(n + 1) * 128]))
                st[key, n] = apart(r) if h == 0 else st[key, n] + r
            return f

        def down(c, n):
            def f():
                if ('h', c) not in st:
                    ms = range(c * FC // 128, (c + 1) * FC // 128)
                    st['h', c] = jnp.concatenate(
                        [_silu(st.pop(('g', m))) * st.pop(('u', m)) for m in ms], axis=1).astype(BF16)
                r = _dot(st['h', c], _upk(wd_buf[c * FC // 2:(c + 1) * FC // 2, n * 128:(n + 1) * 128]))
                st['y', n] = apart(r) if c == 0 else st['y', n] + r
            return f

        steps = []
        for c in range(F // FC + 1):
            ups = [up(w, k, m, h) for m in range(c * FC // 128, (c + 1) * FC // 128)
                   for h in range(2) for w, k in ((wg_buf, 'g'), (wu_buf, 'u'))] if c < F // FC else []
            downs = [down(c - 1, n) for n in range(D // 128)] if c > 0 else []
            while ups or downs:
                steps += ups[:2] + downs[:1]
                ups, downs = ups[2:], downs[1:]
        return steps, st

    for cp in q_cp + [wo_cp] + f_cp:
        cp.wait()
    for j in range(NC):
        fold(j)
    ffn, ffn_st = ffn_steps()

    q = Q(0)
    for c in range(NC):
        q.proj(c, 0)
        if c > 0:
            q.num(c - 1, 1)
        q.proj(c, 1)
        q.num(c, 0)

    pending = [None]

    def out_step():
        step = pending.pop(0)
        if step is not None:
            out_cols(*step)
            if step[1] == D // 128 - 1:
                out_copy(step[0]).start()

    for j in range(1, NT):
        qn = Q(j)
        pending += [(j - 1, n) for n in range(D // 128)]
        for c in range(NC):
            for tok in PATTERN:
                if tok == 'P' or tok == 'Q':
                    qn.proj(c, int(tok == 'Q'))
                elif tok == 'n':
                    (q if c == 0 else qn).num((c - 1) % NC, 1)
                elif tok == 'm':
                    qn.num(c, 0)
                elif tok == 'W':
                    out_step()
                else:
                    ffn.pop(0)()
        q = qn
    assert not ffn
    q.num(NC - 1, 1)
    out_step()

    y = jnp.concatenate([ffn_st['y', n] for n in range(D // 128)], axis=1)
    sub = lax.broadcasted_iota(jnp.int32, (16, D), 0)
    y_row = jnp.sum(jnp.where(sub == idx - blk, y, 0.0), axis=0, keepdims=True)
    gate = 1.0 / (1.0 + jnp.exp(-jnp.full((1, D), r_max, F32)))
    trow = lax.broadcasted_iota(jnp.int32, (T, D), 0)
    upd = jnp.where(trow == idx - sel_tile * T, y_row * gate, 0.0)
    for n in range(D // 128):
        out_cols(NT - 1, n, upd)
        last_copy(n).start()
    for j in range(NT - 1):
        out_copy(j).wait()
    for n in range(D // 128):
        last_copy(n).wait()


@jax.jit
def pallas_recurrent_scan__linear_kernel_hedgehog__moe_arch_mod__prompt_kernel(
    A_x: jax.Array,
    A_wqkv: jax.Array,
    A_w_phi: jax.Array,
    A_wo: jax.Array,
    B_x: jax.Array,
    B_w_r: jax.Array,
    B_w_gate: jax.Array,
    B_w_up: jax.Array,
    B_w_down: jax.Array,
):
    del B_x
    any_spec = pl.BlockSpec(memory_space=pl.ANY)
    out = pl.pallas_call(
        _kernel,
        out_shape=jax.ShapeDtypeStruct((S, D), BF16),
        in_specs=[any_spec] * 8,
        out_specs=any_spec,
        scratch_shapes=[
            pltpu.VMEM((S, D), BF16),
            pltpu.VMEM((S // 2, D), U32),
            pltpu.VMEM((3 * NC, D // 2, MC), U32),
            pltpu.VMEM(((VROW + D) // 2, D), U32),
            pltpu.VMEM((H, DH, DH), BF16),
            pltpu.VMEM((D,), BF16),
            pltpu.VMEM((D // 2, D), U32),
            pltpu.VMEM((D // 2, F), U32),
            pltpu.VMEM((D // 2, F), U32),
            pltpu.VMEM((F // 2, D), U32),
            pltpu.VMEM((9, 64, 128), U32),
            pltpu.VMEM((NP, 64, 128), F32),
            pltpu.VMEM((NP, 32, 128), U32),
            pltpu.VMEM((NP, 128, 128), F32),
            pltpu.VMEM((NP, 128, 128), F32),
            pltpu.VMEM((NT, 8, T), F32),
            pltpu.VMEM((2, T // 2, D), U32),
            pltpu.VMEM((S, D), BF16),
            pltpu.VMEM((8, 128), U32),
            pltpu.SemaphoreType.DMA((NT,)),
            pltpu.SemaphoreType.DMA((3 * NC,)),
            pltpu.SemaphoreType.DMA((6,)),
            pltpu.SemaphoreType.DMA((NT - 1 + D // 128,)),
        ],
        compiler_params=pltpu.CompilerParams(
            vmem_limit_bytes=100 * 1024 * 1024,
            disable_bounds_checks=True,
            disable_semaphore_checks=True,
        ),
        name="hedgehog_mod",
    )(A_x.reshape(S, D), A_wqkv, A_w_phi, A_wo, B_w_r, B_w_gate, B_w_up, B_w_down)
    return out.reshape(1, S, D)
```

```python
import jax
import jax.numpy as jnp
from jax import lax
import jax.experimental.pallas as pl
import jax.experimental.pallas.tpu as pltpu

S, D, H, DH, F = 2048, 1024, 32, 32, 3584
T = 256
NT = S // T
MC = 256
NC = D // MC
PC = MC // 64
NP = H // 2
FC = 512
LNP = 16
PATTERN = "PQffWfnmWf"
KPIECES = (1, 2, 2, 0)
VPIECES = (1, 1, 1, 0)
UP_STEPS = (3, 3, 5, 5, 5)
KROW = D + 16
VROW = KROW + D
LOG2E = 1.4426950408889634
EPS_LN = 1.0013580322265625e-05
F32 = jnp.float32
BF16 = jnp.bfloat16
U32 = jnp.uint32

_NT_DIMS = (((1,), (1,)), ((), ()))


def _dot_nt(a, b):
    return lax.dot_general(a, b, _NT_DIMS, preferred_element_type=F32)


def _dot(a, b):
    return jnp.dot(a, b, preferred_element_type=F32)


def _rb(x):
    return x.astype(BF16).astype(F32)


def _pk(x):
    return pltpu.bitcast(x, U32)


def _upk(x):
    return pltpu.bitcast(x, BF16)


def _phi_pair(p, link=None, link_after=None):
    pos, neg, scale = [], [], []
    for a in range(2):
        ph = p[32 * a:32 * a + 32, :]
        mx = jnp.max(ph, axis=0, keepdims=True)
        mn = jnp.min(ph, axis=0, keepdims=True)
        if link:
            mx = link[0](mx)
        ep = jnp.exp2(ph - mx)
        en = jnp.exp2(mn - ph)
        sp = jnp.sum(ep, axis=0, keepdims=True)
        rn = pl.reciprocal(jnp.sum(en, axis=0, keepdims=True), approx=True)
        if link is None:
            pos.append(ep * pl.reciprocal(sp, approx=True))
            neg.append(en * rn)
        else:
            if a == 1:
                link[:] = [link_after(ep[24:32, :])]
            pos.append(ep)
            neg.append(en * (sp * rn))
            scale.append(sp)
    return jnp.concatenate(pos + neg, axis=0), scale


def _silu(x):
    h = 0.5 * x
    return h + h * jnp.tanh(h)


def _kernel(x_hbm, wqkv_hbm, wphi_hbm, wo_hbm, wr_hbm, wg_hbm, wu_hbm, wd_hbm, out_hbm,
            x_buf, xn_buf, w_buf, wt_buf, wphi_buf, wr_buf, wo_buf, wg_buf, wu_buf, wd_buf,
            bdt_buf, g_acc, g_buf, z_acc, zb_buf, r_buf, o_buf, out_buf, zero_buf, xb_buf,
            sem_x, sem_w, sem_s, sem_o):
    x_cp = [pltpu.make_async_copy(x_hbm.at[rows, :], x_buf.at[rows, :], sem_x.at[i])
            for i, rows in enumerate([pl.ds(0, T), pl.ds(T, T), pl.ds(2 * T, S - 2 * T)])]
    w_cp = [pltpu.make_async_copy(wqkv_hbm.bitcast(U32).at[:, pl.ds(j * MC, MC)], w_buf.at[j], sem_w.at[j])
            for j in range(3 * NC)]
    q_cp, k_cp, v_cp = w_cp[:NC], w_cp[NC:2 * NC], w_cp[2 * NC:]
    phi_cp = pltpu.make_async_copy(wphi_hbm, wphi_buf, sem_s.at[0])
    wr_cp = pltpu.make_async_copy(wr_hbm, wr_buf, sem_s.at[1])
    wo_cp = pltpu.make_async_copy(wo_hbm.bitcast(U32), wo_buf, sem_s.at[2])
    f_cp = [pltpu.make_async_copy(wg_hbm.bitcast(U32), wg_buf, sem_s.at[3]),
            pltpu.make_async_copy(wu_hbm.bitcast(U32), wu_buf, sem_s.at[4]),
            pltpu.make_async_copy(wd_hbm.bitcast(U32), wd_buf, sem_s.at[5])]

    copies = [x_cp[0], wr_cp, v_cp[0], x_cp[1], v_cp[1], phi_cp, k_cp[0], k_cp[1], v_cp[2], k_cp[2],
              v_cp[3], k_cp[3]] + x_cp[2:] + q_cp + [wo_cp] + f_cp

    def start_all(j, carry):
        for k, cp in enumerate(copies):
            pl.when((k + 2) * j == j)(cp.start)
        zero_buf[...] = jnp.zeros_like(zero_buf)
        return carry

    lax.fori_loop(0, 2, start_all, 0)

    def tie(w, dep):
        acc = None
        for r in range(0, dep.shape[0], 8):
            for c in range(0, dep.shape[1], 128):
                piece = dep[r:r + 8, c:c + 128]
                acc = piece if acc is None else acc | piece
        first = w[:8, :128] | (acc & zero_buf[...])
        return jnp.concatenate([jnp.concatenate([first, w[:8, 128:]], axis=1), w[8:, :]], axis=0)

    def after(dep):
        z = pltpu.bitcast(dep, U32)[:1, :] & zero_buf[:1, :]
        return lambda x: pltpu.bitcast(pltpu.bitcast(x, U32) | z, F32)

    side = []

    def take_side():
        f = side.pop(0) if side else None
        return None if f is None else f()

    def layer_norm(i, piece=0, npieces=1):
        n = T // npieces
        r0 = i * T + piece * n
        x = x_buf[r0:r0 + n, :].astype(F32)
        m = jnp.mean(x, axis=-1, keepdims=True)
        mb = _rb(m)
        d = x - mb
        v = jnp.mean(d * d, axis=-1, keepdims=True) - (m - mb) * (m - mb)
        den = _rb(jnp.sqrt(_rb(_rb(v) + EPS_LN)))
        inv = pl.reciprocal(den, approx=True)
        inv = inv * (2.0 - den * inv)
        xn = _pk((_rb(d) * inv).astype(BF16))
        xn_buf[r0 // 2:(r0 + n) // 2, :] = xn
        return xn

    def ln_pieces(i):
        return [lambda p=p: layer_norm(i, p, LNP) for p in range(LNP)]

    def load_wt(r0, r1, dep=None, dep2=None):
        w = wt_buf[r0 // 2:r1 // 2, :]
        if dep is not None:
            w = tie(w, dep)
        if dep2 is not None:
            w = jnp.concatenate([w[:, :D // 2], tie(w[:, D // 2:], dep2)], axis=1)
        return _upk(w)

    def fold(j, hook=None):
        for u in range(MC // 128):
            w = _upk(w_buf[j, :, u * 128:(u + 1) * 128])
            if j < 2 * NC:
                r = _dot_nt(_upk(bdt_buf[(2 * j + u) % 8]), w) * LOG2E
            elif j == 2 * NC:
                r = _dot_nt(_upk(bdt_buf[8]), w)
            else:
                r = w.astype(F32).T
            if hook is not None:
                hook(r[:, :128], 4)
            row = (j * MC + u * 128 + (KROW - D if j >= NC else 0)) // 2
            wt_buf[row:row + 64, :] = _pk(r.astype(BF16))

    ri = lax.broadcasted_iota(jnp.int32, (128, 128), 0)
    ci = lax.broadcasted_iota(jnp.int32, (128, 128), 1)

    def build_bdt(g):
        wg4 = wphi_buf[4 * g:4 * g + 4].reshape(128, 32)
        t = jnp.concatenate([wg4.astype(F32).T] * 4, axis=0)
        b = _pk(jnp.where((ri // 32) == (ci // 32), t, 0.0).astype(BF16))
        bdt_buf[g] = b
        return b

    class KV:
        def __init__(self, i):
            self.i = i
            self.pk, self.vt, self.ph = {}, {}, {}

        def half(self, r0, r1, n, pieces):
            row = (self.i * T + n * 128) // 2
            deps = [take_side() for _ in range(pieces)]
            return _dot_nt(load_wt(r0, r1, *deps), _upk(xn_buf[row:row + 64, :]))

        def proj(self, r0, r1, pieces):
            return jnp.concatenate([self.half(r0, r1, n, pieces) for n in range(2)], axis=1)

        def k(self, c, pieces=0):
            if c == 0:
                kr = self.proj(KROW - 16, KROW + MC, pieces)
                r_buf[self.i] = kr[:8, :]
                self.pk[c] = kr[16:, :]
            else:
                self.pk[c] = self.proj(KROW + c * MC, KROW + (c + 1) * MC, pieces)

        def v(self, c, pieces=0):
            self.vt[c] = self.proj(VROW + c * MC, VROW + (c + 1) * MC, pieces).astype(BF16)

        def v_half(self, c, n):
            r = self.half(VROW + c * MC, VROW + (c + 1) * MC, n, 0).astype(BF16)
            self.vt[c] = r if n == 0 else jnp.concatenate([self.vt[c], r], axis=1)

        def phi(self, c):
            if c not in self.ph:
                pk = self.pk.pop(c)
                self.ph[c] = []
                for u in range(PC):
                    phi, _ = _phi_pair(pk[64 * u:64 * u + 64, :])
                    z = phi[:, :128] + phi[:, 128:]
                    if self.i > 0:
                        z = z + z_acc[c * PC + u]
                    z_acc[c * PC + u] = z
                    self.ph[c].append((phi.astype(BF16), z))
            return self.ph[c]

        def g(self, c):
            vt = self.vt.pop(c)
            for u, (phi, z) in enumerate(self.phi(c)):
                r = _dot_nt(_upk(tie(_pk(vt[64 * u:64 * u + 64, :]), pltpu.bitcast(z, U32)[96:, :])), phi)
                if self.i == 0:
                    g_acc[c * PC + u] = r
                else:
                    g_acc[c * PC + u] += r

    bdt_buf[8] = _pk(jnp.where(ri == ci, 1.0, 0.0).astype(BF16))
    x_cp[0].wait()
    layer_norm(0)
    t0, t1 = KV(0), KV(1)
    wr_cp.wait()
    v_cp[0].wait()
    fold(2 * NC)
    t0.v_half(0, 0)
    x_cp[1].wait()
    t0.v_half(0, 1)
    layer_norm(1)
    t1.v_half(0, 0)
    v_cp[1].wait()
    fold(2 * NC + 1)
    t1.v_half(0, 1)
    t0.v(1)
    t1.v_half(1, 0)
    phi_cp.wait()
    k_cp[0].wait()
    wt_buf[D // 2:D // 2 + 8, :] = _pk(
        jnp.broadcast_to(wr_buf[...].astype(F32).reshape(1, D), (16, D)).astype(BF16))
    build_bdt(0)
    build_bdt(1)
    side += [None] * 2 + [lambda g=g: build_bdt(g) for g in range(2, 8)]
    t1.v_half(1, 1)
    fold(NC)
    t0.k(0, 2)
    t1.k(0, 2)
    t0.g(0)
    t1.phi(0)
    for cp in [k_cp[1], v_cp[2], k_cp[2]]:
        cp.wait()
    fold(NC + 1)
    fold(2 * NC + 2)
    fold(NC + 2)
    t1.g(0)
    t0.k(1)
    t1.k(1)
    t0.k(2)
    t0.g(1)
    t1.k(2)
    t1.g(1)
    t0.v(2)
    t1.v(2)
    t0.g(2)
    t1.phi(2)
    for cp in [v_cp[3], k_cp[3]] + x_cp[2:]:
        cp.wait()
    side += ln_pieces(2)
    fold(NC + 3)
    fold(2 * NC + 3)
    t1.g(2)
    t0.k(3, 2)
    t1.k(3, 2)
    t0.v(3, 2)
    t1.v(3, 2)
    t0.g(3)
    prev = t1

    def route():
        r_all = _rb(r_buf[...])
        tok = (lax.broadcasted_iota(jnp.int32, r_buf.shape, 0) * T
               + lax.broadcasted_iota(jnp.int32, r_buf.shape, 2))
        r_max = jnp.max(jnp.max(r_all, axis=0), axis=1, keepdims=True)
        idx = jnp.min(jnp.where(r_all == r_max[None], tok, S - 1))
        return r_max, idx, idx // T, pl.multiple_of((idx // 16) * 16, 16)

    def xb_piece(k):
        _, idx, _, blk = routed
        xs = _upk(xn_buf[pl.ds(pl.multiple_of(blk // 2, 8), 8), k * 128:(k + 1) * 128]).astype(F32)
        sub = lax.broadcasted_iota(jnp.int32, (16, 128), 0)
        row = jnp.sum(jnp.where(sub == idx - blk, xs, 0.0), axis=0, keepdims=True)
        xb = jnp.broadcast_to(row, (128, 128)).T
        xb_buf[k * 128:(k + 1) * 128, :] = xb
        return pltpu.bitcast(xb, U32)

    for i in range(2, NT):
        if i + 1 < NT:
            side += ln_pieces(i + 1)
        kv = KV(i)
        for c in range(NC):
            kv.k(c, KPIECES[c])
            if (i, c) == (NT - 1, 0):
                routed = route()
                side += [None] * 4 + [lambda k=k: xb_piece(k) for k in range(D // 128)]
            (prev if c == 0 else kv).g((c - 1) % NC)
            kv.v(c, VPIECES[c])
        prev = kv
    prev.g(NC - 1)
    while side:
        take_side()

    same_head = (lax.broadcasted_iota(jnp.int32, (64, 128), 0) // 32
                 == (lax.broadcasted_iota(jnp.int32, (64, 128), 1) % 64) // 32)
    for p in range(NP):
        g_buf[p] = _pk(jnp.where(same_head, g_acc[p], 0.0).astype(BF16))
        zb_buf[p] = jnp.broadcast_to(jnp.sum(z_acc[p], axis=1, keepdims=True), (128, 128))

    r_max, idx, sel_tile, _ = routed

    def tile_of(j):
        return (sel_tile + 1 + j) % NT

    def out_copy(j):
        rows = pl.ds(pl.multiple_of(tile_of(j) * T, T), T)
        return pltpu.make_async_copy(out_buf.at[rows, :], out_hbm.at[rows, :], sem_o.at[j])

    def last_copy(n):
        rows = pl.ds(pl.multiple_of(sel_tile * T, T), T)
        cols = pl.ds(n * 128, 128)
        return pltpu.make_async_copy(out_buf.at[rows, cols], out_hbm.at[rows, cols], sem_o.at[NT - 1 + n])

    up_steps = []

    def anchored(r, kind):
        dep = r[:8, :]
        for _ in range(min(UP_STEPS[kind], len(up_steps))):
            dep = up_steps.pop(0)(pltpu.bitcast(pltpu.bitcast(dep, U32) & zero_buf[...], F32))

    class Q:
        def __init__(self, j):
            self.j = j
            self.row0 = tile_of(j) * (T // 2)
            self.pq = {}

        def proj(self, c, n):
            xn = _upk(xn_buf[pl.ds(pl.multiple_of(self.row0 + n * 64, 64), 64), :])
            self.pq[c, n] = _dot_nt(load_wt(c * MC, (c + 1) * MC), xn)
            anchored(self.pq[c, n], n)

        def num(self, c, n):
            pq = self.pq.pop((c, n))
            parts = []
            link = []
            for u in range(PC):
                phi, scale = _phi_pair(pq[64 * u:64 * u + 64, :], link, after)
                nd = _dot(_upk(g_buf[c * PC + u]), phi.astype(BF16))
                zp = phi * zb_buf[c * PC + u]
                zp = zp[:64, :] + zp[64:, :]
                for a in range(2):
                    den = jnp.sum(zp[32 * a:32 * a + 32, :], axis=0, keepdims=True) + 1e-6 * scale[a]
                    parts.append(nd[32 * a:32 * a + 32, :] * pl.reciprocal(den, approx=True))
            ot = jnp.concatenate(parts, axis=0)
            o_buf[self.j % 2, n * 64:(n + 1) * 64, c * MC:(c + 1) * MC] = _pk(ot.T.astype(BF16))

    def out_cols(j, n, upd=None):
        t = tile_of(j)
        rows = pl.ds(pl.multiple_of(t * T, T), T)
        rows2 = pl.ds(pl.multiple_of(t * (T // 2), T // 2), T // 2)
        cols = slice(n * 128, (n + 1) * 128)
        s = _dot(_upk(o_buf[j % 2]), _upk(wo_buf[:, cols]))
        anchored(s, 2 + n % 2)
        xn = _upk(xn_buf[rows2, cols]).astype(F32)
        if upd is not None:
            xn = xn + upd[:, cols]
        out_buf[rows, cols] = (x_buf[rows, cols].astype(F32) + s * _silu(xn)).astype(BF16)

    def ffn_steps():
        st = {}

        def up(c, w_ref, key, m, e):
            def f(zero):
                p = (_upk(w_ref[e * 64:(e + 1) * 64, m * 128:(m + 1) * 128]).astype(F32)
                     * xb_buf[e * 128:(e + 1) * 128, :])
                accs = [zero, zero]
                for r in range(16):
                    accs[r % 2] = accs[r % 2] + p[8 * r:8 * r + 8, :]
                acc = accs[0] + accs[1]
                st[key, m] = acc if e == 0 else st[key, m] + acc
                if (key, (m + 1) % (FC // 128), e) == ('u', 0, D // 128 - 1):
                    h = [_silu(jnp.sum(st.pop(('g', k)), axis=0, keepdims=True))
                         * jnp.sum(st.pop(('u', k)), axis=0, keepdims=True)
                         for k in range(c * FC // 128, (c + 1) * FC // 128)]
                    st['h', c] = jnp.broadcast_to(jnp.concatenate(h, axis=1), (16, FC)).astype(BF16)
                return acc
            return f

        def apart(r):
            z = zero_buf[...]
            return pltpu.bitcast(pltpu.bitcast(r, U32) | jnp.concatenate([z, z], axis=0), F32)

        def down(c, n):
            def f():
                r = _dot(st['h', c], _upk(wd_buf[c * FC // 2:(c + 1) * FC // 2, n * 128:(n + 1) * 128]))
                st['y', n] = apart(r) if c == 0 else st['y', n] + r
            return f

        up_steps.extend(up(m * 128 // FC, w, k, m, e) for m in range(F // 128)
                        for w, k in ((wg_buf, 'g'), (wu_buf, 'u')) for e in range(D // 128))
        return [(c, down(c, n)) for c in range(F // FC) for n in range(D // 128)], st

    for cp in q_cp + [wo_cp] + f_cp:
        cp.wait()
    ffn, ffn_st = ffn_steps()
    for j in range(NC):
        fold(j, anchored)

    q = Q(0)
    for c in range(NC):
        q.proj(c, 0)
        if c > 0:
            q.num(c - 1, 1)
        q.proj(c, 1)
        q.num(c, 0)

    pending = [None]

    def out_step():
        step = pending.pop(0)
        if step is not None:
            out_cols(*step)
            if step[1] == D // 128 - 1:
                out_copy(step[0]).start()

    for j in range(1, NT):
        qn = Q(j)
        pending += [(j - 1, n) for n in range(D // 128)]
        for c in range(NC):
            for tok in PATTERN:
                if tok == 'P' or tok == 'Q':
                    qn.proj(c, int(tok == 'Q'))
                elif tok == 'n':
                    (q if c == 0 else qn).num((c - 1) % NC, 1)
                elif tok == 'm':
                    qn.num(c, 0)
                elif tok == 'W':
                    out_step()
                elif ffn and ('h', ffn[0][0]) in ffn_st:
                    ffn.pop(0)[1]()
        q = qn
    assert not ffn
    q.num(NC - 1, 1)
    out_step()

    y = jnp.concatenate([ffn_st['y', n] for n in range(D // 128)], axis=1)
    y_row = y[:1, :]
    gate = 1.0 / (1.0 + jnp.exp(-r_max[:1, :]))
    trow = lax.broadcasted_iota(jnp.int32, (T, D), 0)
    upd = jnp.where(trow == idx - sel_tile * T, y_row * gate, 0.0)
    for n in range(D // 128):
        out_cols(NT - 1, n, upd)
        last_copy(n).start()
    for j in range(NT - 1):
        out_copy(j).wait()
    for n in range(D // 128):
        last_copy(n).wait()


@jax.jit
def pallas_recurrent_scan__linear_kernel_hedgehog__moe_arch_mod__prompt_kernel(
    A_x: jax.Array,
    A_wqkv: jax.Array,
    A_w_phi: jax.Array,
    A_wo: jax.Array,
    B_x: jax.Array,
    B_w_r: jax.Array,
    B_w_gate: jax.Array,
    B_w_up: jax.Array,
    B_w_down: jax.Array,
):
    del B_x
    any_spec = pl.BlockSpec(memory_space=pl.ANY)
    out = pl.pallas_call(
        _kernel,
        out_shape=jax.ShapeDtypeStruct((S, D), BF16),
        in_specs=[any_spec] * 8,
        out_specs=any_spec,
        scratch_shapes=[
            pltpu.VMEM((S, D), BF16),
            pltpu.VMEM((S // 2, D), U32),
            pltpu.VMEM((3 * NC, D // 2, MC), U32),
            pltpu.VMEM(((VROW + D) // 2, D), U32),
            pltpu.VMEM((H, DH, DH), BF16),
            pltpu.VMEM((D,), BF16),
            pltpu.VMEM((D // 2, D), U32),
            pltpu.VMEM((D // 2, F), U32),
            pltpu.VMEM((D // 2, F), U32),
            pltpu.VMEM((F // 2, D), U32),
            pltpu.VMEM((9, 64, 128), U32),
            pltpu.VMEM((NP, 64, 128), F32),
            pltpu.VMEM((NP, 32, 128), U32),
            pltpu.VMEM((NP, 128, 128), F32),
            pltpu.VMEM((NP, 128, 128), F32),
            pltpu.VMEM((NT, 8, T), F32),
            pltpu.VMEM((2, T // 2, D), U32),
            pltpu.VMEM((S, D), BF16),
            pltpu.VMEM((8, 128), U32),
            pltpu.VMEM((D, 128), F32),
            pltpu.SemaphoreType.DMA((3,)),
            pltpu.SemaphoreType.DMA((3 * NC,)),
            pltpu.SemaphoreType.DMA((6,)),
            pltpu.SemaphoreType.DMA((NT - 1 + D // 128,)),
        ],
        compiler_params=pltpu.CompilerParams(
            vmem_limit_bytes=100 * 1024 * 1024,
            disable_bounds_checks=True,
            disable_semaphore_checks=True,
        ),
        name="hedgehog_mod",
    )(A_x.reshape(S, D), A_wqkv, A_w_phi, A_wo, B_w_r, B_w_gate, B_w_up, B_w_down)
    return out.reshape(1, S, D)
```
